```python
import os as _os
_os.environ.setdefault('JAX_PLATFORMS', 'cpu')
import jax
import jax.numpy as jnp

def _softmax(x, axis=-1):
    return jax.nn.softmax(x, axis=axis)

def _gelu(x):
    return jax.nn.gelu(x, approximate=True)

def _silu(x):
    return jax.nn.silu(x)

def _sigmoid(x):
    return jax.nn.sigmoid(x)

def _layernorm(x, axis=-1, eps=1e-05):
    m = jnp.mean(x, axis=axis, keepdims=True)
    v = jnp.var(x, axis=axis, keepdims=True)
    return (x - m) / jnp.sqrt(v + eps)

def _scatter_add(tgt, idx, src, axis=0):
    return tgt.at[idx].add(src)

def _segment_sum(src, seg, n):
    return jax.ops.segment_sum(src, seg, n)

class _Rng:

    def __init__(self, key):
        self._k = key

    def _next(self):
        self._k, sub = jax.random.split(self._k)
        return sub

    def normal(self, shape):
        return jax.random.normal(self._next(), shape, dtype=jnp.bfloat16)

    def randint(self, lo, hi, shape):
        return jax.random.randint(self._next(), shape, lo, hi, dtype=jnp.int32)

    def uniform(self, shape, lo=0.0, hi=1.0):
        return jax.random.uniform(self._next(), shape, jnp.bfloat16, lo, hi)

    def permutation(self, n):
        return jax.random.permutation(self._next(), n)
kernel_name = 'concat_heads__spectral_gfnet__memory_aug_recurrent_mem_tr__prompt'

def setup_inputs():
    _rng = _Rng(jax.random.key(int.from_bytes(__import__("os").urandom(4), "little")))
    _w = lambda a: (lambda t: t.astype(jnp.bfloat16) if jnp.issubdtype(t.dtype, jnp.floating) else t)(jnp.asarray(a))

    def _A_setup():
        B, S, D = (1, 2048, 512)
        Df = D // 2 + 1
        return {'x': _w((lambda *s: _rng.normal(s) * 0.05)(B, S, D)), 'w_r': _w((lambda *s: _rng.normal(s) * 0.05)(S, Df) * 0.02), 'w_i': _w((lambda *s: _rng.normal(s) * 0.05)(S, Df) * 0.02)}
    _A_in = _A_setup()

    def _B_setup():
        B, S, Dm = (1, 2048, 512)
        H, Dh = (32, 128)
        M, seg = (8, 32)
        seg = min(seg, S)
        S = S // seg * seg
        return {'x': _w((lambda *s: _rng.normal(s) * 0.05)(B, S, Dm)), 'mem0': _w((lambda *s: _rng.normal(s) * 0.4)(B, M, Dm)), 'Wq': _w((lambda *s: _rng.normal(s) * 3.2)(Dm, H, Dh) * Dm ** (-0.5)), 'Wk': _w((lambda *s: _rng.normal(s) * 3.2)(Dm, H, Dh) * Dm ** (-0.5)), 'Wv': _w((lambda *s: _rng.normal(s) * 0.4)(Dm, H, Dh) * Dm ** (-0.5)), 'Wo': _w((lambda *s: _rng.normal(s) * 0.4)(H, Dh, Dm) * (H * Dh) ** (-0.5)), 'seg_len': seg}
    _B_in = _B_setup()
    return {'A_x': _A_in['x'], 'A_w_r': _A_in['w_r'], 'A_w_i': _A_in['w_i'], 'B_x': _B_in['x'], 'B_mem0': _B_in['mem0'], 'B_Wq': _B_in['Wq'], 'B_Wk': _B_in['Wk'], 'B_Wv': _B_in['Wv'], 'B_Wo': _B_in['Wo'], 'B_seg_len': _B_in['seg_len']}

def reference(A_x, A_w_r, A_w_i, B_x, B_mem0, B_Wq, B_Wk, B_Wv, B_Wo, B_seg_len):

    def _A_ref(x, w_r, w_i):
        B, S, D = x.shape
        X = (lambda x, axes=(-2, -1): jnp.fft.rfft2(x.astype(jnp.float32), axes=axes))(x, axes=(-2, -1))
        W = w_r + 1j * w_i
        X = X * W
        y = (lambda x, s, axes=(-2, -1): jnp.fft.irfft2(x, s=s, axes=axes).astype(jnp.bfloat16))(X, (S, D), axes=(-2, -1))
        return y

    def _B_ref(x, mem0, Wq, Wk, Wv, Wo, seg_len):
        B, S, Dm = x.shape
        H, Dh = (Wq.shape[1], Wq.shape[2])
        M = mem0.shape[1]
        scale = Dh ** (-0.5)
        n_seg = S // seg_len
        L = M + seg_len
        idx = jnp.arange(L)
        mask = (idx[:, None] < M) | (idx[:, None] >= idx[None, :])
        mem = mem0
        outs = []
        for s in range(n_seg):
            xs = x[:, s * seg_len:(s + 1) * seg_len, :].copy()
            h = jnp.concatenate([mem, xs], axis=1)
            q = jnp.einsum('btd,dhe->bhte', h, Wq)
            k = jnp.einsum('btd,dhe->bhte', h, Wk)
            v = jnp.einsum('btd,dhe->bhte', h, Wv)
            scores = jnp.einsum('bhqe,bhke->bhqk', q, k) * scale
            scores = jnp.where(mask[None, None], scores, -1000000000.0)
            p = _softmax(scores, axis=-1)
            o = jnp.einsum('bhqk,bhke->bhqe', p, v)
            o = jnp.einsum('bhte,hed->btd', o, Wo)
            mem = o[:, :M, :].copy()
            outs.append(o[:, M:, :])
        return jnp.concatenate(outs, axis=1)
    a = _A_ref(A_x, A_w_r, A_w_i)
    b = _B_ref(B_x, B_mem0, B_Wq, B_Wk, B_Wv, B_Wo, B_seg_len)
    return jnp.concatenate([a, b], axis=-1)
```

```python
import math

import numpy as np
import jax
import jax.numpy as jnp
from jax import lax
import jax.experimental.pallas as pl
import jax.experimental.pallas.tpu as pltpu

S, D = 2048, 512
H, DH = 32, 128
MEM, SEG = 8, 32
NSEG = S // SEG
NP = H // 2
XT = 8
KEEP = SEG - XT
R2 = 2 * (MEM + SEG)
SCALE = DH ** -0.5
LOG2E = 1.4426950408889634
N1, N2 = 128, 16

f32, bf16, u32 = jnp.float32, jnp.bfloat16, jnp.uint32
NT = (((1,), (1,)), ((), ()))


def _pack_rows(m):
    b = np.asarray(m, np.float32).astype(jnp.bfloat16).view(np.uint16).astype(np.uint32)
    return b[..., 0::2, :] | (b[..., 1::2, :] << 16)


def _dft_tables():
    k = np.arange(D // 2)[:, None]
    d = np.arange(D)[None, :]
    ang = 2.0 * np.pi * ((k * d) % D) / D
    pm = np.cos(ang)
    qm = -np.sin(ang)
    qm[0] = (-1.0) ** np.arange(D)
    fdt = np.stack([pm.reshape(16, 16, D), qm.reshape(16, 16, D)], axis=1).reshape(D, D)
    wgt = np.where(k == 0, 1.0, 2.0) / (S * D)
    fi = np.concatenate([wgt * pm, wgt * qm], axis=0)
    n1 = np.arange(N1)[:, None]
    k1 = np.arange(N1)[None, :]
    mf = []
    for n2 in range(N2):
        a = 2.0 * np.pi * (((N2 * n1 + n2) * k1) % S) / S
        mf.append(np.concatenate([np.cos(a), np.sin(a)], axis=1))
    return _pack_rows(fdt), _pack_rows(fi), _pack_rows(np.stack(mf))


def _sadd(a, b):
    (sa, va), (sb, vb) = a, b
    if sa == sb:
        return (sa, va + vb)
    return (1, va - vb) if sa > 0 else (1, vb - va)


def _sneg(a):
    return (-a[0], a[1])


def _ssub(a, b):
    return _sadd(a, _sneg(b))


def _smul(a, c):
    return (a[0], a[1] * c) if c > 0 else (-a[0], a[1] * (-c))


def _cadd(a, b):
    return (_sadd(a[0], b[0]), _sadd(a[1], b[1]))


def _csub(a, b):
    return (_ssub(a[0], b[0]), _ssub(a[1], b[1]))


def _cmul_i(a, sgn):
    return (_sneg(a[1]), a[0]) if sgn > 0 else (a[1], _sneg(a[0]))


def _radix4(x, sgn):
    t0, t1 = _cadd(x[0], x[2]), _csub(x[0], x[2])
    t2, t3 = _cadd(x[1], x[3]), _cmul_i(_csub(x[1], x[3]), sgn)
    return [_cadd(t0, t2), _cadd(t1, t3), _csub(t0, t2), _csub(t1, t3)]


def _twiddle16(a, m, sgn):
    if m == 0:
        return a
    if m == 4:
        return _cmul_i(a, sgn)
    c, s = math.cos(2 * math.pi * m / 16), sgn * math.sin(2 * math.pi * m / 16)
    if m in (2, 6):
        if c * s > 0:
            return (_smul(_ssub(a[0], a[1]), c), _smul(_sadd(a[0], a[1]), c))
        return (_smul(_sadd(a[0], a[1]), c), _smul(_ssub(a[1], a[0]), c))
    return (_ssub(_smul(a[0], c), _smul(a[1], s)), _sadd(_smul(a[0], s), _smul(a[1], c)))


def _fft16(x, sgn):
    a = [_radix4([x[4 * n1 + n2] for n1 in range(4)], sgn) for n2 in range(4)]
    out = [None] * 16
    for k1 in range(4):
        y = _radix4([_twiddle16(a[n2][k1], n2 * k1, sgn) for n2 in range(4)], sgn)
        for k2 in range(4):
            out[k1 + 4 * k2] = y[k2]
    return out


def _val(a):
    return a[1] if a[0] > 0 else -a[1]


def _split_pairs(u):
    lo = pltpu.bitcast(u << 16, f32).astype(bf16)
    hi = pltpu.bitcast(u & jnp.uint32(0xFFFF0000), f32).astype(bf16)
    return lo, hi


_XE, _XA, _W, _FD, _MF, _WR, _WI, _WO, _XB, _FI, _M0, _OUT = 0, 1, 5, 17, 18, 19, 20, 21, 22, 23, 24, 25
_NSEM = 26


def _kernel(xa_hbm, wr_hbm, wi_hbm, xb_hbm, m0_hbm, wq_hbm, wk_hbm, wv_hbm, wo_hbm,
            fd_hbm, fi_hbm, mf_hbm, out_hbm,
            xe, xe32, xa, xst, xg, wst, wcp, wsl, xq, fd, fi, mf, wr, wi, tsc, rp, rq, rn,
            z32, wo, wo32, xb, m0, stage, sems):
    w_hbms = (wq_hbm, wk_hbm, wv_hbm)

    def cp_w(m, g):
        return pltpu.make_async_copy(w_hbms[m].at[:, pl.ds(8 * g, 8), :], wst.at[4 * m + g],
                                     sems.at[_W + 4 * m + g])

    def cp_xa(t):
        return pltpu.make_async_copy(xa_hbm.at[:, pl.ds(128 * t, 128)], xa.at[t], sems.at[_XA + t])

    cp_xe = pltpu.make_async_copy(xb_hbm.at[:, pl.ds(KEEP, XT), :], xe, sems.at[_XE])
    cp_fd = pltpu.make_async_copy(fd_hbm, fd, sems.at[_FD])
    cp_mf = pltpu.make_async_copy(mf_hbm, mf, sems.at[_MF])
    cp_wr = pltpu.make_async_copy(wr_hbm, wr, sems.at[_WR])
    cp_wi = pltpu.make_async_copy(wi_hbm, wi, sems.at[_WI])
    cp_wo = pltpu.make_async_copy(wo_hbm, wo, sems.at[_WO])
    cp_xb = pltpu.make_async_copy(xb_hbm, xb, sems.at[_XB])
    cp_fi = pltpu.make_async_copy(fi_hbm, fi, sems.at[_FI])
    cp_m0 = pltpu.make_async_copy(m0_hbm, m0, sems.at[_M0])

    cp_xe.start()
    for g in range(4):
        cp_w(0, g).start()
        cp_xa(g).start()
    cp_fd.start()
    cp_mf.start()
    cp_wr.start()
    cp_wi.start()
    for g in range(4):
        cp_w(1, g).start()
    cp_wo.start()
    for g in range(4):
        cp_w(2, g).start()
    cp_xb.start()
    cp_fi.start()
    cp_m0.start()

    def x_loop(m, pre, companion):
        def body(g, carry):
            g8 = pl.multiple_of(8 * g, 8)
            pltpu.make_async_copy(w_hbms[m].at[:, pl.ds(g8, 8), :], wst.at[4 * m + g],
                                  sems.at[_W + 4 * m + g]).wait()
            pre(g)
            wcp[...] = pltpu.bitcast(wst[4 * m + g].reshape(8 * D, DH), u32)
            lhs = pltpu.bitcast(xe32[...], bf16)
            for j in range(4):
                lo, hi = _split_pairs(wcp[pl.ds(j, D, stride=4), :])
                wsl[H * m + 8 * g + 2 * j] = pltpu.bitcast(lo, u32)
                wsl[H * m + 8 * g + 2 * j + 1] = pltpu.bitcast(hi, u32)
                y1 = jnp.dot(lhs, lo, preferred_element_type=f32).reshape(NSEG, XT, DH)
                y2 = jnp.dot(lhs, hi, preferred_element_type=f32).reshape(NSEG, XT, DH)
                xq[NP * m + 4 * g + j] = jnp.concatenate([y1, y2], axis=1).astype(bf16)
            companion(g)
            return carry
        lax.fori_loop(0, 4, body, 0)

    cp_xe.wait()
    xe32[...] = pltpu.bitcast(xe[...].reshape(NSEG * XT, D), u32)

    def wait_xa(t):
        t128 = pl.multiple_of(128 * t, 128)
        pltpu.make_async_copy(xa_hbm.at[:, pl.ds(t128, 128)], xa.at[t], sems.at[_XA + t]).wait()

    def gather_x(t):
        xst[...] = pltpu.bitcast(xa[t], u32)
        for j in range(8):
            lo, hi = _split_pairs(xst[pl.ds(j, N1, stride=8), :])
            xg[2 * j, t] = lo
            xg[2 * j + 1, t] = hi

    x_loop(0, wait_xa, gather_x)

    cp_fd.wait()
    cp_mf.wait()
    row8 = lax.broadcasted_iota(jnp.int32, (8, 2 * N1), 0)

    def a1(n2):
        xn = jnp.concatenate([xg[n2, t] for t in range(4)], axis=1)
        yt = lax.dot_general(pltpu.bitcast(fd[...], bf16), xn, NT, preferred_element_type=f32)
        return yt.astype(bf16)

    def s_fwd(n2, yt):
        g = pltpu.bitcast(mf[n2], bf16)
        for hf in range(2):
            cs = jnp.dot(yt[256 * hf:256 * hf + 256], g, preferred_element_type=f32)
            cs = cs.reshape(8, 32, 2 * N1)
            p = cs[:, 0:16, :].reshape(128, 2 * N1)
            q = cs[:, 16:32, :].reshape(128, 2 * N1)
            if hf == 0:
                q0 = q[0:8]
                tsc[n2, 0, 256:264, :] = q0[:, :N1]
                tsc[n2, 1, 256:264, :] = -q0[:, N1:]
                q = jnp.concatenate([jnp.where(row8 == 0, 0.0, q0), q[8:]], axis=0)
            tsc[n2, 0, 128 * hf:128 * hf + 128, :] = p[:, :N1] + q[:, N1:]
            tsc[n2, 1, 128 * hf:128 * hf + 128, :] = q[:, :N1] - p[:, N1:]

    def fwd_body(i, carry):
        yts = [a1(4 * i)]
        for k in range(4):
            if k + 1 < 4:
                yts.append(a1(4 * i + k + 1))
            s_fwd(4 * i + k, yts[k])
        return carry
    lax.fori_loop(0, 4, fwd_body, 0)

    cp_wr.wait()
    cp_wi.wait()

    def spectral_unit(rows, w_rows):
        t = [((1, tsc[n2, 0, rows, :]), (1, tsc[n2, 1, rows, :])) for n2 in range(N2)]
        x = _fft16(t, -1)
        y = []
        for k2 in range(N2):
            a = wr[w_rows, 128 * k2:128 * k2 + 128].astype(f32)
            b = wi[w_rows, 128 * k2:128 * k2 + 128].astype(f32)
            (sr, xr), (si, xi) = x[k2]
            y.append((_ssub((sr, xr * a), (si, xi * b)), _sadd((sr, xr * b), (si, xi * a))))
        u = _fft16(y, 1)
        return [(_val(ur), _val(ui), _val(_sneg(ui))) for ur, ui in u]

    def spectral(g):
        for k in range(8):
            rows = pl.ds(pl.multiple_of(64 * g + 8 * k, 8), 8)
            for n2, (ur, ui, nui) in enumerate(spectral_unit(rows, rows)):
                rp[n2, rows, :] = jnp.concatenate([ur, nui], axis=1).astype(bf16)
                rq[n2, rows, :] = jnp.concatenate([ui, ur], axis=1).astype(bf16)
        for n2, (ur, ui, nui) in enumerate(spectral_unit(pl.ds(256, 8), pl.ds(256, 1))):
            rn[n2] = jnp.concatenate([ur, nui], axis=1)

    x_loop(1, lambda g: None, spectral)

    row16 = lax.broadcasted_iota(jnp.int32, (16, 2 * N1), 0)
    for j in range(8):
        zz = []
        for n2 in (2 * j, 2 * j + 1):
            nyq = rn[n2]
            q0 = jnp.where(row16 == 0, jnp.concatenate([nyq, nyq], axis=0),
                           rq[n2, 0:16, :].astype(f32)).astype(bf16)
            r = jnp.concatenate([rp[n2], q0, rq[n2, 16:256, :]], axis=0)
            zz.append(lax.dot_general(pltpu.bitcast(mf[n2], bf16), r, NT, preferred_element_type=f32))
        z = pltpu.pack_elementwise(zz, packed_dtype=bf16)
        z = pltpu.bitcast(z, u32) if z.dtype != u32 else z
        for t in range(4):
            z32[t, pl.ds(j, N1, stride=8), :] = z[:, 128 * t:128 * t + 128]

    cp_wo.wait()

    def copy_wo(g):
        r0 = pl.multiple_of(1024 * g, 1024)
        r1 = pl.multiple_of(512 * g, 512)
        wo32[pl.ds(r1, 512), :] = pltpu.bitcast(wo[pl.ds(r0, 1024), :], u32)

    x_loop(2, lambda g: None, copy_wo)

    cp_xb.wait()
    cp_fi.wait()
    cp_m0.wait()

    r = lax.broadcasted_iota(jnp.int32, (R2, R2), 0)
    c = lax.broadcasted_iota(jnp.int32, (R2, R2), 1)

    def head_pos(i):
        head = jnp.where(i < 32, 0, jnp.where(i < 64, 1, jnp.where(i < 72, 0, 1)))
        pos = jnp.where(i < 32, i, jnp.where(i < 72, i - 32, i - 40))
        return head, pos

    rh, rpos = head_pos(r)
    ch, cpos = head_pos(c)
    same = (rh - ch) == 0
    ok = jnp.logical_and(same, jnp.logical_or(rpos < MEM, rpos >= cpos))
    fill = jnp.where(same, jnp.float32(-1e9 / SCALE), jnp.float32(-jnp.inf))

    lag_qk, lag_pv = 1, 3

    def step(s, mem, mk_olhs):
        lhs = jnp.concatenate([mem, xb[s, 0:KEEP, :].astype(f32)], axis=0).astype(bf16)
        qkv = [None] * NP
        pr = [None] * NP
        oh = [None] * H
        ox = [None] * H
        acc = [None] * 4

        def do_qkv(hp):
            res = []
            for m in range(3):
                ys = [jnp.dot(lhs, pltpu.bitcast(wsl[H * m + 2 * hp + hh], bf16),
                              preferred_element_type=f32).astype(bf16) for hh in range(2)]
                res.append(jnp.concatenate(ys + [xq[NP * m + hp, s]], axis=0))
            qkv[hp] = res

        def do_qk(hp):
            sc = lax.dot_general(qkv[hp][0], qkv[hp][1], NT, preferred_element_type=f32)
            sc = jnp.where(ok, sc, fill)
            mx = jnp.max(sc, axis=-1, keepdims=True)
            e = jnp.exp2((sc - mx) * (SCALE * LOG2E))
            l = jnp.sum(e, axis=-1, keepdims=True)
            rl = pl.reciprocal(l, approx=True)
            rl = rl * (2.0 - l * rl)
            pr[hp] = (e.astype(bf16), rl)

        def do_pv(hp):
            o2 = jnp.dot(pr[hp][0], qkv[hp][2], preferred_element_type=f32) * pr[hp][1]
            oh[2 * hp], oh[2 * hp + 1] = o2[0:32], o2[32:64]
            ox[2 * hp], ox[2 * hp + 1] = o2[64:72], o2[72:80]

        def do_o(p0, p1):
            ol = jnp.concatenate([mk_olhs(h, oh[h], ox[h]) for h in range(2 * p0, 2 * p1)],
                                 axis=1).astype(bf16)
            for n in range(4):
                w = pltpu.bitcast(wo32[p0 * 128:p1 * 128, 128 * n:128 * n + 128], bf16)
                y = jnp.dot(ol, w, preferred_element_type=f32)
                acc[n] = y if acc[n] is None else acc[n] + y

        for hp in range(NP):
            do_qkv(hp)
            if hp - lag_qk >= 0:
                do_qk(hp - lag_qk)
            if hp - lag_pv >= 0:
                do_pv(hp - lag_pv)
        nqk, npv = NP - lag_qk, NP - lag_pv
        for (p0, p1) in [(0, 2), (2, 6), (6, 10), (10, 12), (12, 14), (14, 15), (15, 16)]:
            while npv < p1:
                while nqk <= npv:
                    do_qk(nqk)
                    nqk += 1
                do_pv(npv)
                npv += 1
            do_o(p0, p1)
            if nqk < NP:
                do_qk(nqk)
                nqk += 1
            if npv < NP and npv < nqk:
                do_pv(npv)
                npv += 1
        zr = pl.ds(pl.multiple_of(16 * s, 16), 16)
        zl = jnp.concatenate([pltpu.bitcast(z32[t, zr, :], bf16) for t in range(4)], axis=1)
        ya = jnp.dot(zl, pltpu.bitcast(fi[...], bf16), preferred_element_type=f32)
        stage[s, :, 0:D] = ya.astype(bf16)
        return jnp.concatenate(acc, axis=1), ox

    def body(i, mem):
        sa, sb = 2 * i, 2 * i + 1
        ya, oxa = step(sa, mem, lambda h, o, x: o)
        stage[sa, 0:KEEP, D:2 * D] = ya[MEM:].astype(bf16)
        mem_b = ya[0:MEM].astype(bf16).astype(f32)
        yb, _ = step(sb, mem_b, lambda h, o, x: jnp.concatenate([o, oxa[h], x], axis=0))
        stage[sa, KEEP:SEG, D:2 * D] = yb[32:40].astype(bf16)
        stage[sb, :, D:2 * D] = jnp.concatenate([yb[MEM:32], yb[40:48]], axis=0).astype(bf16)
        pltpu.make_async_copy(stage.at[pl.ds(sa, 2)], out_hbm.at[pl.ds(sa, 2)], sems.at[_OUT]).start()
        return yb[0:MEM].astype(bf16).astype(f32)

    lax.fori_loop(0, NSEG // 2, body, m0[...].astype(f32))
    pltpu.make_async_copy(stage, out_hbm, sems.at[_OUT]).wait()


@jax.jit
def pallas_concat_heads__spectral_gfnet__memory_aug_recurrent_mem_tr__prompt_kernel(
    A_x: jax.Array,
    A_w_r: jax.Array,
    A_w_i: jax.Array,
    B_x: jax.Array,
    B_mem0: jax.Array,
    B_Wq: jax.Array,
    B_Wk: jax.Array,
    B_Wv: jax.Array,
    B_Wo: jax.Array,
    B_seg_len: jax.Array,
):
    del B_seg_len
    assert A_x.shape == (1, S, D) and B_x.shape == (1, S, D) and B_mem0.shape == (1, MEM, D)
    assert B_Wq.shape == (D, H, DH) and B_Wo.shape == (H, DH, D)
    fd, fi, mf = _dft_tables()
    vm = pltpu.VMEM
    scratch = [
        vm((NSEG, XT, D), bf16),
        vm((NSEG * XT // 2, D), u32),
        vm((4, S, 128), bf16),
        vm((S // 2, 128), u32),
        vm((N2, 4, N1, 128), bf16),
        vm((12, D, 8, DH), bf16),
        vm((4 * D, DH), u32),
        vm((3 * H, D // 2, DH), u32),
        vm((3 * NP, NSEG, 2 * XT, DH), bf16),
        vm((D // 2, D), u32),
        vm((D // 2, D), u32),
        vm((N2, N1 // 2, 2 * N1), u32),
        vm((D // 2 + 1, S), bf16),
        vm((D // 2 + 1, S), bf16),
        vm((N2, 2, 264, N1), f32),
        vm((N2, 256, 2 * N1), bf16),
        vm((N2, 256, 2 * N1), bf16),
        vm((N2, 8, 2 * N1), f32),
        vm((4, S // 2, 128), u32),
        vm((H * DH, D), bf16),
        vm((H * DH // 2, D), u32),
        vm((NSEG, SEG, D), bf16),
        vm((MEM, D), bf16),
        vm((NSEG, SEG, 2 * D), bf16),
        pltpu.SemaphoreType.DMA((_NSEM,)),
    ]
    out = pl.pallas_call(
        _kernel,
        out_shape=jax.ShapeDtypeStruct((NSEG, SEG, 2 * D), bf16),
        in_specs=[pl.BlockSpec(memory_space=pl.ANY)] * 12,
        out_specs=pl.BlockSpec(memory_space=pl.ANY),
        scratch_shapes=scratch,
        compiler_params=pltpu.CompilerParams(vmem_limit_bytes=110 * 1024 * 1024),
    )(A_x.reshape(S, D), A_w_r.T, A_w_i.T, B_x.reshape(NSEG, SEG, D), B_mem0.reshape(MEM, D),
      B_Wq, B_Wk, B_Wv, B_Wo.reshape(H * DH, D), fd, fi, mf)
    return out.reshape(1, S, 2 * D)
```

```python
import math
import contextlib

import numpy as np
import jax
import jax.numpy as jnp
from jax import lax
import jax.experimental.pallas as pl
import jax.experimental.pallas.tpu as pltpu

S, D = 2048, 512
H, DH = 32, 128
MEM, SEG = 8, 32
NSEG = S // SEG
NP = H // 2
XT = 8
KEEP = SEG - XT
R2 = 2 * (MEM + SEG)
SCALE = DH ** -0.5
LOG2E = 1.4426950408889634
N1, N2 = 128, 16
SPB = 4

f32, bf16, u32 = jnp.float32, jnp.bfloat16, jnp.uint32
NT = (((1,), (1,)), ((), ()))


def _pack_rows(m):
    b = np.asarray(m, np.float32).astype(jnp.bfloat16).view(np.uint16).astype(np.uint32)
    return b[..., 0::2, :] | (b[..., 1::2, :] << 16)


def _dft_tables():
    k = np.arange(D // 2)[:, None]
    d = np.arange(D // 2)[None, :]
    ang = 2.0 * np.pi * ((k * d) % D) / D
    pm = np.cos(ang)
    qm = -np.sin(ang)
    qm[0] = (-1.0) ** np.arange(D // 2)

    def inter(parts):
        c = parts[0].shape[1]
        return np.stack([p.reshape(-1, 8, c) for p in parts], axis=1).reshape(-1, c)

    f0 = inter([pm[0::4, :128], qm[0::4, :128]])
    f2 = inter([pm[2::4, :128], qm[2::4, :128]])
    qo = qm[:, :128].copy()
    qo[:, 0] = qm[:, 128]
    fp = inter([pm[1::4, :128], pm[3::4, :128]])
    fq = inter([qo[1::4], qo[3::4]])
    fd = np.concatenate([np.concatenate([f0, f2, fp, fq], axis=1), np.zeros((16, 512))], axis=0)
    wgt = np.where(k == 0, 1.0, 2.0) / (S * D)
    pw, qw = wgt * pm, wgt * qm
    ii = np.arange(64)
    i0 = np.zeros((128, 128))
    i2 = np.zeros((128, 128))
    i0[2 * ii], i0[2 * ii + 1] = pw[0::4, :128], qw[0::4, :128]
    i2[2 * ii + 1], i2[(2 * ii + 2) % 128] = pw[2::4, :128], qw[2::4, :128]
    fi = np.concatenate([i0, i2, pw[1::2, :128], (wgt * qo)[1::2]], axis=1)
    m = ii[:, None]
    gs = np.zeros((N2, 128, 256))
    for a in range(N2):
        for e in range(2):
            an = 2.0 * np.pi * (((N2 * m + a) * (2 * ii[None, :] + e)) % S) / S
            g = np.zeros((2, 64, 128))
            re_l, im_l = 2 * ii + e, (2 * ii + e + 1) % 128
            g[e][:, re_l], g[e][:, im_l] = np.cos(an), -np.sin(an)
            g[1 - e][:, re_l], g[1 - e][:, im_l] = np.sin(an), np.cos(an)
            gs[a, :, 128 * e:128 * e + 128] = g.reshape(128, 128)
    return _pack_rows(fd), _pack_rows(fi), _pack_rows(gs)


def _sadd(a, b):
    (sa, va), (sb, vb) = a, b
    if sa == sb:
        return (sa, va + vb)
    return (1, va - vb) if sa > 0 else (1, vb - va)


def _sneg(a):
    return (-a[0], a[1])


def _ssub(a, b):
    return _sadd(a, _sneg(b))


def _smul(a, c):
    return (a[0], a[1] * c) if c > 0 else (-a[0], a[1] * (-c))


def _cadd(a, b):
    return (_sadd(a[0], b[0]), _sadd(a[1], b[1]))


def _csub(a, b):
    return (_ssub(a[0], b[0]), _ssub(a[1], b[1]))


def _cmul_i(a, sgn):
    return (_sneg(a[1]), a[0]) if sgn > 0 else (a[1], _sneg(a[0]))


def _radix4(x, sgn):
    t0, t1 = _cadd(x[0], x[2]), _csub(x[0], x[2])
    t2, t3 = _cadd(x[1], x[3]), _cmul_i(_csub(x[1], x[3]), sgn)
    return [_cadd(t0, t2), _cadd(t1, t3), _csub(t0, t2), _csub(t1, t3)]


def _twiddle16(a, m, sgn):
    if m == 0:
        return a
    if m == 4:
        return _cmul_i(a, sgn)
    c, s = math.cos(2 * math.pi * m / 16), sgn * math.sin(2 * math.pi * m / 16)
    if m in (2, 6):
        if c * s > 0:
            return (_smul(_ssub(a[0], a[1]), c), _smul(_sadd(a[0], a[1]), c))
        return (_smul(_sadd(a[0], a[1]), c), _smul(_ssub(a[1], a[0]), c))
    return (_ssub(_smul(a[0], c), _smul(a[1], s)), _sadd(_smul(a[0], s), _smul(a[1], c)))


def _gate(x, t):
    if t is None:
        return x
    (sr, vr), (si, vi) = x
    return ((sr, vr + t), (si, vi + t))


def _fft16(x, sgn, g1=None, g2=None):
    g1 = g1 or [None] * 4
    g2 = g2 or [None] * 4
    a = [_radix4([_gate(x[n2], g1[n2])] + [x[4 * n1 + n2] for n1 in range(1, 4)], sgn) for n2 in range(4)]
    out = [None] * 16
    for k1 in range(4):
        y = _radix4([_gate(a[0][k1], g2[k1])]
                    + [_twiddle16(a[n2][k1], n2 * k1, sgn) for n2 in range(1, 4)], sgn)
        for k2 in range(4):
            out[k1 + 4 * k2] = y[k2]
    return out


def _val(a):
    return a[1] if a[0] > 0 else -a[1]


def _lo(u):
    return pltpu.bitcast(u << 16, f32)


def _hi(u):
    return pltpu.bitcast(u & jnp.uint32(0xFFFF0000), f32)


def _pack2(a, b):
    z = pltpu.pack_elementwise([a, b], packed_dtype=bf16)
    return z if z.dtype == u32 else pltpu.bitcast(z, u32)


def _bf(u):
    return pltpu.bitcast(u, bf16)


def _dot(a, b):
    return jnp.dot(a, b, preferred_element_type=f32)


def _dot_nt(a, b):
    return lax.dot_general(a, b, NT, preferred_element_type=f32)


_PROFILE = False


def _scope(name):
    return jax.named_scope(name) if _PROFILE else contextlib.nullcontext()


_NGRP = 9
_S_XB, _S_OUT = _NGRP, _NGRP + 1
_NSEM = _NGRP + 2
XVP = 6

_SCHED = ('k0-4 v0-4 q0-4 k4-8 v4-8 p0-4 q4-8 k8-12 v8-12 p4-8 q8-12 k12-16 v12-16 p8-12 q12-16 '
          'o0-4 o4-9 p12-16 a o9-12 o12-16').split()


def _kernel(xa_hbm, wr_hbm, wi_hbm, xb_hbm, m0_hbm, wq_hbm, wk_hbm, wv_hbm, wo_hbm,
            fd_hbm, fi_hbm, gs_hbm, out_hbm,
            xe, xe32, xa, xst, xg, wst, wca, wcb, wsl, xq, fd, fi, gs, wr, wi, tsc, rv, rn,
            z32, wo, wo32, xb, m0, stage, zq, psc, qsc, osc, sems):
    w_hbms = (wq_hbm, wk_hbm, wv_hbm)

    def dyn(start, size):
        return pl.ds(start, size) if isinstance(start, int) else pl.ds(pl.multiple_of(start, size), size)

    def cp_w(m, g, sem):
        return pltpu.make_async_copy(w_hbms[m].at[:, :, dyn(8 * g, 8), :], wst.at[4 * m + g], sems.at[sem])

    def cp(src, dst, sem):
        return pltpu.make_async_copy(src, dst, sems.at[sem])

    def cp_xa(c0, c1, sem):
        rows = pl.ds(128 * c0, 128 * (c1 - c0))
        return cp(xa_hbm.at[:, rows, :], xa.at[:, rows, :], sem)

    def cp_f(src, dst, part, sem):
        rows = pl.ds(0, 160) if part == 0 else pl.ds(160, D // 2 + 1 - 160)
        return cp(src.at[rows, :], dst.at[rows, :], sem)

    grp = [
        [cp_w(0, 0, 0)],
        [cp(xb_hbm.at[:, pl.ds(KEEP, XT), :], xe, 1)],
        [cp(fd_hbm.at[pl.ds(64, 8), pl.ds(0, 128)], zq, 2), cp_w(0, 1, 2), cp_xa(0, 2, 2)],
        [cp_w(0, 2, 3), cp_w(0, 3, 3)],
        [cp_xa(2, 8, 4), cp(fd_hbm.at[pl.ds(0, 64), :], fd, 4), cp(gs_hbm, gs, 4)],
        [cp_w(1, 0, 5), cp_f(wr_hbm, wr, 0, 5), cp_f(wi_hbm, wi, 0, 5), cp_w(1, 1, 5)],
        [cp_f(wr_hbm, wr, 1, 6), cp_f(wi_hbm, wi, 1, 6),
         cp_w(1, 2, 6), cp_w(1, 3, 6), cp_w(2, 0, 6), cp_w(2, 1, 6)],
        [cp_w(2, 2, 7), cp_w(2, 3, 7), cp(wo_hbm, wo, 7)],
        [cp(fi_hbm, fi, 8), cp(m0_hbm, m0, 8),
         cp(xb_hbm.at[pl.ds(0, SPB), pl.ds(0, KEEP), :], xb.at[pl.ds(0, SPB)], 8)],
    ]
    cp_xb = cp(xb_hbm.at[pl.ds(SPB, NSEG - SPB), pl.ds(0, KEEP), :], xb.at[pl.ds(SPB, NSEG - SPB)], _S_XB)
    for g_ in grp + [[cp_xb]]:
        for c_ in g_:
            c_.start()

    def wait(name, grp):
        with _scope(name):
            for c_ in grp:
                c_.wait()

    def tokens(stream, lo=0.0, hi=0.92):
        zero = zq[...]

        def tok(k, n, delay=0):
            y, r = stream[min(int((lo + (hi - lo) * k / n) * len(stream)) + delay, len(stream) - 1)]
            return pltpu.bitcast(y[r:r + 8, 0:128], u32) & zero
        return tok

    def rows_of(y):
        return [(y, r) for r in range(0, y.shape[0], 8)]

    RC = 8

    def relayout(i, tok=None):
        wc = wcb if isinstance(i, int) and i % 2 == 1 else wca
        for c in range(D // 2 // RC):
            m_lo, m_hi = jnp.uint32(0xFFFF), jnp.uint32(0xFFFF0000)
            if tok is not None:
                t = tok(c, D // 2 // RC)
                m_lo = jnp.concatenate([t | m_lo] * (RC // 2), axis=0)
                m_hi = jnp.concatenate([t | m_hi] * (RC // 2), axis=0)
            ev = pltpu.bitcast(wst[i, RC * c:RC * c + RC, 0].reshape(8 * RC, DH), u32)
            od = pltpu.bitcast(wst[i, RC * c:RC * c + RC, 1].reshape(8 * RC, DH), u32)
            wc[0, 4 * RC * c:4 * RC * (c + 1), :] = (ev & m_lo) | (od << 16)
            wc[1, 4 * RC * c:4 * RC * (c + 1), :] = (ev >> 16) | (od & m_hi)
            t2 = None if tok is None else tok(c, D // 2 // RC, 12)
            for j in range(4):
                for p in range(2):
                    v = wc[p, pl.ds(4 * RC * c + j, RC, stride=4), :]
                    wsl[8 * i + 2 * j + p, RC * c:RC * c + RC, :] = v if t2 is None else v | t2

    def x_heads(h0, h1, mc=NSEG * XT):
        stream = []
        lhs = _bf(xe32[...])
        for h in range(h0, h1):
            for r0 in range(0, NSEG * XT, mc):
                y = _dot(lhs[r0:r0 + mc], _bf(wsl[h]))
                xq[h, r0:r0 + mc, :] = y.astype(bf16)
                stream += rows_of(y)
        return stream

    def lane_mask(rows, fn):
        return fn(lax.broadcasted_iota(jnp.int32, (rows, 128), 1))

    def is_even(rows):
        return lane_mask(rows, lambda l: (l & 1) == 0)

    def mirror(v):
        return jnp.take_along_axis(v, lane_mask(v.shape[0], lambda l: (128 - l) & 127), axis=1)

    def gather_x(chunks, tok):
        n = 24 * len(chunks)
        first = lane_mask(8, lambda l: l == 0)
        for ci, c in enumerate(chunks):
            for hf in range(2):
                for q in range(4):
                    u = pltpu.bitcast(xa[hf, dyn(128 * c + 32 * q, 32), :], u32)
                    tk = tok(24 * ci + 4 * hf + q, n)
                    r0 = 128 * (ci % 2) + 64 * hf + 16 * q
                    for a in range(4):
                        xst[a, r0:r0 + 16, :] = u[:, 128 * a:128 * a + 128] | jnp.concatenate([tk, tk], axis=0)
            for j in range(8):
                for p, part in enumerate((_lo, _hi)):
                    tk = pltpu.bitcast(tok(24 * ci + 8 + 2 * j + p, n), f32)
                    xl, xh = [[part(xst[a, pl.ds(128 * (ci % 2) + 64 * hf + j, 8, stride=8), :])
                               for a in range(4)] for hf in range(2)]
                    xl[0], xl[1] = xl[0] + tk, xl[1] + tk
                    for hf in range(2):
                        x0, x1, x2, x3 = [(l + h if hf == 0 else l - h) for l, h in zip(xl, xh)]
                        s02, s13 = x0 + x2, x1 + x3
                        al, rb = x0 - x2, mirror(x1 - x3)
                        v = jnp.concatenate([s02 + s13, s02 - s13, al - jnp.where(first, 0.0, rb),
                                             jnp.where(first, 0.0, al) + rb], axis=1)
                        xg[2 * j + p, dyn(64 * hf + 8 * c, 8), :] = v.astype(bf16)

    def a1(a, z0):
        y = [_dot_nt(_bf(fd[:, 128 * t:128 * t + 128]), xg[z0 + a, :, 128 * t:128 * t + 128]) for t in range(4)]
        ye = _pack2(y[0], y[1]).reshape(8, 2, 8, 128)
        po, qo = [y_.reshape(8, 2, 8, 128) for y_ in y[2:4]]
        p = jnp.concatenate([ye[:, 0], _pack2(po[:, 0], po[:, 1])], axis=0).reshape(128, 128)
        q = jnp.concatenate([ye[:, 1], _pack2(qo[:, 0], qo[:, 1])], axis=0).reshape(128, 128)
        q = pltpu.roll(q, 64, axis=1)
        q0 = q[0:8]
        row = lax.broadcasted_iota(jnp.int32, (8, 128), 0)
        q = jnp.concatenate([jnp.where(row == 0, q0 & jnp.uint32(0xFFFF0000), q0), q[8:]], axis=0)
        lo, lo8 = lane_mask(128, lambda l: l < 64), lane_mask(8, lambda l: l < 64)
        nil = jnp.zeros((8, 128), u32)
        l0 = jnp.concatenate([jnp.where(lo, p, q), jnp.where(lo8, nil, q0)], axis=0)
        l1 = jnp.concatenate([jnp.where(lo, q, p), jnp.where(lo8, q0, nil)], axis=0)
        return _bf(l0), _bf(l1)

    def s_fwd(a, ls):
        o0 = _dot(ls[0], _bf(gs[a, :, 0:128]))[0:264]
        o1 = _dot(ls[1], _bf(gs[a, :, 128:256]))[0:264]
        ev = is_even(264)
        tsc[a, 0] = jnp.where(ev, o0, o1)
        tsc[a, 1] = jnp.where(ev, o1, o0)
        return rows_of(o1)

    def spectral_fwd(filler):
        z0 = zq[0, 0].astype(jnp.int32)
        ls = [a1(a, z0) for a in range(4)]
        for a in range(0, N2, 2):
            if a + 4 < N2:
                ls += [a1(a + 4, z0), a1(a + 5, z0)]
            if a == N2 - 2:
                filler()
            s_fwd(a, ls[a])
            s_fwd(a + 1, ls[a + 1])

    rel = [0, 1, 2, 3, 4, 7, 10, 13, 16, 17.5, 19, 20.5]

    def spectral_mid(units, tok):
        ev = is_even(8)
        zs = zq[0, 0].astype(jnp.int32)
        for ui_, u in enumerate(units):
            gates = [pltpu.bitcast(tok(22 * ui_ + r, 22 * len(units)), f32) for r in rel]
            pre = [pltpu.bitcast(tok(max(22 * ui_ + r - 4, 0), 22 * len(units)), f32) for r in rel[0:4]]
            if u == 32:
                r0 = 256
                filt = lambda w, k2: w[256:257, 128 * k2:128 * k2 + 128].astype(f32)
            else:
                v, p = divmod(u, 2)
                r0 = 128 * p + 8 * v
                filt = lambda w, k2: (_lo, _hi)[p](
                    pltpu.bitcast(w[16 * v:16 * v + 16, 128 * k2:128 * k2 + 128], u32))
            t = [((1, tsc[zs + a, 0, r0:r0 + 8, :]),
                  (1, pltpu.roll(tsc[zs + a, 1, r0:r0 + 8, :] + pre[a % 4], 127, axis=1))) for a in range(N2)]
            if u == 32:
                t = [_cmul_i(v, -1) for v in t]
            x = _fft16(t, -1, gates[0:4], gates[4:8])
            y = []
            for k2 in range(N2):
                fa, fb = filt(wr, k2), filt(wi, k2)
                (sr, xr), (si, xi) = x[k2]
                y.append((_ssub((sr, xr * fa), (si, xi * fb)), _sadd((sr, xr * fb), (si, xi * fa))))
            for a, (sur, sui) in enumerate(_fft16(y, 1, None, gates[8:12])):
                ur, us = _val(sur), pltpu.roll(_val(sui), 1, axis=1)
                v01 = jnp.concatenate([jnp.where(ev, ur, us), jnp.where(ev, us, ur)], axis=1)
                if u == 32:
                    rn[a] = v01
                else:
                    rv[a, r0:r0 + 8, :] = v01.astype(bf16)

    def spectral_inv():
        stream = []
        first = lane_mask(64, lambda l: l == 0)
        ev = is_even(64)
        z0 = zq[0, 0].astype(jnp.int32)

        def comb(zs):
            return [_pack2(zs[0][0] + zs[0][1], zs[1][0] + zs[1][1]),
                    _pack2(zs[0][0] - zs[0][1], zs[1][0] - zs[1][1])]

        for j in range(8):
            gre, gri = [], []
            for a in (2 * j, 2 * j + 1):
                g = gs[a]
                re = [g[0:32, 0:128], g[32:64, 128:256]]
                im = [g[32:64, 0:128], g[0:32, 128:256]]
                gre.append([_bf(v) for v in re])
                gri.append([_bf(jnp.stack([r_.reshape(4, 8, 128), i_.reshape(4, 8, 128)], axis=1).reshape(64, 128))
                            for r_, i_ in zip(re, im)])

            def tile(t):
                zs = [[_dot_nt(gri[c][e], rv[z0 + 2 * j + c, 128 * t:128 * t + 128, 128 * e:128 * e + 128])
                       for e in range(2)] for c in range(2)]
                stream.extend(rows_of(zs[1][1]))
                out = [z.reshape(4, 2, 16, 128) for z in comb(zs)]
                return [(z[:, 0].reshape(64, 128), z[:, 1].reshape(64, 128)) for z in out]

            if j < 7:
                odd = tile(1)
            nq = [jnp.concatenate([rn[z0 + 2 * j + c], jnp.zeros((120, 256), f32)], axis=0).astype(bf16)
                  for c in range(2)]
            nyq = comb([[_dot_nt(gre[c][e], nq[c][:, 128 * e:128 * e + 128]) for e in range(2)]
                        for c in range(2)])
            even = tile(0)
            if j == 7:
                odd = tile(1)
            for be in range(2):
                zr, zi = even[be]
                sh = pltpu.roll(jnp.where(first, nyq[be], zi), 1, axis=1)
                tiles = [jnp.where(ev, zr, sh), jnp.where(ev, sh, zr), odd[be][0], odd[be][1]]
                for t in range(4):
                    z32[t, pl.ds(512 * be + j, 64, stride=8), :] = tiles[t]
        return stream

    def copy_wo(tok):
        for q in range(128):
            tk = tok(q, 128)
            tk = jnp.concatenate([jnp.concatenate([tk] * 4, axis=1)] * 2, axis=0)
            wo32[16 * q:16 * q + 16, :] = pltpu.bitcast(wo[32 * q:32 * q + 32, :], u32) | tk

    def xv_part(b, h0, h1):
        lhs = _bf(xe32[dyn(16 * b, 16), :])
        stream = []
        for h in range(h0, h1):
            y = _dot(lhs, _bf(wsl[2 * H + h]))
            xq[2 * H + h, dyn(32 * b, 32), :] = y.astype(bf16)
            stream += rows_of(y)
        return stream

    wait('w0', grp[0])
    with _scope('b0'):
        relayout(0)
    wait('w1', grp[1])
    with _scope('b1'):
        xe32[...] = pltpu.bitcast(xe[...].reshape(NSEG * XT, D), u32)
        x_heads(0, 6)

    wait('w2', grp[2])
    with _scope('b2'):
        relayout(1, tokens(x_heads(6, 8), hi=0.65))
        gather_x([0, 1], tokens(x_heads(8, 14), hi=0.85))

    wait('w3', grp[3])
    with _scope('b3'):
        relayout(2, tokens(x_heads(14, 16), hi=0.65))
        relayout(3, tokens(x_heads(16, 24), hi=0.9))

    wait('w4', grp[4])
    with _scope('b4'):
        gather_x(list(range(2, 8)), tokens(x_heads(24, 29), hi=0.9))
        spectral_fwd(lambda: x_heads(29, 30))

    wait('w5', grp[5])
    with _scope('b5'):
        relayout(4, tokens(x_heads(30, 32), hi=0.65))
        st = x_heads(32, 40)
        relayout(5, tokens(st, hi=0.9))
        spectral_mid(list(range(0, 10)), tokens(st, hi=1.0))
        spectral_mid(list(range(10, 18)), tokens(x_heads(40, 46), hi=0.9))

    wait('w6', grp[6])
    with _scope('b6'):
        relayout(6, tokens(x_heads(46, 48), hi=0.65))
        st = x_heads(48, 56)
        relayout(7, tokens(st, hi=0.45))
        relayout(8, tokens(st, lo=0.45, hi=0.9))
        spectral_mid(list(range(18, 24)), tokens(st, hi=1.0))
        st = x_heads(56, 62)
        relayout(9, tokens(st, hi=0.9))
        spectral_mid(list(range(24, 33)), tokens(st + x_heads(64, 64 + XVP // 2), hi=0.9))
        spectral_inv()

    wait('w7', grp[7])
    with _scope('b7'):
        st = x_heads(62, 64) + x_heads(64 + XVP // 2, 64 + XVP) + xv_part(0, XVP, 16)
        relayout(10, tokens(st, hi=0.4))
        relayout(11, tokens(st, lo=0.4, hi=0.8))
        copy_wo(tokens(st + xv_part(0, 16, H), hi=0.92))
    wait('w8', grp[8])

    r = lax.broadcasted_iota(jnp.int32, (R2, 128), 0)
    c = lax.broadcasted_iota(jnp.int32, (R2, 128), 1)

    def head_pos(i):
        head = jnp.where(i < 32, 0, jnp.where(i < 64, 1, jnp.where(i < 72, 0, jnp.where(i < R2, 1, 2))))
        pos = jnp.where(i < 32, i, jnp.where(i < 72, i - 32, i - 40))
        return head, pos

    rh, rpos = head_pos(r)
    ch, cpos = head_pos(c)
    same = (rh - ch) == 0
    ok = jnp.logical_and(same, jnp.logical_or(rpos < MEM, rpos >= cpos))
    fill = jnp.where(same, jnp.float32(-1e9 / SCALE), jnp.float32(-jnp.inf))

    def step(s, mem, second, filler):
        mo = 48 if second else 32
        lhs = jnp.concatenate([mem, xb[s].astype(f32)], axis=0).astype(bf16)
        xrows = dyn(XT * s, XT)
        acc = [None] * 4

        def proj(m, hp):
            ys = [_dot(lhs, _bf(wsl[H * m + 2 * hp + hh])) for hh in range(2)]
            qsc[m, hp] = jnp.concatenate(ys, axis=0).astype(bf16)

        def oper(m, hp):
            xs = [xq[H * m + 2 * hp + hh, xrows, :] for hh in range(2)]
            if m > 0:
                xs.append(jnp.zeros((128 - R2, DH), bf16))
            return jnp.concatenate([qsc[m, hp]] + xs, axis=0)

        def do_qkp(hp):
            proj(0, hp)
            proj(1, hp)

        def do_v(hp):
            proj(2, hp)

        def do_qk(hp):
            sc = _dot_nt(oper(0, hp), oper(1, hp))
            sc = jnp.where(ok, sc, fill)
            mx = jnp.max(sc, axis=-1, keepdims=True)
            e = jnp.exp2((sc - mx) * (SCALE * LOG2E))
            l = jnp.sum(e, axis=-1, keepdims=True)
            rl = pl.reciprocal(l, approx=True)
            rl = rl * (2.0 - l * rl)
            psc[hp] = (e * rl).astype(bf16)

        def do_pv(hp):
            o2 = _dot(psc[hp], oper(2, hp))
            r0 = 40 if second else 32
            for hh in range(2):
                osc[2 * hp + hh, 0:32, :] = o2[32 * hh:32 * hh + 32].astype(bf16)
                osc[2 * hp + hh, r0:r0 + 8, :] = o2[64 + 8 * hh:72 + 8 * hh].astype(bf16)

        def do_o(p0, p1):
            ol = jnp.concatenate([osc[h, 0:mo, :] for h in range(2 * p0, 2 * p1)], axis=1)
            for n in range(4):
                y = _dot(ol, _bf(wo32[p0 * 128:p1 * 128, 128 * n:128 * n + 128]))
                acc[n] = y if acc[n] is None else acc[n] + y

        def do_a3():
            zr = dyn(16 * s, 16)
            v0, v2, vc, vs = [_dot(_bf(z32[t, zr, :]), _bf(fi[:, 128 * t:128 * t + 128])) for t in range(4)]
            sp, sm = v0 + v2, v0 - v2
            first = lane_mask(SEG, lambda l: l == 0)
            al, be = vc + jnp.where(first, 0.0, vs), mirror(vs - jnp.where(first, 0.0, vc))
            stage[s, :, 0:D] = jnp.concatenate([sp + al, sm + be, sp - al, sm - be], axis=1).astype(bf16)

        for op in _SCHED:
            if op == 'a':
                do_a3()
                continue
            p0, p1 = [int(v) for v in op[1:].split('-')]
            if op[0] == 'o':
                do_o(p0, p1)
            else:
                for hp in range(p0, p1):
                    {'k': do_qkp, 'v': do_v, 'q': do_qk, 'p': do_pv}[op[0]](hp)
        filler()
        return jnp.concatenate(acc, axis=1)

    nb = NSEG // SPB

    hv = [XVP + (H - XVP) * k // SPB for k in range(SPB + 1)]

    def body(b, mem):
        @pl.when(b == 1)
        def _():
            cp_xb.wait()
        nxt = jnp.minimum(b + 1, nb - 1)
        for k in range(0, SPB, 2):
            sa, sb = SPB * b + k, SPB * b + k + 1
            ya = step(sa, mem, False, lambda: xv_part(nxt, hv[k], hv[k + 1]))
            stage[sa, 0:KEEP, D:2 * D] = ya[MEM:].astype(bf16)
            mem_b = ya[0:MEM].astype(bf16).astype(f32)
            yb = step(sb, mem_b, True, lambda: xv_part(nxt, hv[k + 1], hv[k + 2]))
            stage[sa, KEEP:SEG, D:2 * D] = yb[32:40].astype(bf16)
            stage[sb, :, D:2 * D] = jnp.concatenate([yb[MEM:32], yb[40:48]], axis=0).astype(bf16)
            mem = yb[0:MEM].astype(bf16).astype(f32)
            rows = pl.ds(sa, 2)
            cp(stage.at[rows], out_hbm.at[rows], _S_OUT).start()
        return mem

    with _scope('main'):
        lax.fori_loop(0, nb, body, m0[...].astype(f32))
    wait('w9', [cp(stage, out_hbm, _S_OUT)])


@jax.jit
def pallas_concat_heads__spectral_gfnet__memory_aug_recurrent_mem_tr__prompt_kernel(
    A_x: jax.Array,
    A_w_r: jax.Array,
    A_w_i: jax.Array,
    B_x: jax.Array,
    B_mem0: jax.Array,
    B_Wq: jax.Array,
    B_Wk: jax.Array,
    B_Wv: jax.Array,
    B_Wo: jax.Array,
    B_seg_len: jax.Array,
):
    del B_seg_len
    assert A_x.shape == (1, S, D) and B_x.shape == (1, S, D) and B_mem0.shape == (1, MEM, D)
    assert B_Wq.shape == (D, H, DH) and B_Wo.shape == (H, DH, D)
    fd, fi, gs = _dft_tables()
    vm = pltpu.VMEM
    scratch = [
        vm((NSEG, XT, D), bf16),
        vm((NSEG * XT // 2, D), u32),
        vm((2, S // 2, D), bf16),
        vm((4, 256, 128), u32),
        vm((N2, N1, D), bf16),
        vm((12, D // 2, 2, 8, DH), bf16),
        vm((2, 2 * D, DH), u32),
        vm((2, 2 * D, DH), u32),
        vm((3 * H, D // 2, DH), u32),
        vm((3 * H, NSEG * XT, DH), bf16),
        vm((64, 512), u32),
        vm((64, 512), u32),
        vm((N2, N1 // 2, 2 * N1), u32),
        vm((D // 2 + 1, S), bf16),
        vm((D // 2 + 1, S), bf16),
        vm((N2, 2, 264, N1), f32),
        vm((N2, 256, 2 * N1), bf16),
        vm((N2, 8, 2 * N1), f32),
        vm((4, S // 2, 128), u32),
        vm((H * DH, D), bf16),
        vm((H * DH // 2, D), u32),
        vm((NSEG, KEEP, D), bf16),
        vm((MEM, D), bf16),
        vm((NSEG, SEG, 2 * D), bf16),
        vm((8, 128), u32),
        vm((NP, R2, 128), bf16),
        vm((3, NP, 64, DH), bf16),
        vm((H, 48, DH), bf16),
        pltpu.SemaphoreType.DMA((_NSEM,)),
    ]
    w4 = lambda w: w.reshape(D // 2, 2, H, DH)
    out = pl.pallas_call(
        _kernel,
        out_shape=jax.ShapeDtypeStruct((NSEG, SEG, 2 * D), bf16),
        in_specs=[pl.BlockSpec(memory_space=pl.ANY)] * 12,
        out_specs=pl.BlockSpec(memory_space=pl.ANY),
        scratch_shapes=scratch,
        compiler_params=pltpu.CompilerParams(vmem_limit_bytes=110 * 1024 * 1024),
    )(A_x.reshape(2, S // 2, D), A_w_r.T, A_w_i.T, B_x.reshape(NSEG, SEG, D), B_mem0.reshape(MEM, D),
      w4(B_Wq), w4(B_Wk), w4(B_Wv), B_Wo.reshape(H * DH, D), fd, fi, gs)
    return out.reshape(1, S, 2 * D)
```

```python
import contextlib
import math

import numpy as np
import jax
import jax.numpy as jnp
from jax import lax
import jax.experimental.pallas as pl
import jax.experimental.pallas.tpu as pltpu

S, D = 2048, 512
H, DH = 32, 128
MEM, SEG = 8, 32
NSEG = S // SEG
NP = H // 2
XT = 8
KEEP = SEG - XT
R2 = 2 * (MEM + SEG)
SCALE = DH ** -0.5
LOG2E = 1.4426950408889634
NC = 16
SPB = 4
XVP = 6

f32, bf16, u32 = jnp.float32, jnp.bfloat16, jnp.uint32
NT = (((1,), (1,)), ((), ()))


def _pack_rows(m):
    b = np.asarray(m, np.float32).astype(jnp.bfloat16).view(np.uint16).astype(np.uint32)
    return b[0::2, :] | (b[1::2, :] << 16)


def _dft_tables():
    k = np.arange(D // 2)[:, None]
    d = np.arange(D // 2)[None, :]
    ang = 2.0 * np.pi * ((k * d) % D) / D
    pm = np.cos(ang)
    qm = -np.sin(ang)
    qm[0] = (-1.0) ** np.arange(D // 2)
    qo = qm[:, :128].copy()
    qo[:, 0] = qm[:, 128]

    def inter(parts):
        c = parts[0].shape[1]
        return np.stack([p.reshape(-1, 8, c) for p in parts], axis=1).reshape(-1, c)

    f0 = inter([pm[0::4, :128], qm[0::4, :128]])
    f2 = inter([pm[2::4, :128], qm[2::4, :128]])
    fp = inter([pm[1::4, :128], pm[3::4, :128]])
    fq = inter([qo[1::4], qo[3::4]])
    fd = np.concatenate([np.concatenate([f0, f2, fp, fq], axis=1), np.zeros((16, 512))], axis=0)
    wgt = np.where(k == 0, 1.0, 2.0) / (S * D)
    pw, qw = wgt * pm, wgt * qm
    ii = np.arange(64)
    i0 = np.zeros((128, 128))
    i2 = np.zeros((128, 128))
    i0[2 * ii], i0[2 * ii + 1] = pw[0::4, :128], qw[0::4, :128]
    i2[2 * ii + 1], i2[(2 * ii + 2) % 128] = pw[2::4, :128], qw[2::4, :128]
    fi = np.concatenate([i0, i2, pw[1::2, :128], (wgt * qo)[1::2]], axis=1)
    k1 = np.arange(128)[None, :]
    mo = np.concatenate([ii[0::2], ii[1::2]])[:, None]
    ae = 2.0 * np.pi * ((NC * mo * k1) % S) / S
    at = 2.0 * np.pi * (np.arange(NC)[:, None] * k1) / S
    sd = np.concatenate([np.cos(ae), np.sin(ae), np.cos(at), np.sin(at)], axis=0).astype(np.float32)
    return _pack_rows(fd), _pack_rows(fi), sd


def _sadd(a, b):
    (sa, va), (sb, vb) = a, b
    if sa == sb:
        return (sa, va + vb)
    return (1, va - vb) if sa > 0 else (1, vb - va)


def _sneg(a):
    return (-a[0], a[1])


def _ssub(a, b):
    return _sadd(a, _sneg(b))


def _smul(a, c):
    return (a[0], a[1] * c) if c > 0 else (-a[0], a[1] * (-c))


def _cadd(a, b):
    return (_sadd(a[0], b[0]), _sadd(a[1], b[1]))


def _csub(a, b):
    return (_ssub(a[0], b[0]), _ssub(a[1], b[1]))


def _cmul_i(a, sgn):
    return (_sneg(a[1]), a[0]) if sgn > 0 else (a[1], _sneg(a[0]))


def _radix4(x, sgn):
    t0, t1 = _cadd(x[0], x[2]), _csub(x[0], x[2])
    t2, t3 = _cadd(x[1], x[3]), _cmul_i(_csub(x[1], x[3]), sgn)
    return [_cadd(t0, t2), _cadd(t1, t3), _csub(t0, t2), _csub(t1, t3)]


def _twiddle16(a, m, sgn):
    if m == 0:
        return a
    if m == 4:
        return _cmul_i(a, sgn)
    c, s = math.cos(2 * math.pi * m / 16), sgn * math.sin(2 * math.pi * m / 16)
    if m in (2, 6):
        if c * s > 0:
            return (_smul(_ssub(a[0], a[1]), c), _smul(_sadd(a[0], a[1]), c))
        return (_smul(_sadd(a[0], a[1]), c), _smul(_ssub(a[1], a[0]), c))
    return (_ssub(_smul(a[0], c), _smul(a[1], s)), _sadd(_smul(a[0], s), _smul(a[1], c)))


def _gate(x, t):
    if t is None:
        return x
    (sr, vr), (si, vi) = x
    return ((sr, vr + t), (si, vi + t))


def _fft16(x, sgn, g1=None, g2=None):
    g1 = g1 or [None] * 4
    g2 = g2 or [None] * 4
    a = [_radix4([_gate(x[n2], g1[n2])] + [x[4 * n1 + n2] for n1 in range(1, 4)], sgn) for n2 in range(4)]
    out = [None] * 16
    for k1 in range(4):
        y = _radix4([_gate(a[0][k1], g2[k1])]
                    + [_twiddle16(a[n2][k1], n2 * k1, sgn) for n2 in range(1, 4)], sgn)
        for k2 in range(4):
            out[k1 + 4 * k2] = y[k2]
    return out


def _val(a):
    return a[1] if a[0] > 0 else -a[1]


def _lo(u):
    return pltpu.bitcast(u << 16, f32)


def _hi(u):
    return pltpu.bitcast(u & jnp.uint32(0xFFFF0000), f32)


def _pack2(a, b):
    lo = pltpu.bitcast(a.astype(bf16).astype(f32), u32) >> 16
    return lo | pltpu.bitcast(b.astype(bf16).astype(f32), u32)


def _bf(u):
    return pltpu.bitcast(u, bf16)


def _dot(a, b):
    return jnp.dot(a, b, preferred_element_type=f32)


def _dot_nt(a, b):
    return lax.dot_general(a, b, NT, preferred_element_type=f32)


def _lane(rows):
    return lax.broadcasted_iota(jnp.int32, (rows, 128), 1)


def _mirror(v):
    return jnp.take_along_axis(v, (128 - _lane(v.shape[0])) & 127, axis=1)


def _rep(t, n):
    k = t.shape[0] // 8
    return jnp.broadcast_to(t.reshape(k, 1, 8, 128), (k, n, 8, 128)).reshape(k * n * 8, 128)


_PROFILE = False


def _scope(name):
    return jax.named_scope(name) if _PROFILE else contextlib.nullcontext()


_NGRP = 9
_S_OUT = _NGRP

_SCHED = ('k0-4 v0-4 q0-4 k4-8 v4-8 p0-4 q4-8 k8-12 v8-12 p4-8 q8-12 k12-16 v12-16 p8-12 q12-16 '
          'o0-4 o4-9 p12-16 a o9-12 o12-16').split()


def _kernel(xa_hbm, wr_hbm, wi_hbm, xb_hbm, m0_hbm, wq_hbm, wk_hbm, wv_hbm, wo_hbm,
            fd_hbm, fi_hbm, sd_hbm, out_hbm,
            xe, xe32, xa, xst, xg, wst, wca, wcb, wsl, xq, fd, fi, gs, wr, wi, tsc, rv, rn,
            z32, wo, wo32, xb, m0, stage, zq, psc, qsc, osc, ssc, sd, part, sems):
    w_hbms = (wq_hbm, wk_hbm, wv_hbm)

    def dyn(start, size):
        return pl.ds(start, size) if isinstance(start, int) else pl.ds(pl.multiple_of(start, size), size)

    def cp(src, dst, sem):
        return pltpu.make_async_copy(src, dst, sems.at[sem])

    def cp_w(m, g, sem):
        return cp(w_hbms[m].at[:, :, pl.ds(8 * g, 8), :], wst.at[4 * m + g], sem)

    def cp_xa(c0, c1, sem):
        rows = pl.ds(128 * c0, 128 * (c1 - c0))
        return cp(xa_hbm.at[:, rows, :], xa.at[:, rows, :], sem)

    def cp_f(src, dst, part, sem):
        rows = pl.ds(0, 160) if part == 0 else pl.ds(160, D // 2 + 1 - 160)
        return cp(src.at[rows, :], dst.at[rows, :], sem)

    def cp_half(k, sem):
        rows, cols = pl.ds(128 * k, 128), pl.ds(256 * k, 256)
        return [cp(wq_hbm.at[rows, :, pl.ds(0, 8), :], wst.at[0, rows], sem),
                cp(xb_hbm.at[:, pl.ds(KEEP, XT), cols], xe.at[:, :, cols], sem)]

    grp = [
        cp_half(0, 0),
        cp_half(1, 1) + [cp(fd_hbm.at[pl.ds(64, 8), pl.ds(0, 128)], zq, 1)],
        [cp_w(0, 1, 2)],
        [cp(sd_hbm, sd, 3), cp_w(0, 2, 3), cp_xa(0, 4, 3)],
        [cp_w(0, 3, 4), cp_xa(4, 8, 4), cp(fd_hbm.at[pl.ds(0, 64), :], fd, 4)],
        [cp_w(1, 0, 5), cp_f(wr_hbm, wr, 0, 5), cp_f(wi_hbm, wi, 0, 5), cp_w(1, 1, 5)],
        [cp_f(wr_hbm, wr, 1, 6), cp_f(wi_hbm, wi, 1, 6),
         cp_w(1, 2, 6), cp_w(1, 3, 6), cp_w(2, 0, 6), cp_w(2, 1, 6)],
        [cp_w(2, 2, 7), cp_w(2, 3, 7), cp(wo_hbm, wo, 7)],
        [cp(fi_hbm, fi, 8), cp(m0_hbm, m0, 8), cp(xb_hbm.at[:, pl.ds(0, KEEP), :], xb, 8)],
    ]
    for g_ in grp:
        for c_ in g_:
            c_.start()

    def wait(name, copies):
        with _scope(name):
            for c_ in copies:
                c_.wait()

    def tokens(stream):
        ys = jnp.concatenate(stream, axis=0)
        n = ys.shape[0] // 8

        def tok(start, count, step):
            assert start + (count - 1) * step < n, (start, count, step, n)
            first = min(start, n - count * step)
            y = ys[8 * first:8 * (first + count * step)].reshape(count, step, 8, 128)[:, start - first]
            return (pltpu.bitcast(y, u32) & zq[...][None]).reshape(count * 8, 128)
        return tok

    def opaque():
        z0 = zq[0, 0].astype(jnp.int32)
        idx = [jnp.clip(z0 + a, 0, NC - 1) for a in range(NC)]
        return lambda a: idx[a]

    def relayout(i, tok=None, start=0, step=1, r0=0, r1=D // 2):
        wc = (wca, wcb)[i % 2]
        n = r1 - r0
        m_lo, m_hi = jnp.uint32(0xFFFF), jnp.uint32(0xFFFF0000)
        if tok is not None:
            t1 = tok(start, n // 8, step)
            m_lo, m_hi = _rep(t1 | m_lo, 4), _rep(t1 | m_hi, 4)
            t2 = tok(start + 12, n // 8, step)
        ev = pltpu.bitcast(wst[i, r0:r1, 0].reshape(8 * n, DH), u32)
        od = pltpu.bitcast(wst[i, r0:r1, 1].reshape(8 * n, DH), u32)
        wc[0, 4 * r0:4 * r1, :] = (ev & m_lo) | (od << 16)
        wc[1, 4 * r0:4 * r1, :] = (ev >> 16) | (od & m_hi)
        for j in range(4):
            for p in range(2):
                v = wc[p, pl.ds(4 * r0 + j, n, stride=4), :]
                wsl[8 * i + 2 * j + p, r0:r1, :] = v if tok is None else v | t2

    def x_half(k, h0, h1):
        lhs = _bf(xe32[:, 256 * k:256 * k + 256])
        ys = []
        for h in range(h0, h1):
            ys.append(_dot(lhs, _bf(wsl[h, 128 * k:128 * k + 128, :])))
            if k == 0:
                part[h] = ys[-1]
            else:
                xq[h] = (ys[-1] + part[h]).astype(bf16)
        return ys

    def pack_xe(k, tok=None):
        v = pltpu.bitcast(xe[:, :, 256 * k:256 * k + 256].reshape(NSEG * XT, 256), u32)
        if tok is not None:
            v = v | jnp.concatenate([tok(0, 32, 1)] * 2, axis=1)
        xe32[:, 256 * k:256 * k + 256] = v

    def x_heads(h0, h1):
        lhs = _bf(xe32[...])
        ys = []
        for h in range(h0, h1):
            ys.append(_dot(lhs, _bf(wsl[h])))
            xq[h] = ys[-1].astype(bf16)
        return ys

    def gather_x(c0, c1, tok, per):
        nc = c1 - c0
        first = _lane(8 * nc) == 0
        for hf in range(2):
            tk = jnp.stack([tok((4 * hf + q) * per // 24, nc, per).reshape(nc, 8, 128) for q in range(4)], axis=1)
            tk = _rep(tk.reshape(32 * nc, 128), 2)
            u = pltpu.bitcast(xa[hf, 128 * c0:128 * c1, :], u32)
            for a in range(4):
                xst[a, hf, 64 * c0:64 * c1, :] = u[:, 128 * a:128 * a + 128] | tk
        for j in range(8):
            for p, part in enumerate((_lo, _hi)):
                tk = pltpu.bitcast(tok((8 + 2 * j + p) * per // 24, nc, per), f32)
                xl, xh = [[part(xst[a, hf, pl.ds(64 * c0 + j, 8 * nc, stride=8), :]) for a in range(4)]
                          for hf in range(2)]
                xl[0], xl[1] = xl[0] + tk, xl[1] + tk
                for hf in range(2):
                    x0, x1, x2, x3 = [(l + h if hf == 0 else l - h) for l, h in zip(xl, xh)]
                    s02, s13 = x0 + x2, x1 + x3
                    al, rb = x0 - x2, _mirror(x1 - x3)
                    v = jnp.concatenate([s02 + s13, s02 - s13, al - jnp.where(first, 0.0, rb),
                                         jnp.where(first, 0.0, al) + rb], axis=1)
                    xg[2 * j + p, 64 * hf + 8 * c0:64 * hf + 8 * c1, :] = v.astype(bf16)

    def build_gs(tok, step):
        tk = pltpu.bitcast(tok(0, 4 * NC, step), f32)
        ct, st = [jnp.concatenate([jnp.broadcast_to(sd[r0 + a:r0 + a + 1, :], (32, 128)) for a in range(NC)],
                                  axis=0) + tk for r0 in (128, 144)]
        ce, se = [[jnp.concatenate([sd[r0 + 32 * p:r0 + 32 * p + 32, :]] * NC, axis=0) for p in range(2)]
                  for r0 in (0, 64)]
        co = _pack2(*[ce[p] * ct - se[p] * st for p in range(2)])
        si = _pack2(*[se[p] * ct + ce[p] * st for p in range(2)])
        cr = pltpu.roll(co, 1, axis=1)
        ns = pltpu.roll(si, 1, axis=1) ^ jnp.uint32(0x80008000)
        ev = (_lane(32 * NC) & 1) == 0
        gs[:, 0:32, :] = jnp.concatenate(
            [jnp.where(ev, co, ns), jnp.where(ev, cr, si)], axis=1).reshape(NC, 32, 256)
        gs[:, 32:64, :] = jnp.concatenate(
            [jnp.where(ev, si, cr), jnp.where(ev, ns, co)], axis=1).reshape(NC, 32, 256)

    def d_fwd(a, at):
        y = [_dot_nt(_bf(fd[:, 128 * t:128 * t + 128]), xg[at(a), :, 128 * t:128 * t + 128]) for t in range(4)]
        ye = _pack2(y[0], y[1]).reshape(8, 2, 8, 128)
        po, qo = [y_.reshape(8, 2, 8, 128) for y_ in y[2:4]]
        p = jnp.concatenate([ye[:, 0], _pack2(po[:, 0], po[:, 1])], axis=0).reshape(128, 128)
        q = jnp.concatenate([ye[:, 1], _pack2(qo[:, 0], qo[:, 1])], axis=0).reshape(128, 128)
        q = pltpu.roll(q, 64, axis=1)
        q0 = q[0:8]
        row = lax.broadcasted_iota(jnp.int32, (8, 128), 0)
        q = jnp.concatenate([jnp.where(row == 0, q0 & jnp.uint32(0xFFFF0000), q0), q[8:]], axis=0)
        lo, lo8 = _lane(128) < 64, _lane(8) < 64
        nil = jnp.zeros((8, 128), u32)
        l0 = jnp.concatenate([jnp.where(lo, p, q), jnp.where(lo8, nil, q0)], axis=0)
        l1 = jnp.concatenate([jnp.where(lo, q, p), jnp.where(lo8, q0, nil)], axis=0)
        return _bf(l0), _bf(l1)

    def s_fwd(a, ls, at):
        o0 = _dot(ls[0], _bf(gs[at(a), :, 0:128]))[0:264]
        o1 = _dot(ls[1], _bf(gs[at(a), :, 128:256]))[0:264]
        ev = (_lane(264) & 1) == 0
        tsc[a, 0] = jnp.where(ev, o0, o1)
        tsc[a, 1] = jnp.where(ev, o1, o0)
        return o1

    def spectral_fwd(filler):
        at = opaque()
        ls = [d_fwd(a, at) for a in range(4)]
        stream = []
        for a in range(0, NC, 2):
            if a + 4 < NC:
                ls += [d_fwd(a + 4, at), d_fwd(a + 5, at)]
            if a == NC - 2:
                filler()
            s_fwd(a, ls[a], at)
            stream.append(s_fwd(a + 1, ls[a + 1], at))
        return stream

    rel = [0, 1, 2, 3, 4, 7, 10, 13, 16, 17.5, 19, 20.5]

    def spectral_mid(p, v0, v1, tok, start, per):
        nu = v1 - v0
        at = opaque()
        gate = lambda r: pltpu.bitcast(tok(start + int((r + 4) * per / 24), nu, per), f32)
        gates = [gate(r) for r in rel]
        pre = [gate(r - 4) for r in rel[0:4]]
        r0, r1 = 128 * p + 8 * v0, 128 * p + 8 * v1
        if p == 2:
            filt = lambda w, k2: w[256:257, 128 * k2:128 * k2 + 128].astype(f32)
        else:
            filt = lambda w, k2: (_lo, _hi)[p](pltpu.bitcast(w[16 * v0:16 * v1, 128 * k2:128 * k2 + 128], u32))
        t = [((1, tsc[at(a), 0, r0:r1, :]), (1, pltpu.roll(tsc[at(a), 1, r0:r1, :] + pre[a % 4], 127, axis=1)))
             for a in range(NC)]
        if p == 2:
            t = [_cmul_i(v, -1) for v in t]
        x = _fft16(t, -1, gates[0:4], gates[4:8])
        y = []
        for k2 in range(NC):
            fa, fb = filt(wr, k2), filt(wi, k2)
            (sr, xr), (si, xi) = x[k2]
            y.append((_ssub((sr, xr * fa), (si, xi * fb)), _sadd((sr, xr * fb), (si, xi * fa))))
        ev = (_lane(8 * nu) & 1) == 0
        u = _fft16(y, 1, None, gates[8:12])
        for k1 in range(4):
            ui = jnp.stack([_val(u[k1 + 4 * k2][1]).reshape(nu, 8, 128) for k2 in range(4)], axis=1)
            us4 = pltpu.roll(ui.reshape(32 * nu, 128), 1, axis=1).reshape(nu, 4, 8, 128)
            for k2 in range(4):
                ur, us = _val(u[k1 + 4 * k2][0]), us4[:, k2].reshape(8 * nu, 128)
                v01 = jnp.concatenate([jnp.where(ev, ur, us), jnp.where(ev, us, ur)], axis=1)
                if p == 2:
                    rn[k1 + 4 * k2] = v01
                else:
                    rv[k1 + 4 * k2, r0:r1, :] = v01.astype(bf16)

    def spectral_inv():
        first = _lane(64) == 0
        ev = (_lane(64) & 1) == 0
        at = opaque()

        def comb(zs):
            return [_pack2(zs[0][0] + zs[0][1], zs[1][0] + zs[1][1]),
                    _pack2(zs[0][0] - zs[0][1], zs[1][0] - zs[1][1])]

        for j in range(8):
            gre, gri = [], []
            for a in (2 * j, 2 * j + 1):
                g = gs[at(a)]
                re = [g[0:32, 0:128], g[32:64, 128:256]]
                im = [g[32:64, 0:128], g[0:32, 128:256]]
                gre.append([_bf(v) for v in re])
                gri.append([_bf(jnp.stack([r_.reshape(4, 8, 128), i_.reshape(4, 8, 128)], axis=1).reshape(64, 128))
                            for r_, i_ in zip(re, im)])

            def tile(t):
                zs = [[_dot_nt(gri[c][e], rv[at(2 * j + c), 128 * t:128 * t + 128, 128 * e:128 * e + 128])
                       for e in range(2)] for c in range(2)]
                out = [z.reshape(4, 2, 16, 128) for z in comb(zs)]
                return [(z[:, 0].reshape(64, 128), z[:, 1].reshape(64, 128)) for z in out]

            if j < 7:
                odd = tile(1)
            nq = [jnp.concatenate([rn[at(2 * j + c)], jnp.zeros((120, 256), f32)], axis=0).astype(bf16)
                  for c in range(2)]
            nyq = comb([[_dot_nt(gre[c][e], nq[c][:, 128 * e:128 * e + 128]) for e in range(2)]
                        for c in range(2)])
            even = tile(0)
            if j == 7:
                odd = tile(1)
            for be in range(2):
                zr, zi = even[be]
                sh = pltpu.roll(jnp.where(first, nyq[be], zi), 1, axis=1)
                tiles = [jnp.where(ev, zr, sh), jnp.where(ev, sh, zr), odd[be][0], odd[be][1]]
                for t in range(4):
                    z32[t, pl.ds(512 * be + j, 64, stride=8), :] = tiles[t]

    def copy_wo(tok, step):
        tk = _rep(tok(0, 128, step), 2)
        wo32[...] = pltpu.bitcast(wo[...], u32) | jnp.concatenate([tk] * 4, axis=1)

    def xv_part(b, h0, h1):
        lhs = _bf(xe32[dyn(16 * b, 16), :])
        ys = []
        for h in range(h0, h1):
            ys.append(_dot(lhs, _bf(wsl[2 * H + h])))
            xq[2 * H + h, dyn(32 * b, 32), :] = ys[-1].astype(bf16)
        return ys

    wait('w0', grp[0])
    with _scope('b0'):
        for c in range(4):
            relayout(0, r0=32 * c, r1=32 * c + 32)
        pack_xe(0)
        x_half(0, 0, 6)

    wait('w1', grp[1])
    with _scope('b1'):
        tok = tokens(x_half(0, 6, 8)[1:])
        relayout(0, tok, 0, 2, r0=128)
        pack_xe(1, tok)
        x_half(1, 0, 4)

    wait('w2', grp[2])
    with _scope('b2'):
        relayout(1, tokens(x_half(1, 4, 8)[1::2]), 0, 3)
        x_heads(8, 14)

    wait('w3', grp[3])
    with _scope('b3'):
        relayout(2, tokens(x_heads(14, 16)), 0, 3)
        tok = tokens(x_heads(16, 22))
        gather_x(0, 4, tok, 84)
        build_gs(tok, 5)

    wait('w4', grp[4])
    with _scope('b4'):
        relayout(3, tokens(x_heads(22, 24)), 0, 3)
        gather_x(4, 8, tokens(x_heads(24, 29)), 68)
        spectral_fwd(lambda: x_heads(29, 30))

    wait('w5', grp[5])
    with _scope('b5'):
        relayout(4, tokens(x_heads(30, 32)), 0, 3)
        tok = tokens(x_heads(32, 40))
        relayout(5, tok, 0, 14)
        spectral_mid(0, 0, 10, tok, 0, 50)
        spectral_mid(1, 0, 6, tokens(x_heads(40, 46)), 0, 54)

    wait('w6', grp[6])
    with _scope('b6'):
        relayout(6, tokens(x_heads(46, 48)), 0, 3)
        tok = tokens(x_heads(48, 56))
        relayout(7, tok, 0, 7)
        relayout(8, tok, 230, 7)
        spectral_mid(0, 10, 16, tok, 0, 72)
        spectral_mid(2, 0, 1, tok, 430, 72)
        tok = tokens(x_heads(56, 62) + x_heads(64, 64 + XVP // 2))
        relayout(9, tok, 0, 16)
        spectral_mid(1, 6, 16, tok, 0, 52)
        spectral_inv()

    wait('w7', grp[7])
    with _scope('b7'):
        st = x_heads(62, 64) + x_heads(64 + XVP // 2, 64 + XVP) + xv_part(0, XVP, 16)
        tok = tokens(st)
        relayout(10, tok, 0, 4)
        relayout(11, tok, 150, 4)
        copy_wo(tokens(st + xv_part(0, 16, H)), 3)
    wait('w8', grp[8])

    r = lax.broadcasted_iota(jnp.int32, (R2, 128), 0)
    c = lax.broadcasted_iota(jnp.int32, (R2, 128), 1)

    def head_pos(i):
        head = jnp.where(i < 32, 0, jnp.where(i < 64, 1, jnp.where(i < 72, 0, jnp.where(i < R2, 1, 2))))
        pos = jnp.where(i < 32, i, jnp.where(i < 72, i - 32, i - 40))
        return head, pos

    rh, rpos = head_pos(r)
    ch, cpos = head_pos(c)
    same = (rh - ch) == 0
    ok = jnp.logical_and(same, jnp.logical_or(rpos < MEM, rpos >= cpos))
    fill = jnp.where(same, jnp.float32(-1e9 / SCALE), jnp.float32(-jnp.inf))

    def step(s, mem, second, filler):
        mo = 48 if second else 32
        lhs = jnp.concatenate([mem, xb[s].astype(f32)], axis=0).astype(bf16)
        xrows = dyn(XT * s, XT)
        acc = [None] * 4
        stream = []

        def proj(m, hp):
            y = jnp.concatenate([_dot(lhs, _bf(wsl[H * m + 2 * hp + hh])) for hh in range(2)], axis=0)
            qsc[m, hp] = y.astype(bf16)
            stream.append(y)

        def oper(m, hp):
            xs = [xq[H * m + 2 * hp + hh, xrows, :] for hh in range(2)]
            if m > 0:
                xs.append(jnp.zeros((128 - R2, DH), bf16))
            return jnp.concatenate([qsc[m, hp]] + xs, axis=0)

        def do_qkp(hp):
            proj(0, hp)
            proj(1, hp)

        def do_v(hp):
            proj(2, hp)

        def do_qk(hp):
            ssc[hp] = jnp.where(ok, _dot_nt(oper(0, hp), oper(1, hp)), fill)
            stream.clear()

        def do_softmax(p0, p1):
            nt = 20 if p1 < NP else 5
            g = pltpu.bitcast(_rep(tokens(stream[0:3])(0, nt, 1), 40 // nt), f32)
            sc = ssc[p0:p1].reshape(4 * R2, 128) + g
            mx = jnp.max(sc, axis=-1, keepdims=True)
            e = jnp.exp2((sc - mx) * (SCALE * LOG2E))
            l = jnp.sum(e, axis=-1, keepdims=True)
            rl = pl.reciprocal(l, approx=True)
            rl = rl * (2.0 - l * rl)
            psc[p0:p1] = (e * rl).astype(bf16).reshape(4, R2, 128)

        def do_pv(hp):
            o2 = _dot(psc[hp], oper(2, hp))
            r0 = 40 if second else 32
            for hh in range(2):
                osc[2 * hp + hh, 0:32, :] = o2[32 * hh:32 * hh + 32].astype(bf16)
                osc[2 * hp + hh, r0:r0 + 8, :] = o2[64 + 8 * hh:72 + 8 * hh].astype(bf16)

        def do_o(p0, p1):
            ol = jnp.concatenate([osc[h, 0:mo, :] for h in range(2 * p0, 2 * p1)], axis=1)
            for n in range(4):
                y = _dot(ol, _bf(wo32[p0 * 128:p1 * 128, 128 * n:128 * n + 128]))
                acc[n] = y if acc[n] is None else acc[n] + y
                stream.append(y)

        def do_a3():
            zr = dyn(16 * s, 16)
            v0, v2, vc, vs = [_dot(_bf(z32[t, zr, :]), _bf(fi[:, 128 * t:128 * t + 128])) for t in range(4)]
            sp, sm = v0 + v2, v0 - v2
            first = _lane(SEG) == 0
            al, be = vc + jnp.where(first, 0.0, vs), _mirror(vs - jnp.where(first, 0.0, vc))
            stage[s, :, 0:D] = jnp.concatenate([sp + al, sm + be, sp - al, sm - be], axis=1).astype(bf16)

        for op in _SCHED:
            if op == 'a':
                do_a3()
                continue
            p0, p1 = [int(v) for v in op[1:].split('-')]
            if op[0] == 'p':
                do_softmax(p0, p1)
            if op[0] == 'o':
                do_o(p0, p1)
            else:
                for hp in range(p0, p1):
                    {'k': do_qkp, 'v': do_v, 'q': do_qk, 'p': do_pv}[op[0]](hp)
        filler()
        return jnp.concatenate(acc, axis=1)

    nb = NSEG // SPB
    hv = [XVP + (H - XVP) * k // SPB for k in range(SPB + 1)]

    def body(b, mem):
        nxt = jnp.minimum(b + 1, nb - 1)
        for k in range(0, SPB, 2):
            sa, sb = SPB * b + k, SPB * b + k + 1
            ya = step(sa, mem, False, lambda: xv_part(nxt, hv[k], hv[k + 1]))
            stage[sa, 0:KEEP, D:2 * D] = ya[MEM:].astype(bf16)
            mem_b = ya[0:MEM].astype(bf16).astype(f32)
            yb = step(sb, mem_b, True, lambda: xv_part(nxt, hv[k + 1], hv[k + 2]))
            stage[sa, KEEP:SEG, D:2 * D] = yb[32:40].astype(bf16)
            stage[sb, :, D:2 * D] = jnp.concatenate([yb[MEM:32], yb[40:48]], axis=0).astype(bf16)
            mem = yb[0:MEM].astype(bf16).astype(f32)
            rows = pl.ds(sa, 2)
            cp(stage.at[rows], out_hbm.at[rows], _S_OUT).start()
        return mem

    with _scope('main'):
        lax.fori_loop(0, nb, body, m0[...].astype(f32))
    wait('w9', [cp(stage, out_hbm, _S_OUT)])


@jax.jit
def pallas_concat_heads__spectral_gfnet__memory_aug_recurrent_mem_tr__prompt_kernel(
    A_x: jax.Array,
    A_w_r: jax.Array,
    A_w_i: jax.Array,
    B_x: jax.Array,
    B_mem0: jax.Array,
    B_Wq: jax.Array,
    B_Wk: jax.Array,
    B_Wv: jax.Array,
    B_Wo: jax.Array,
    B_seg_len: jax.Array,
):
    del B_seg_len
    assert A_x.shape == (1, S, D) and B_x.shape == (1, S, D) and B_mem0.shape == (1, MEM, D)
    assert B_Wq.shape == (D, H, DH) and B_Wo.shape == (H, DH, D)
    fd, fi, sd = _dft_tables()
    vm = pltpu.VMEM
    scratch = [
        vm((NSEG, XT, D), bf16),
        vm((NSEG * XT // 2, D), u32),
        vm((2, S // 2, D), bf16),
        vm((4, 2, S // 4, 128), u32),
        vm((NC, 128, D), bf16),
        vm((12, D // 2, 2, 8, DH), bf16),
        vm((2, 2 * D, DH), u32),
        vm((2, 2 * D, DH), u32),
        vm((3 * H, D // 2, DH), u32),
        vm((3 * H, NSEG * XT, DH), bf16),
        vm((64, 512), u32),
        vm((64, 512), u32),
        vm((NC, 64, 256), u32),
        vm((D // 2 + 1, S), bf16),
        vm((D // 2 + 1, S), bf16),
        vm((NC, 2, 264, 128), f32),
        vm((NC, 256, 256), bf16),
        vm((NC, 8, 256), f32),
        vm((4, S // 2, 128), u32),
        vm((H * DH, D), bf16),
        vm((H * DH // 2, D), u32),
        vm((NSEG, KEEP, D), bf16),
        vm((MEM, D), bf16),
        vm((NSEG, SEG, 2 * D), bf16),
        vm((8, 128), u32),
        vm((NP, R2, 128), bf16),
        vm((3, NP, 64, DH), bf16),
        vm((H, 48, DH), bf16),
        vm((NP, R2, 128), f32),
        vm((160, 128), f32),
        vm((8, NSEG * XT, DH), f32),
        pltpu.SemaphoreType.DMA((_NGRP + 1,)),
    ]
    w4 = lambda w: w.reshape(D // 2, 2, H, DH)
    out = pl.pallas_call(
        _kernel,
        out_shape=jax.ShapeDtypeStruct((NSEG, SEG, 2 * D), bf16),
        in_specs=[pl.BlockSpec(memory_space=pl.ANY)] * 12,
        out_specs=pl.BlockSpec(memory_space=pl.ANY),
        scratch_shapes=scratch,
        compiler_params=pltpu.CompilerParams(vmem_limit_bytes=110 * 1024 * 1024),
    )(A_x.reshape(2, S // 2, D), A_w_r.T, A_w_i.T, B_x.reshape(NSEG, SEG, D), B_mem0.reshape(MEM, D),
      w4(B_Wq), w4(B_Wk), w4(B_Wv), B_Wo.reshape(H * DH, D), fd, fi, sd)
    return out.reshape(1, S, 2 * D)
```

```python
import contextlib
import math

import numpy as np
import jax
import jax.numpy as jnp
from jax import lax
import jax.experimental.pallas as pl
import jax.experimental.pallas.tpu as pltpu

S, D = 2048, 512
H, DH = 32, 128
MEM, SEG = 8, 32
NSEG = S // SEG
NP = H // 2
XT = 8
KEEP = SEG - XT
R2 = 2 * (MEM + SEG)
SCALE = DH ** -0.5
LOG2E = 1.4426950408889634
NC = 16
SPB = 4
XVP = 6

f32, bf16, u32 = jnp.float32, jnp.bfloat16, jnp.uint32
NT = (((1,), (1,)), ((), ()))


def _pack_rows(m):
    b = np.asarray(m, np.float32).astype(jnp.bfloat16).view(np.uint16).astype(np.uint32)
    return b[0::2, :] | (b[1::2, :] << 16)


def _dft_tables():
    k = np.arange(D // 2)[:, None]
    d = np.arange(D // 2)[None, :]
    ang = 2.0 * np.pi * ((k * d) % D) / D
    pm = np.cos(ang)
    qm = -np.sin(ang)
    qm[0] = (-1.0) ** np.arange(D // 2)
    qo = qm[:, :128].copy()
    qo[:, 0] = qm[:, 128]

    def inter(parts):
        c = parts[0].shape[1]
        return np.stack([p.reshape(-1, 8, c) for p in parts], axis=1).reshape(-1, c)

    f0 = inter([pm[0::4, :128], qm[0::4, :128]])
    f2 = inter([pm[2::4, :128], qm[2::4, :128]])
    fp = inter([pm[1::4, :128], pm[3::4, :128]])
    fq = inter([qo[1::4], qo[3::4]])
    fd = np.concatenate([np.concatenate([f0, f2, fp, fq], axis=1), np.zeros((16, 512))], axis=0)
    wgt = np.where(k == 0, 1.0, 2.0) / (S * D)
    pw, qw = wgt * pm, wgt * qm
    ii = np.arange(64)
    i0 = np.zeros((128, 128))
    i2 = np.zeros((128, 128))
    i0[2 * ii], i0[2 * ii + 1] = pw[0::4, :128], qw[0::4, :128]
    i2[2 * ii + 1], i2[(2 * ii + 2) % 128] = pw[2::4, :128], qw[2::4, :128]
    fi = np.concatenate([i0, i2, pw[1::2, :128], (wgt * qo)[1::2]], axis=1)
    k1 = np.arange(128)[None, :]
    mo = np.concatenate([ii[0::2], ii[1::2]])[:, None]
    ae = 2.0 * np.pi * ((NC * mo * k1) % S) / S
    at = 2.0 * np.pi * (np.arange(NC)[:, None] * k1) / S
    sd = np.concatenate([np.cos(ae), np.sin(ae), np.cos(at), np.sin(at)], axis=0).astype(np.float32)
    return _pack_rows(fd), _pack_rows(fi), sd


def _sadd(a, b):
    (sa, va), (sb, vb) = a, b
    if sa == sb:
        return (sa, va + vb)
    return (1, va - vb) if sa > 0 else (1, vb - va)


def _sneg(a):
    return (-a[0], a[1])


def _ssub(a, b):
    return _sadd(a, _sneg(b))


def _smul(a, c):
    return (a[0], a[1] * c) if c > 0 else (-a[0], a[1] * (-c))


def _cadd(a, b):
    return (_sadd(a[0], b[0]), _sadd(a[1], b[1]))


def _csub(a, b):
    return (_ssub(a[0], b[0]), _ssub(a[1], b[1]))


def _cmul_i(a, sgn):
    return (_sneg(a[1]), a[0]) if sgn > 0 else (a[1], _sneg(a[0]))


def _radix4(x, sgn):
    t0, t1 = _cadd(x[0], x[2]), _csub(x[0], x[2])
    t2, t3 = _cadd(x[1], x[3]), _cmul_i(_csub(x[1], x[3]), sgn)
    return [_cadd(t0, t2), _cadd(t1, t3), _csub(t0, t2), _csub(t1, t3)]


def _twiddle16(a, m, sgn):
    if m == 0:
        return a
    if m == 4:
        return _cmul_i(a, sgn)
    c, s = math.cos(2 * math.pi * m / 16), sgn * math.sin(2 * math.pi * m / 16)
    if m in (2, 6):
        if c * s > 0:
            return (_smul(_ssub(a[0], a[1]), c), _smul(_sadd(a[0], a[1]), c))
        return (_smul(_sadd(a[0], a[1]), c), _smul(_ssub(a[1], a[0]), c))
    return (_ssub(_smul(a[0], c), _smul(a[1], s)), _sadd(_smul(a[0], s), _smul(a[1], c)))


def _gate(x, t):
    if t is None:
        return x
    (sr, vr), (si, vi) = x
    return ((sr, vr + t), (si, vi + t))


def _fft16(x, sgn, g1=None, g2=None):
    g1 = g1 or [None] * 4
    g2 = g2 or [None] * 4
    a = [_radix4([_gate(x[n2], g1[n2])] + [x[4 * n1 + n2] for n1 in range(1, 4)], sgn) for n2 in range(4)]
    out = [None] * 16
    for k1 in range(4):
        y = _radix4([_gate(a[0][k1], g2[k1])]
                    + [_twiddle16(a[n2][k1], n2 * k1, sgn) for n2 in range(1, 4)], sgn)
        for k2 in range(4):
            out[k1 + 4 * k2] = y[k2]
    return out


def _val(a):
    return a[1] if a[0] > 0 else -a[1]


def _lo(u):
    return pltpu.bitcast(u << 16, f32)


def _hi(u):
    return pltpu.bitcast(u & jnp.uint32(0xFFFF0000), f32)


def _pack2(a, b):
    lo = pltpu.bitcast(a.astype(bf16).astype(f32), u32) >> 16
    return lo | pltpu.bitcast(b.astype(bf16).astype(f32), u32)


def _bf(u):
    return pltpu.bitcast(u, bf16)


def _dot(a, b):
    return jnp.dot(a, b, preferred_element_type=f32)


def _dot_nt(a, b):
    return lax.dot_general(a, b, NT, preferred_element_type=f32)


def _lane(rows):
    return lax.broadcasted_iota(jnp.int32, (rows, 128), 1)


def _mirror(v):
    return jnp.take_along_axis(v, (128 - _lane(v.shape[0])) & 127, axis=1)


def _rep(t, n):
    k = t.shape[0] // 8
    return jnp.broadcast_to(t.reshape(k, 1, 8, 128), (k, n, 8, 128)).reshape(k * n * 8, 128)


_PROFILE = False


def _scope(name):
    return jax.named_scope(name) if _PROFILE else contextlib.nullcontext()


_NGRP = 9
_S_OUT = _NGRP

_SCHED = ('a k0-4 v0-4 q0-4 k4-8 v4-8 p0-4 q4-8 k8-12 v8-12 p4-8 q8-12 k12-16 v12-16 p8-12 q12-16 '
          'o0-4 o4-9 p12-16 o9-12 o12-16').split()


def _kernel(xa_hbm, wr_hbm, wi_hbm, xb_hbm, m0_hbm, wq_hbm, wk_hbm, wv_hbm, wo_hbm,
            fd_hbm, fi_hbm, sd_hbm, out_hbm,
            xe, xe32, xa, xst, xg, wst, wca, wcb, wsl, xq, fd, fi, gs, wr, wi, tsc, rv, rn,
            z32, wo, wo32, xb, m0, stage, zq, psc, qsc, osc, ssc, sd, part, sems):
    w_hbms = (wq_hbm, wk_hbm, wv_hbm)

    def dyn(start, size):
        return pl.ds(start, size) if isinstance(start, int) else pl.ds(pl.multiple_of(start, size), size)

    def cp(src, dst, sem):
        return pltpu.make_async_copy(src, dst, sems.at[sem])

    def cp_w(m, g, sem):
        return cp(w_hbms[m].at[:, :, pl.ds(8 * g, 8), :], wst.at[4 * m + g], sem)

    def cp_xa(c0, c1, sem):
        rows = pl.ds(128 * c0, 128 * (c1 - c0))
        return cp(xa_hbm.at[:, rows, :], xa.at[:, rows, :], sem)

    def cp_f(src, dst, part, sem):
        rows = pl.ds(0, 160) if part == 0 else pl.ds(160, D // 2 + 1 - 160)
        return cp(src.at[rows, :], dst.at[rows, :], sem)

    def cp_half(k, sem):
        rows, cols = pl.ds(128 * k, 128), pl.ds(256 * k, 256)
        return [cp(wq_hbm.at[rows, :, pl.ds(0, 8), :], wst.at[0, rows], sem),
                cp(xb_hbm.at[:, pl.ds(KEEP, XT), cols], xe.at[:, :, cols], sem)]

    grp = [
        cp_half(0, 0),
        cp_half(1, 1) + [cp(fd_hbm.at[pl.ds(64, 8), pl.ds(0, 128)], zq, 1)],
        [cp_w(0, 1, 2)],
        [cp(sd_hbm, sd, 3), cp_w(0, 2, 3), cp_xa(0, 4, 3)],
        [cp_w(0, 3, 4), cp_xa(4, 8, 4), cp(fd_hbm.at[pl.ds(0, 64), :], fd, 4)],
        [cp_w(1, 0, 5), cp_f(wr_hbm, wr, 0, 5), cp_f(wi_hbm, wi, 0, 5), cp_w(1, 1, 5)],
        [cp_f(wr_hbm, wr, 1, 6), cp_f(wi_hbm, wi, 1, 6),
         cp_w(1, 2, 6), cp_w(1, 3, 6), cp_w(2, 0, 6), cp_w(2, 1, 6)],
        [cp_w(2, 2, 7), cp_w(2, 3, 7), cp(wo_hbm, wo, 7)],
        [cp(fi_hbm, fi, 8), cp(m0_hbm, m0, 8), cp(xb_hbm.at[:, pl.ds(0, KEEP), :], xb, 8)],
    ]
    for g_ in grp:
        for c_ in g_:
            c_.start()

    def wait(name, copies):
        with _scope(name):
            for c_ in copies:
                c_.wait()

    def tokens(stream):
        ys = jnp.concatenate(stream, axis=0)
        n = ys.shape[0] // 8

        def tok(start, count, step):
            assert start + (count - 1) * step < n, (start, count, step, n)
            first = min(start, n - count * step)
            y = ys[8 * first:8 * (first + count * step)].reshape(count, step, 8, 128)[:, start - first]
            return (pltpu.bitcast(y, u32) & zq[...][None]).reshape(count * 8, 128)
        return tok

    def opaque():
        z0 = zq[0, 0].astype(jnp.int32)
        idx = [jnp.clip(z0 + a, 0, NC - 1) for a in range(NC)]
        return lambda a: idx[a]

    def relayout(i, tok=None, start=0, step=1, r0=0, r1=D // 2):
        wc = (wca, wcb)[i % 2]
        n = r1 - r0
        m_lo, m_hi = jnp.uint32(0xFFFF), jnp.uint32(0xFFFF0000)
        if tok is not None:
            t1 = tok(start, n // 8, step)
            m_lo, m_hi = _rep(t1 | m_lo, 4), _rep(t1 | m_hi, 4)
            t2 = tok(start + 12, n // 8, step)
        ev = pltpu.bitcast(wst[i, r0:r1, 0].reshape(8 * n, DH), u32)
        od = pltpu.bitcast(wst[i, r0:r1, 1].reshape(8 * n, DH), u32)
        wc[0, 4 * r0:4 * r1, :] = (ev & m_lo) | (od << 16)
        wc[1, 4 * r0:4 * r1, :] = (ev >> 16) | (od & m_hi)
        for j in range(4):
            for p in range(2):
                v = wc[p, pl.ds(4 * r0 + j, n, stride=4), :]
                wsl[8 * i + 2 * j + p, r0:r1, :] = v if tok is None else v | t2

    def x_half(k, h0, h1):
        lhs = _bf(xe32[:, 256 * k:256 * k + 256])
        ys = []
        for h in range(h0, h1):
            ys.append(_dot(lhs, _bf(wsl[h, 128 * k:128 * k + 128, :])))
            if k == 0:
                part[h] = ys[-1]
            else:
                xq[:, h] = (ys[-1] + part[h]).astype(bf16).reshape(NSEG // SPB, SPB * XT, DH)
        return ys

    def pack_xe(k, tok=None):
        v = pltpu.bitcast(xe[:, :, 256 * k:256 * k + 256].reshape(NSEG * XT, 256), u32)
        if tok is not None:
            v = v | jnp.concatenate([tok(0, 32, 1)] * 2, axis=1)
        xe32[:, 256 * k:256 * k + 256] = v

    def x_heads(h0, h1):
        lhs = _bf(xe32[...])
        ys = []
        for h in range(h0, h1):
            ys.append(_dot(lhs, _bf(wsl[h])))
            xq[:, h] = ys[-1].astype(bf16).reshape(NSEG // SPB, SPB * XT, DH)
        return ys

    def gather_x(c0, c1, tok, per):
        nc = c1 - c0
        first = _lane(8 * nc) == 0
        for hf in range(2):
            tk = jnp.stack([tok((4 * hf + q) * per // 24, nc, per).reshape(nc, 8, 128) for q in range(4)], axis=1)
            tk = _rep(tk.reshape(32 * nc, 128), 2)
            u = pltpu.bitcast(xa[hf, 128 * c0:128 * c1, :], u32)
            for a in range(4):
                xst[a, hf, 64 * c0:64 * c1, :] = u[:, 128 * a:128 * a + 128] | tk
        for j in range(8):
            for p, part in enumerate((_lo, _hi)):
                tk = pltpu.bitcast(tok((8 + 2 * j + p) * per // 24, nc, per), f32)
                xl, xh = [[part(xst[a, hf, pl.ds(64 * c0 + j, 8 * nc, stride=8), :]) for a in range(4)]
                          for hf in range(2)]
                xl[0], xl[1] = xl[0] + tk, xl[1] + tk
                for hf in range(2):
                    x0, x1, x2, x3 = [(l + h if hf == 0 else l - h) for l, h in zip(xl, xh)]
                    s02, s13 = x0 + x2, x1 + x3
                    al, rb = x0 - x2, _mirror(x1 - x3)
                    v = jnp.concatenate([s02 + s13, s02 - s13, al - jnp.where(first, 0.0, rb),
                                         jnp.where(first, 0.0, al) + rb], axis=1)
                    xg[2 * j + p, 64 * hf + 8 * c0:64 * hf + 8 * c1, :] = v.astype(bf16)

    def build_gs(tok, step):
        tk = pltpu.bitcast(tok(0, 4 * NC, step), f32)
        ct, st = [jnp.concatenate([jnp.broadcast_to(sd[r0 + a:r0 + a + 1, :], (32, 128)) for a in range(NC)],
                                  axis=0) + tk for r0 in (128, 144)]
        ce, se = [[jnp.concatenate([sd[r0 + 32 * p:r0 + 32 * p + 32, :]] * NC, axis=0) for p in range(2)]
                  for r0 in (0, 64)]
        co = _pack2(*[ce[p] * ct - se[p] * st for p in range(2)])
        si = _pack2(*[se[p] * ct + ce[p] * st for p in range(2)])
        cr = pltpu.roll(co, 1, axis=1)
        ns = pltpu.roll(si, 1, axis=1) ^ jnp.uint32(0x80008000)
        ev = (_lane(32 * NC) & 1) == 0
        gs[:, 0:32, :] = jnp.concatenate(
            [jnp.where(ev, co, ns), jnp.where(ev, cr, si)], axis=1).reshape(NC, 32, 256)
        gs[:, 32:64, :] = jnp.concatenate(
            [jnp.where(ev, si, cr), jnp.where(ev, ns, co)], axis=1).reshape(NC, 32, 256)

    def d_fwd(a, at):
        y = [_dot_nt(_bf(fd[:, 128 * t:128 * t + 128]), xg[at(a), :, 128 * t:128 * t + 128]) for t in range(4)]
        ye = _pack2(y[0], y[1]).reshape(8, 2, 8, 128)
        po, qo = [y_.reshape(8, 2, 8, 128) for y_ in y[2:4]]
        p = jnp.concatenate([ye[:, 0], _pack2(po[:, 0], po[:, 1])], axis=0).reshape(128, 128)
        q = jnp.concatenate([ye[:, 1], _pack2(qo[:, 0], qo[:, 1])], axis=0).reshape(128, 128)
        q = pltpu.roll(q, 64, axis=1)
        q0 = q[0:8]
        row = lax.broadcasted_iota(jnp.int32, (8, 128), 0)
        q = jnp.concatenate([jnp.where(row == 0, q0 & jnp.uint32(0xFFFF0000), q0), q[8:]], axis=0)
        lo, lo8 = _lane(128) < 64, _lane(8) < 64
        nil = jnp.zeros((8, 128), u32)
        l0 = jnp.concatenate([jnp.where(lo, p, q), jnp.where(lo8, nil, q0)], axis=0)
        l1 = jnp.concatenate([jnp.where(lo, q, p), jnp.where(lo8, q0, nil)], axis=0)
        return _bf(l0), _bf(l1)

    def s_fwd(a, ls, at):
        o0 = _dot(ls[0], _bf(gs[at(a), :, 0:128]))[0:264]
        o1 = _dot(ls[1], _bf(gs[at(a), :, 128:256]))[0:264]
        ev = (_lane(264) & 1) == 0
        tsc[a, 0, 0:264, :] = jnp.where(ev, o0, o1)
        tsc[a, 1, 0:264, :] = jnp.where(ev, o1, o0)
        return o1

    def spectral_fwd(filler):
        at = opaque()
        ls = [d_fwd(a, at) for a in range(4)]
        stream = []
        for a in range(0, NC, 2):
            if a + 4 < NC:
                ls += [d_fwd(a + 4, at), d_fwd(a + 5, at)]
            if a == NC - 2:
                filler()
            s_fwd(a, ls[a], at)
            stream.append(s_fwd(a + 1, ls[a + 1], at))
        return stream

    rel = [0, 1, 2, 3, 4, 7, 10, 13, 16, 17.5, 19, 20.5]

    def spectral_mid(p, v0, v1, tok, start, per):
        nu = v1 - v0
        at = opaque()
        gate = lambda r: pltpu.bitcast(tok(start + int((r + 4) * per / 24), nu, per), f32)
        gates = [gate(r) for r in rel]
        pre = [gate(r - 4) for r in rel[0:4]]
        r0, r1 = 128 * p + 8 * v0, 128 * p + 8 * v1
        if p == 2:
            filt = lambda w, k2: w[256:257, 128 * k2:128 * k2 + 128].astype(f32)
        else:
            filt = lambda w, k2: (_lo, _hi)[p](pltpu.bitcast(w[16 * v0:16 * v1, 128 * k2:128 * k2 + 128], u32))
        t = [((1, tsc[at(a), 0, r0:r1, :]), (1, pltpu.roll(tsc[at(a), 1, r0:r1, :] + pre[a % 4], 127, axis=1)))
             for a in range(NC)]
        if p == 2:
            t = [_cmul_i(v, -1) for v in t]
        x = _fft16(t, -1, gates[0:4], gates[4:8])
        y = []
        for k2 in range(NC):
            fa, fb = filt(wr, k2), filt(wi, k2)
            (sr, xr), (si, xi) = x[k2]
            y.append((_ssub((sr, xr * fa), (si, xi * fb)), _sadd((sr, xr * fb), (si, xi * fa))))
        ev = (_lane(8 * nu) & 1) == 0
        u = _fft16(y, 1, None, gates[8:12])
        for k1 in range(4):
            ui = jnp.stack([_val(u[k1 + 4 * k2][1]).reshape(nu, 8, 128) for k2 in range(4)], axis=1)
            us4 = pltpu.roll(ui.reshape(32 * nu, 128), 1, axis=1).reshape(nu, 4, 8, 128)
            for k2 in range(4):
                ur, us = _val(u[k1 + 4 * k2][0]), us4[:, k2].reshape(8 * nu, 128)
                v01 = jnp.concatenate([jnp.where(ev, ur, us), jnp.where(ev, us, ur)], axis=1)
                if p == 2:
                    rn[k1 + 4 * k2, 0:8, :] = v01
                else:
                    rv[k1 + 4 * k2, r0:r1, :] = v01.astype(bf16)

    def spectral_inv():
        first = _lane(64) == 0
        ev = (_lane(64) & 1) == 0
        at = opaque()

        def comb(zs):
            return [_pack2(zs[0][0] + zs[0][1], zs[1][0] + zs[1][1]),
                    _pack2(zs[0][0] - zs[0][1], zs[1][0] - zs[1][1])]

        for j in range(8):
            gre, gri = [], []
            for a in (2 * j, 2 * j + 1):
                g = gs[at(a)]
                re = [g[0:32, 0:128], g[32:64, 128:256]]
                im = [g[32:64, 0:128], g[0:32, 128:256]]
                gre.append([_bf(v) for v in re])
                gri.append([_bf(jnp.stack([r_.reshape(4, 8, 128), i_.reshape(4, 8, 128)], axis=1).reshape(64, 128))
                            for r_, i_ in zip(re, im)])

            def tile(t):
                zs = [[_dot_nt(gri[c][e], rv[at(2 * j + c), 128 * t:128 * t + 128, 128 * e:128 * e + 128])
                       for e in range(2)] for c in range(2)]
                out = [z.reshape(4, 2, 16, 128) for z in comb(zs)]
                return [(z[:, 0].reshape(64, 128), z[:, 1].reshape(64, 128)) for z in out]

            if j < 7:
                odd = tile(1)
            nq = [jnp.concatenate([rn[at(2 * j + c), 0:8, :], jnp.zeros((120, 256), f32)], axis=0).astype(bf16)
                  for c in range(2)]
            nyq = comb([[_dot_nt(gre[c][e], nq[c][:, 128 * e:128 * e + 128]) for e in range(2)]
                        for c in range(2)])
            even = tile(0)
            if j == 7:
                odd = tile(1)
            for be in range(2):
                zr, zi = even[be]
                sh = pltpu.roll(jnp.where(first, nyq[be], zi), 1, axis=1)
                tiles = [jnp.where(ev, zr, sh), jnp.where(ev, sh, zr), odd[be][0], odd[be][1]]
                for t in range(4):
                    z32[t, pl.ds(512 * be + j, 64, stride=8), :] = tiles[t]

    def copy_wo(tok, step):
        tk = _rep(tok(0, 128, step), 2)
        wo32[...] = pltpu.bitcast(wo[...], u32) | jnp.concatenate([tk] * 4, axis=1)

    def xv_part(b, h0, h1):
        lhs = _bf(xe32[dyn(16 * b, 16), :])
        ys = []
        for h in range(h0, h1):
            ys.append(_dot(lhs, _bf(wsl[2 * H + h])))
            xq[b, 2 * H + h] = ys[-1].astype(bf16)
        return ys

    wait('w0', grp[0])
    with _scope('b0'):
        for c in range(4):
            relayout(0, r0=32 * c, r1=32 * c + 32)
        pack_xe(0)
        x_half(0, 0, 6)

    wait('w1', grp[1])
    with _scope('b1'):
        tok = tokens(x_half(0, 6, 8)[1:])
        relayout(0, tok, 0, 2, r0=128)
        pack_xe(1, tok)
        x_half(1, 0, 4)

    wait('w2', grp[2])
    with _scope('b2'):
        relayout(1, tokens(x_half(1, 4, 8)[1::2]), 0, 3)
        x_heads(8, 14)

    wait('w3', grp[3])
    with _scope('b3'):
        relayout(2, tokens(x_heads(14, 16)), 0, 3)
        tok = tokens(x_heads(16, 22))
        gather_x(0, 4, tok, 84)
        build_gs(tok, 5)

    wait('w4', grp[4])
    with _scope('b4'):
        relayout(3, tokens(x_heads(22, 24)), 0, 3)
        gather_x(4, 8, tokens(x_heads(24, 29)), 68)
        spectral_fwd(lambda: x_heads(29, 30))

    wait('w5', grp[5])
    with _scope('b5'):
        relayout(4, tokens(x_heads(30, 32)), 0, 3)
        tok = tokens(x_heads(32, 40))
        relayout(5, tok, 0, 14)
        spectral_mid(0, 0, 10, tok, 0, 50)
        spectral_mid(1, 0, 6, tokens(x_heads(40, 46)), 0, 54)

    wait('w6', grp[6])
    with _scope('b6'):
        relayout(6, tokens(x_heads(46, 48)), 0, 3)
        tok = tokens(x_heads(48, 56))
        relayout(7, tok, 0, 7)
        relayout(8, tok, 230, 7)
        spectral_mid(0, 10, 16, tok, 0, 72)
        spectral_mid(2, 0, 1, tok, 430, 72)
        tok = tokens(x_heads(56, 62) + x_heads(64, 64 + XVP // 2))
        relayout(9, tok, 0, 16)
        spectral_mid(1, 6, 16, tok, 0, 52)
        spectral_inv()

    wait('w7', grp[7])
    with _scope('b7'):
        st = x_heads(62, 64) + x_heads(64 + XVP // 2, 64 + XVP) + xv_part(0, XVP, 16)
        tok = tokens(st)
        relayout(10, tok, 0, 4)
        relayout(11, tok, 150, 4)
        copy_wo(tokens(st + xv_part(0, 16, H)), 3)
    wait('w8', grp[8])

    r = lax.broadcasted_iota(jnp.int32, (R2, 128), 0)
    c = lax.broadcasted_iota(jnp.int32, (R2, 128), 1)

    def head_pos(i):
        head = jnp.where(i < 32, 0, jnp.where(i < 64, 1, jnp.where(i < 72, 0, jnp.where(i < R2, 1, 2))))
        pos = jnp.where(i < 32, i, jnp.where(i < 72, i - 32, i - 40))
        return head, pos

    rh, rpos = head_pos(r)
    ch, cpos = head_pos(c)
    same = (rh - ch) == 0
    ok = jnp.logical_and(same, jnp.logical_or(rpos < MEM, rpos >= cpos))
    fill = jnp.where(same, jnp.float32(-1e9 / SCALE), jnp.float32(-jnp.inf))

    def step(b, k, mem, filler):
        s = SPB * b + k
        second = k % 2 == 1
        mo = 48 if second else 32
        lhs = jnp.concatenate([mem, xb[s].astype(f32)], axis=0).astype(bf16)
        acc = [None] * 4
        stream = []

        def proj(m, hp):
            y = jnp.concatenate([_dot(lhs, _bf(wsl[H * m + 2 * hp + hh])) for hh in range(2)], axis=0)
            qsc[m, hp] = y.astype(bf16)
            stream.append(y)

        def oper(m, hp):
            xs = [xq[b, H * m + 2 * hp + hh, XT * k:XT * k + XT, :] for hh in range(2)]
            if m > 0:
                xs.append(jnp.zeros((128 - R2, DH), bf16))
            return jnp.concatenate([qsc[m, hp]] + xs, axis=0)

        def do_qkp(hp):
            proj(0, hp)
            proj(1, hp)

        def do_v(hp):
            proj(2, hp)

        def do_qk(hp):
            ssc[hp] = jnp.where(ok, _dot_nt(oper(0, hp), oper(1, hp)), fill)
            stream.clear()

        def do_softmax(p0, p1):
            nt = 20 if p1 < NP else 5
            g = pltpu.bitcast(_rep(tokens(stream[0:3])(0, nt, 1), 40 // nt), f32)
            sc = ssc[p0:p1].reshape(4 * R2, 128) + g
            mx = jnp.max(sc, axis=-1, keepdims=True)
            e = jnp.exp2((sc - mx) * (SCALE * LOG2E))
            l = jnp.sum(e, axis=-1, keepdims=True)
            rl = pl.reciprocal(l, approx=True)
            rl = rl * (2.0 - l * rl)
            psc[p0:p1] = (e * rl).astype(bf16).reshape(4, R2, 128)

        def do_pv(hp):
            o2 = _dot(psc[hp], oper(2, hp))
            r0 = 40 if second else 32
            for hh in range(2):
                osc[2 * hp + hh, 0:32, :] = o2[32 * hh:32 * hh + 32].astype(bf16)
                osc[2 * hp + hh, r0:r0 + 8, :] = o2[64 + 8 * hh:72 + 8 * hh].astype(bf16)

        def do_o(p0, p1):
            ol = jnp.concatenate([osc[h, 0:mo, :] for h in range(2 * p0, 2 * p1)], axis=1)
            for n in range(4):
                y = _dot(ol, _bf(wo32[p0 * 128:p1 * 128, 128 * n:128 * n + 128]))
                acc[n] = y if acc[n] is None else acc[n] + y
                stream.append(y)

        def do_a3():
            zr = dyn(16 * s, 32)
            v0, v2, vc, vs = [_dot(_bf(z32[t, zr, :]), _bf(fi[:, 128 * t:128 * t + 128])) for t in range(4)]
            sp, sm = v0 + v2, v0 - v2
            first = _lane(2 * SEG) == 0
            al, be = vc + jnp.where(first, 0.0, vs), _mirror(vs - jnp.where(first, 0.0, vc))
            ya = jnp.concatenate([sp + al, sm + be, sp - al, sm - be], axis=1).astype(bf16)
            stage[pl.ds(s, 2), :, 0:D] = ya.reshape(2, SEG, D)

        for op in _SCHED:
            if op == 'a':
                if not second:
                    do_a3()
                continue
            p0, p1 = [int(v) for v in op[1:].split('-')]
            if op[0] == 'p':
                do_softmax(p0, p1)
            if op[0] == 'o':
                do_o(p0, p1)
            else:
                for hp in range(p0, p1):
                    {'k': do_qkp, 'v': do_v, 'q': do_qk, 'p': do_pv}[op[0]](hp)
        filler()
        return jnp.concatenate(acc, axis=1)

    nb = NSEG // SPB
    hv = [XVP + (H - XVP) * k // SPB for k in range(SPB + 1)]

    def body(b, mem):
        nxt = jnp.minimum(b + 1, nb - 1)
        for k in range(0, SPB, 2):
            sa, sb = SPB * b + k, SPB * b + k + 1
            ya = step(b, k, mem, lambda: xv_part(nxt, hv[k], hv[k + 1]))
            stage[sa, 0:KEEP, D:2 * D] = ya[MEM:].astype(bf16)
            mem_b = ya[0:MEM].astype(bf16).astype(f32)
            yb = step(b, k + 1, mem_b, lambda: xv_part(nxt, hv[k + 1], hv[k + 2]))
            stage[sa, KEEP:SEG, D:2 * D] = yb[32:40].astype(bf16)
            stage[sb, :, D:2 * D] = jnp.concatenate([yb[MEM:32], yb[40:48]], axis=0).astype(bf16)
            mem = yb[0:MEM].astype(bf16).astype(f32)
            rows = pl.ds(sa, 2)
            cp(stage.at[rows], out_hbm.at[rows], _S_OUT).start()
        return mem

    with _scope('main'):
        lax.fori_loop(0, nb, body, m0[...].astype(f32))
    wait('w9', [cp(stage, out_hbm, _S_OUT)])


@jax.jit
def pallas_concat_heads__spectral_gfnet__memory_aug_recurrent_mem_tr__prompt_kernel(
    A_x: jax.Array,
    A_w_r: jax.Array,
    A_w_i: jax.Array,
    B_x: jax.Array,
    B_mem0: jax.Array,
    B_Wq: jax.Array,
    B_Wk: jax.Array,
    B_Wv: jax.Array,
    B_Wo: jax.Array,
    B_seg_len: jax.Array,
):
    del B_seg_len
    assert A_x.shape == (1, S, D) and B_x.shape == (1, S, D) and B_mem0.shape == (1, MEM, D)
    assert B_Wq.shape == (D, H, DH) and B_Wo.shape == (H, DH, D)
    fd, fi, sd = _dft_tables()
    vm = pltpu.VMEM
    scratch = [
        vm((NSEG, XT, D), bf16),
        vm((NSEG * XT // 2, D), u32),
        vm((2, S // 2, D), bf16),
        vm((4, 2, S // 4, 128), u32),
        vm((NC, 128, D), bf16),
        vm((12, D // 2, 2, 8, DH), bf16),
        vm((2, 2 * D, DH), u32),
        vm((2, 2 * D, DH), u32),
        vm((3 * H, D // 2, DH), u32),
        vm((NSEG // SPB, 3 * H, SPB * XT, DH), bf16),
        vm((64, 512), u32),
        vm((64, 512), u32),
        vm((NC, 64, 256), u32),
        vm((D // 2 + 1, S), bf16),
        vm((D // 2 + 1, S), bf16),
        vm((NC, 2, 272, 128), f32),
        vm((NC, 256, 256), bf16),
        vm((NC, 16, 256), f32),
        vm((4, S // 2, 128), u32),
        vm((H * DH, D), bf16),
        vm((H * DH // 2, D), u32),
        vm((NSEG, KEEP, D), bf16),
        vm((MEM, D), bf16),
        vm((NSEG, SEG, 2 * D), bf16),
        vm((8, 128), u32),
        vm((NP, R2, 128), bf16),
        vm((3, NP, 64, DH), bf16),
        vm((H, 48, DH), bf16),
        vm((NP, R2, 128), f32),
        vm((160, 128), f32),
        vm((8, NSEG * XT, DH), f32),
        pltpu.SemaphoreType.DMA((_NGRP + 1,)),
    ]
    w4 = lambda w: w.reshape(D // 2, 2, H, DH)
    out = pl.pallas_call(
        _kernel,
        out_shape=jax.ShapeDtypeStruct((NSEG, SEG, 2 * D), bf16),
        in_specs=[pl.BlockSpec(memory_space=pl.ANY)] * 12,
        out_specs=pl.BlockSpec(memory_space=pl.ANY),
        scratch_shapes=scratch,
        compiler_params=pltpu.CompilerParams(vmem_limit_bytes=110 * 1024 * 1024),
    )(A_x.reshape(2, S // 2, D), A_w_r.T, A_w_i.T, B_x.reshape(NSEG, SEG, D), B_mem0.reshape(MEM, D),
      w4(B_Wq), w4(B_Wk), w4(B_Wv), B_Wo.reshape(H * DH, D), fd, fi, sd)
    return out.reshape(1, S, 2 * D)
```

```python
import contextlib
import math

import numpy as np
import jax
import jax.numpy as jnp
from jax import lax
import jax.experimental.pallas as pl
import jax.experimental.pallas.tpu as pltpu

S, D = 2048, 512
H, DH = 32, 128
MEM, SEG = 8, 32
NSEG = S // SEG
NP = H // 2
XT = 8
KEEP = SEG - XT
R2 = 2 * (MEM + SEG)
SCALE = DH ** -0.5
LOG2E = 1.4426950408889634
NC = 16
SPB = 4
XVP = 6
XVL = 20

f32, bf16, u32 = jnp.float32, jnp.bfloat16, jnp.uint32
NT = (((1,), (1,)), ((), ()))


def _pack_rows(m):
    b = np.asarray(m, np.float32).astype(jnp.bfloat16).view(np.uint16).astype(np.uint32)
    return b[0::2, :] | (b[1::2, :] << 16)


def _dft_tables():
    k = np.arange(D // 2)[:, None]
    d = np.arange(D // 2)[None, :]
    ang = 2.0 * np.pi * ((k * d) % D) / D
    pm = np.cos(ang)
    qm = -np.sin(ang)
    qm[0] = (-1.0) ** np.arange(D // 2)
    qo = qm[:, :128].copy()
    qo[:, 0] = qm[:, 128]

    def inter(parts):
        c = parts[0].shape[1]
        return np.stack([p.reshape(-1, 8, c) for p in parts], axis=1).reshape(-1, c)

    f0 = inter([pm[0::4, :128], qm[0::4, :128]])
    f2 = inter([pm[2::4, :128], qm[2::4, :128]])
    fp = inter([pm[1::4, :128], pm[3::4, :128]])
    fq = inter([qo[1::4], qo[3::4]])
    fd = np.concatenate([np.concatenate([f0, f2, fp, fq], axis=1), np.zeros((16, 512))], axis=0)
    wgt = np.where(k == 0, 1.0, 2.0) / (S * D)
    pw, qw = wgt * pm, wgt * qm
    ii = np.arange(64)
    i0 = np.zeros((128, 128))
    i2 = np.zeros((128, 128))
    i0[2 * ii], i0[2 * ii + 1] = pw[0::4, :128], qw[0::4, :128]
    i2[2 * ii + 1], i2[(2 * ii + 2) % 128] = pw[2::4, :128], qw[2::4, :128]
    fi = np.concatenate([i0, i2, pw[1::2, :128], (wgt * qo)[1::2]], axis=1)
    k1 = np.arange(128)[None, :]
    mo = np.concatenate([ii[0::2], ii[1::2]])[:, None]
    ae = 2.0 * np.pi * ((NC * mo * k1) % S) / S
    at = 2.0 * np.pi * (np.arange(NC)[:, None] * k1) / S
    sd = np.concatenate([np.cos(ae), np.sin(ae), np.cos(at), np.sin(at)], axis=0).astype(np.float32)
    return _pack_rows(fd), _pack_rows(fi), sd


def _sadd(a, b):
    (sa, va), (sb, vb) = a, b
    if sa == sb:
        return (sa, va + vb)
    return (1, va - vb) if sa > 0 else (1, vb - va)


def _sneg(a):
    return (-a[0], a[1])


def _ssub(a, b):
    return _sadd(a, _sneg(b))


def _smul(a, c):
    return (a[0], a[1] * c) if c > 0 else (-a[0], a[1] * (-c))


def _cadd(a, b):
    return (_sadd(a[0], b[0]), _sadd(a[1], b[1]))


def _csub(a, b):
    return (_ssub(a[0], b[0]), _ssub(a[1], b[1]))


def _cmul_i(a, sgn):
    return (_sneg(a[1]), a[0]) if sgn > 0 else (a[1], _sneg(a[0]))


def _radix4(x, sgn):
    t0, t1 = _cadd(x[0], x[2]), _csub(x[0], x[2])
    t2, t3 = _cadd(x[1], x[3]), _cmul_i(_csub(x[1], x[3]), sgn)
    return [_cadd(t0, t2), _cadd(t1, t3), _csub(t0, t2), _csub(t1, t3)]


def _twiddle16(a, m, sgn):
    if m == 0:
        return a
    if m == 4:
        return _cmul_i(a, sgn)
    c, s = math.cos(2 * math.pi * m / 16), sgn * math.sin(2 * math.pi * m / 16)
    if m in (2, 6):
        if c * s > 0:
            return (_smul(_ssub(a[0], a[1]), c), _smul(_sadd(a[0], a[1]), c))
        return (_smul(_sadd(a[0], a[1]), c), _smul(_ssub(a[1], a[0]), c))
    return (_ssub(_smul(a[0], c), _smul(a[1], s)), _sadd(_smul(a[0], s), _smul(a[1], c)))


def _gate(x, t):
    if t is None:
        return x
    (sr, vr), (si, vi) = x
    return ((sr, vr + t), (si, vi + t))


def _fft16(x, sgn, g1=None, g2=None):
    g1 = g1 or [None] * 4
    g2 = g2 or [None] * 4
    a = [_radix4([_gate(x[n2], g1[n2])] + [x[4 * n1 + n2] for n1 in range(1, 4)], sgn) for n2 in range(4)]
    out = [None] * 16
    for k1 in range(4):
        y = _radix4([_gate(a[0][k1], g2[k1])]
                    + [_twiddle16(a[n2][k1], n2 * k1, sgn) for n2 in range(1, 4)], sgn)
        for k2 in range(4):
            out[k1 + 4 * k2] = y[k2]
    return out


def _val(a):
    return a[1] if a[0] > 0 else -a[1]


def _lo(u):
    return pltpu.bitcast(u << 16, f32)


def _hi(u):
    return pltpu.bitcast(u & jnp.uint32(0xFFFF0000), f32)


def _pack2(a, b):
    lo = pltpu.bitcast(a.astype(bf16).astype(f32), u32) >> 16
    return lo | pltpu.bitcast(b.astype(bf16).astype(f32), u32)


def _bf(u):
    return pltpu.bitcast(u, bf16)


def _dot(a, b):
    return jnp.dot(a, b, preferred_element_type=f32)


def _dot_nt(a, b):
    return lax.dot_general(a, b, NT, preferred_element_type=f32)


def _lane(rows):
    return lax.broadcasted_iota(jnp.int32, (rows, 128), 1)


def _mirror(v):
    return jnp.take_along_axis(v, (128 - _lane(v.shape[0])) & 127, axis=1)


def _rep(t, n):
    k = t.shape[0] // 8
    return jnp.broadcast_to(t.reshape(k, 1, 8, 128), (k, n, 8, 128)).reshape(k * n * 8, 128)


_PROFILE = False


def _scope(name):
    return jax.named_scope(name) if _PROFILE else contextlib.nullcontext()


_NGRP = 9
_S_OUT = _NGRP

_SCHED = ('a k0-4 v0-4 q0-4 k4-8 v4-8 p0-4 q4-8 k8-12 v8-12 p4-8 q8-12 k12-16 v12-16 p8-12 q12-16 '
          'o0-4 o4-9 p12-16 o9-12 o12-16').split()


def _kernel(xa_hbm, wr_hbm, wi_hbm, xb_hbm, m0_hbm, wq_hbm, wk_hbm, wv_hbm, wo_hbm,
            fd_hbm, fi_hbm, sd_hbm, out_hbm,
            xe, xe32, xa, xst, xg, wst, wca, wcb, wsl, xq, fd, fi, gs, wr, wi, tsc, rv, rn,
            z32, wo, wo32, xb, m0, stage, zq, psc, qsc, osc, ssc, sd, part, sems):
    w_hbms = (wq_hbm, wk_hbm, wv_hbm)

    def dyn(start, size):
        return pl.ds(start, size) if isinstance(start, int) else pl.ds(pl.multiple_of(start, size), size)

    def cp(src, dst, sem):
        return pltpu.make_async_copy(src, dst, sems.at[sem])

    def cp_w(m, g, sem):
        return cp(w_hbms[m].at[:, :, pl.ds(8 * g, 8), :], wst.at[4 * m + g], sem)

    def cp_xa(c0, c1, sem):
        rows = pl.ds(128 * c0, 128 * (c1 - c0))
        return cp(xa_hbm.at[:, rows, :], xa.at[:, rows, :], sem)

    def cp_f(src, dst, part, sem):
        rows = pl.ds(0, 160) if part == 0 else pl.ds(160, D // 2 + 1 - 160)
        return cp(src.at[rows, :], dst.at[rows, :], sem)

    def cp_half(k, sem):
        rows, cols = pl.ds(128 * k, 128), pl.ds(256 * k, 256)
        return [cp(wq_hbm.at[rows, :, pl.ds(0, 8), :], wst.at[0, rows], sem),
                cp(xb_hbm.at[:, pl.ds(KEEP, XT), cols], xe.at[:, :, cols], sem)]

    grp = [
        cp_half(0, 0),
        cp_half(1, 1) + [cp(fd_hbm.at[pl.ds(64, 8), pl.ds(0, 128)], zq, 1)],
        [cp_w(0, 1, 2)],
        [cp(sd_hbm, sd, 3), cp_w(0, 2, 3), cp_xa(0, 4, 3)],
        [cp_w(0, 3, 4), cp_xa(4, 8, 4), cp(fd_hbm.at[pl.ds(0, 64), :], fd, 4)],
        [cp_w(1, 0, 5), cp_f(wr_hbm, wr, 0, 5), cp_f(wi_hbm, wi, 0, 5), cp_w(1, 1, 5)],
        [cp_f(wr_hbm, wr, 1, 6), cp_f(wi_hbm, wi, 1, 6),
         cp_w(1, 2, 6), cp_w(1, 3, 6), cp_w(2, 0, 6), cp_w(2, 1, 6)],
        [cp_w(2, 2, 7), cp_w(2, 3, 7), cp(wo_hbm, wo, 7)],
        [cp(fi_hbm, fi, 8), cp(m0_hbm, m0, 8), cp(xb_hbm.at[:, pl.ds(0, KEEP), :], xb, 8)],
    ]
    for g_ in grp:
        for c_ in g_:
            c_.start()

    def wait(name, copies):
        with _scope(name):
            for c_ in copies:
                c_.wait()

    def tokens(stream):
        ys = jnp.concatenate(stream, axis=0)
        n = ys.shape[0] // 8

        def tok(start, count, step):
            assert start + (count - 1) * step < n, (start, count, step, n)
            first = min(start, n - count * step)
            y = ys[8 * first:8 * (first + count * step)].reshape(count, step, 8, 128)[:, start - first]
            return (pltpu.bitcast(y, u32) & zq[...][None]).reshape(count * 8, 128)
        return tok

    def opaque():
        z0 = zq[0, 0].astype(jnp.int32)
        idx = [jnp.clip(z0 + a, 0, NC - 1) for a in range(NC)]
        return lambda a: idx[a]

    def relayout(i, tok=None, start=0, step=1, r0=0, r1=D // 2):
        wc = (wca, wcb)[i % 2]
        n = r1 - r0
        m_lo, m_hi = jnp.uint32(0xFFFF), jnp.uint32(0xFFFF0000)
        if tok is not None:
            t1 = tok(start, n // 8, step)
            m_lo, m_hi = _rep(t1 | m_lo, 4), _rep(t1 | m_hi, 4)
            t2 = tok(start + 12, n // 8, step)
        ev = pltpu.bitcast(wst[i, r0:r1, 0].reshape(8 * n, DH), u32)
        od = pltpu.bitcast(wst[i, r0:r1, 1].reshape(8 * n, DH), u32)
        wc[0, 4 * r0:4 * r1, :] = (ev & m_lo) | (od << 16)
        wc[1, 4 * r0:4 * r1, :] = (ev >> 16) | (od & m_hi)
        for j in range(4):
            for p in range(2):
                v = wc[p, pl.ds(4 * r0 + j, n, stride=4), :]
                wsl[8 * i + 2 * j + p, r0:r1, :] = v if tok is None else v | t2

    def x_half(k, h0, h1):
        lhs = _bf(xe32[:, 256 * k:256 * k + 256])
        ys = []
        for h in range(h0, h1):
            ys.append(_dot(lhs, _bf(wsl[h, 128 * k:128 * k + 128, :])))
            if k == 0:
                part[h] = ys[-1]
            else:
                xq[:, h] = (ys[-1] + part[h]).astype(bf16).reshape(NSEG // SPB, SPB * XT, DH)
        return ys

    def pack_xe(k, tok=None):
        v = pltpu.bitcast(xe[:, :, 256 * k:256 * k + 256].reshape(NSEG * XT, 256), u32)
        if tok is not None:
            v = v | jnp.concatenate([tok(0, 32, 1)] * 2, axis=1)
        xe32[:, 256 * k:256 * k + 256] = v

    def x_heads(h0, h1):
        lhs = _bf(xe32[...])
        ys = []
        for h in range(h0, h1):
            ys.append(_dot(lhs, _bf(wsl[h])))
            xq[:, h] = ys[-1].astype(bf16).reshape(NSEG // SPB, SPB * XT, DH)
        return ys

    def gather_x(c0, c1, tok, per):
        nc = c1 - c0
        first = _lane(8 * nc) == 0
        for hf in range(2):
            tk = jnp.stack([tok((4 * hf + q) * per // 24, nc, per).reshape(nc, 8, 128) for q in range(4)], axis=1)
            tk = _rep(tk.reshape(32 * nc, 128), 2)
            u = pltpu.bitcast(xa[hf, 128 * c0:128 * c1, :], u32)
            for a in range(4):
                xst[a, hf, 64 * c0:64 * c1, :] = u[:, 128 * a:128 * a + 128] | tk
        for j in range(8):
            for p, part in enumerate((_lo, _hi)):
                tk = pltpu.bitcast(tok((8 + 2 * j + p) * per // 24, nc, per), f32)
                xl, xh = [[part(xst[a, hf, pl.ds(64 * c0 + j, 8 * nc, stride=8), :]) for a in range(4)]
                          for hf in range(2)]
                xl[0], xl[1] = xl[0] + tk, xl[1] + tk
                for hf in range(2):
                    x0, x1, x2, x3 = [(l + h if hf == 0 else l - h) for l, h in zip(xl, xh)]
                    s02, s13 = x0 + x2, x1 + x3
                    al, rb = x0 - x2, _mirror(x1 - x3)
                    v = jnp.concatenate([s02 + s13, s02 - s13, al - jnp.where(first, 0.0, rb),
                                         jnp.where(first, 0.0, al) + rb], axis=1)
                    xg[2 * j + p, 64 * hf + 8 * c0:64 * hf + 8 * c1, :] = v.astype(bf16)

    def build_gs(tok, step):
        tk = pltpu.bitcast(tok(0, 4 * NC, step), f32)
        ct, st = [jnp.concatenate([jnp.broadcast_to(sd[r0 + a:r0 + a + 1, :], (32, 128)) for a in range(NC)],
                                  axis=0) + tk for r0 in (128, 144)]
        ce, se = [[jnp.concatenate([sd[r0 + 32 * p:r0 + 32 * p + 32, :]] * NC, axis=0) for p in range(2)]
                  for r0 in (0, 64)]
        co = _pack2(*[ce[p] * ct - se[p] * st for p in range(2)])
        si = _pack2(*[se[p] * ct + ce[p] * st for p in range(2)])
        cr = pltpu.roll(co, 1, axis=1)
        ns = pltpu.roll(si, 1, axis=1) ^ jnp.uint32(0x80008000)
        ev = (_lane(32 * NC) & 1) == 0
        gs[:, 0:32, :] = jnp.concatenate(
            [jnp.where(ev, co, ns), jnp.where(ev, cr, si)], axis=1).reshape(NC, 32, 256)
        gs[:, 32:64, :] = jnp.concatenate(
            [jnp.where(ev, si, cr), jnp.where(ev, ns, co)], axis=1).reshape(NC, 32, 256)

    def d_fwd(a, at):
        y = [_dot_nt(_bf(fd[:, 128 * t:128 * t + 128]), xg[at(a), :, 128 * t:128 * t + 128]) for t in range(4)]
        ye = _pack2(y[0], y[1]).reshape(8, 2, 8, 128)
        po, qo = [y_.reshape(8, 2, 8, 128) for y_ in y[2:4]]
        p = jnp.concatenate([ye[:, 0], _pack2(po[:, 0], po[:, 1])], axis=0).reshape(128, 128)
        q = jnp.concatenate([ye[:, 1], _pack2(qo[:, 0], qo[:, 1])], axis=0).reshape(128, 128)
        q = pltpu.roll(q, 64, axis=1)
        q0 = q[0:8]
        row = lax.broadcasted_iota(jnp.int32, (8, 128), 0)
        q = jnp.concatenate([jnp.where(row == 0, q0 & jnp.uint32(0xFFFF0000), q0), q[8:]], axis=0)
        lo, lo8 = _lane(128) < 64, _lane(8) < 64
        nil = jnp.zeros((8, 128), u32)
        l0 = jnp.concatenate([jnp.where(lo, p, q), jnp.where(lo8, nil, q0)], axis=0)
        l1 = jnp.concatenate([jnp.where(lo, q, p), jnp.where(lo8, q0, nil)], axis=0)
        return _bf(l0), _bf(l1)

    def s_fwd(a, ls, at):
        o0 = _dot(ls[0], _bf(gs[at(a), :, 0:128]))[0:264]
        o1 = _dot(ls[1], _bf(gs[at(a), :, 128:256]))[0:264]
        ev = (_lane(264) & 1) == 0
        tsc[a, 0, 0:264, :] = jnp.where(ev, o0, o1)
        tsc[a, 1, 0:264, :] = jnp.where(ev, o1, o0)
        return o1

    def spectral_fwd(filler):
        at = opaque()
        ls = [d_fwd(a, at) for a in range(4)]
        stream = []
        for a in range(0, NC, 2):
            if a + 4 < NC:
                ls += [d_fwd(a + 4, at), d_fwd(a + 5, at)]
            if a == NC - 2:
                filler()
            s_fwd(a, ls[a], at)
            stream.append(s_fwd(a + 1, ls[a + 1], at))
        return stream

    rel = [0, 1, 2, 3, 4, 7, 10, 13, 16, 17.5, 19, 20.5]

    def spectral_mid(p, v0, v1, tok, start, per):
        nu = v1 - v0
        at = opaque()
        gate = lambda r: pltpu.bitcast(tok(start + int((r + 4) * per / 24), nu, per), f32)
        gates = [gate(r) for r in rel]
        pre = [gate(r - 4) for r in rel[0:4]]
        r0, r1 = 128 * p + 8 * v0, 128 * p + 8 * v1
        if p == 2:
            filt = lambda w, k2: w[256:257, 128 * k2:128 * k2 + 128].astype(f32)
        else:
            filt = lambda w, k2: (_lo, _hi)[p](pltpu.bitcast(w[16 * v0:16 * v1, 128 * k2:128 * k2 + 128], u32))
        t = [((1, tsc[at(a), 0, r0:r1, :]), (1, pltpu.roll(tsc[at(a), 1, r0:r1, :] + pre[a % 4], 127, axis=1)))
             for a in range(NC)]
        if p == 2:
            t = [_cmul_i(v, -1) for v in t]
        x = _fft16(t, -1, gates[0:4], gates[4:8])
        y = []
        for k2 in range(NC):
            fa, fb = filt(wr, k2), filt(wi, k2)
            (sr, xr), (si, xi) = x[k2]
            y.append((_ssub((sr, xr * fa), (si, xi * fb)), _sadd((sr, xr * fb), (si, xi * fa))))
        ev = (_lane(8 * nu) & 1) == 0
        u = _fft16(y, 1, None, gates[8:12])
        for k1 in range(4):
            ui = jnp.stack([_val(u[k1 + 4 * k2][1]).reshape(nu, 8, 128) for k2 in range(4)], axis=1)
            us4 = pltpu.roll(ui.reshape(32 * nu, 128), 1, axis=1).reshape(nu, 4, 8, 128)
            for k2 in range(4):
                ur, us = _val(u[k1 + 4 * k2][0]), us4[:, k2].reshape(8 * nu, 128)
                v01 = jnp.concatenate([jnp.where(ev, ur, us), jnp.where(ev, us, ur)], axis=1)
                if p == 2:
                    rn[k1 + 4 * k2, 0:8, :] = v01
                else:
                    rv[k1 + 4 * k2, r0:r1, :] = v01.astype(bf16)

    def spectral_inv():
        first = _lane(64) == 0
        ev = (_lane(64) & 1) == 0
        at = opaque()

        def comb(zs):
            return [_pack2(zs[0][0] + zs[0][1], zs[1][0] + zs[1][1]),
                    _pack2(zs[0][0] - zs[0][1], zs[1][0] - zs[1][1])]

        for j in range(8):
            gre, gri = [], []
            for a in (2 * j, 2 * j + 1):
                g = gs[at(a)]
                re = [g[0:32, 0:128], g[32:64, 128:256]]
                im = [g[32:64, 0:128], g[0:32, 128:256]]
                gre.append([_bf(v) for v in re])
                gri.append([_bf(jnp.stack([r_.reshape(4, 8, 128), i_.reshape(4, 8, 128)], axis=1).reshape(64, 128))
                            for r_, i_ in zip(re, im)])

            def tile(t):
                zs = [[_dot_nt(gri[c][e], rv[at(2 * j + c), 128 * t:128 * t + 128, 128 * e:128 * e + 128])
                       for e in range(2)] for c in range(2)]
                out = [z.reshape(4, 2, 16, 128) for z in comb(zs)]
                return [(z[:, 0].reshape(64, 128), z[:, 1].reshape(64, 128)) for z in out]

            if j < 7:
                odd = tile(1)
            nq = [jnp.concatenate([rn[at(2 * j + c), 0:8, :], jnp.zeros((120, 256), f32)], axis=0).astype(bf16)
                  for c in range(2)]
            nyq = comb([[_dot_nt(gre[c][e], nq[c][:, 128 * e:128 * e + 128]) for e in range(2)]
                        for c in range(2)])
            even = tile(0)
            if j == 7:
                odd = tile(1)
            for be in range(2):
                zr, zi = even[be]
                sh = pltpu.roll(jnp.where(first, nyq[be], zi), 1, axis=1)
                tiles = [jnp.where(ev, zr, sh), jnp.where(ev, sh, zr), odd[be][0], odd[be][1]]
                for t in range(4):
                    z32[t, pl.ds(512 * be + j, 64, stride=8), :] = tiles[t]

    def copy_wo(tok, step):
        tk = _rep(tok(0, 64, step), 4)
        wo32[...] = pltpu.bitcast(wo[...], u32) | jnp.concatenate([tk] * 4, axis=1)

    def xv_part(b, h0, h1):
        lhs = _bf(xe32[dyn(16 * b, 16), :])
        ys = []
        for h in range(h0, h1):
            ys.append(_dot(lhs, _bf(wsl[2 * H + h])))
            xq[b, 2 * H + h] = ys[-1].astype(bf16)
        return ys

    wait('w0', grp[0])
    with _scope('b0'):
        for c in range(4):
            relayout(0, r0=32 * c, r1=32 * c + 32)
        pack_xe(0)
        x_half(0, 0, 6)

    wait('w1', grp[1])
    with _scope('b1'):
        tok = tokens(x_half(0, 6, 8)[1:])
        relayout(0, tok, 0, 2, r0=128)
        pack_xe(1, tok)
        x_half(1, 0, 4)

    wait('w2', grp[2])
    with _scope('b2'):
        relayout(1, tokens(x_half(1, 4, 8)[1::2]), 0, 3)
        x_heads(8, 14)

    wait('w3', grp[3])
    with _scope('b3'):
        relayout(2, tokens(x_heads(14, 16)), 0, 3)
        tok = tokens(x_heads(16, 22))
        gather_x(0, 4, tok, 84)
        build_gs(tok, 5)

    wait('w4', grp[4])
    with _scope('b4'):
        relayout(3, tokens(x_heads(22, 24)), 0, 3)
        gather_x(4, 8, tokens(x_heads(24, 29)), 68)
        spectral_fwd(lambda: x_heads(29, 30))

    wait('w5', grp[5])
    with _scope('b5'):
        relayout(4, tokens(x_heads(30, 32)), 0, 3)
        tok = tokens(x_heads(32, 40))
        relayout(5, tok, 0, 14)
        spectral_mid(0, 0, 10, tok, 0, 50)
        spectral_mid(1, 0, 6, tokens(x_heads(40, 46)), 0, 54)

    wait('w6', grp[6])
    with _scope('b6'):
        relayout(6, tokens(x_heads(46, 48)), 0, 3)
        tok = tokens(x_heads(48, 56))
        relayout(7, tok, 0, 7)
        relayout(8, tok, 230, 7)
        spectral_mid(0, 10, 16, tok, 0, 72)
        spectral_mid(2, 0, 1, tok, 430, 72)
        tok = tokens(x_heads(56, 62) + x_heads(64, 64 + XVP // 2))
        relayout(9, tok, 0, 16)
        spectral_mid(1, 6, 16, tok, 0, 52)
        spectral_inv()

    wait('w7', grp[7])
    with _scope('b7'):
        st = x_heads(62, 64) + x_heads(64 + XVP // 2, 64 + XVP) + xv_part(0, XVP, 16)
        tok = tokens(st)
        relayout(10, tok, 0, 4)
        relayout(11, tok, 150, 4)
        copy_wo(tokens(st + xv_part(0, 16, XVL)), 5)
    wait('w8', grp[8])

    r = lax.broadcasted_iota(jnp.int32, (R2, 128), 0)
    c = lax.broadcasted_iota(jnp.int32, (R2, 128), 1)

    def head_pos(i):
        head = jnp.where(i < 32, 0, jnp.where(i < 64, 1, jnp.where(i < 72, 0, jnp.where(i < R2, 1, 2))))
        pos = jnp.where(i < 32, i, jnp.where(i < 72, i - 32, i - 40))
        return head, pos

    rh, rpos = head_pos(r)
    ch, cpos = head_pos(c)
    same = (rh - ch) == 0
    ok = jnp.logical_and(same, jnp.logical_or(rpos < MEM, rpos >= cpos))
    fill = jnp.where(same, jnp.float32(-1e9 / SCALE), jnp.float32(-jnp.inf))

    def step(b, k, mem, filler):
        s = SPB * b + k
        second = k % 2 == 1
        mo = 48 if second else 32
        lhs = jnp.concatenate([mem, xb[s].astype(f32)], axis=0).astype(bf16)
        if not second:
            lhs48 = jnp.concatenate([lhs, _bf(xe32[dyn(4 * s, 8), :])], axis=0)
        acc = [None] * 4
        stream = []

        def proj(m, hp):
            y = jnp.concatenate([_dot(lhs, _bf(wsl[H * m + 2 * hp + hh])) for hh in range(2)], axis=0)
            qsc[m, hp] = y.astype(bf16)
            stream.append(y)

        def oper(m, hp):
            xs = [xq[b, H * m + 2 * hp + hh, XT * k:XT * k + XT, :] for hh in range(2)]
            if m > 0:
                xs.append(jnp.zeros((128 - R2, DH), bf16))
            return jnp.concatenate([qsc[m, hp]] + xs, axis=0)

        def do_qkp(hp):
            proj(0, hp)
            proj(1, hp)

        def do_v(hp):
            if second or 2 * hp < XVL:
                proj(2, hp)
                return
            ys = [_dot(lhs48, _bf(wsl[2 * H + 2 * hp + hh])) for hh in range(2)]
            y = jnp.concatenate([ys[0][0:32], ys[1][0:32]], axis=0)
            qsc[2, hp] = y.astype(bf16)
            for hh in range(2):
                xq[b, 2 * H + 2 * hp + hh, XT * k:XT * k + 2 * XT, :] = ys[hh][32:48].astype(bf16)
            stream.append(y)

        def do_qk(hp):
            ssc[hp] = jnp.where(ok, _dot_nt(oper(0, hp), oper(1, hp)), fill)
            stream.clear()

        def do_softmax(p0, p1):
            nt = 20 if p1 < NP else 5
            g = pltpu.bitcast(_rep(tokens(stream[0:3])(0, nt, 1), 40 // nt), f32)
            sc = ssc[p0:p1].reshape(4 * R2, 128) + g
            mx = jnp.max(sc, axis=-1, keepdims=True)
            e = jnp.exp2((sc - mx) * (SCALE * LOG2E))
            l = jnp.sum(e, axis=-1, keepdims=True)
            rl = pl.reciprocal(l, approx=True)
            rl = rl * (2.0 - l * rl)
            psc[p0:p1] = (e * rl).astype(bf16).reshape(4, R2, 128)

        def do_pv(hp):
            o2 = _dot(psc[hp], oper(2, hp))
            r0 = 40 if second else 32
            for hh in range(2):
                osc[2 * hp + hh, 0:32, :] = o2[32 * hh:32 * hh + 32].astype(bf16)
                osc[2 * hp + hh, r0:r0 + 8, :] = o2[64 + 8 * hh:72 + 8 * hh].astype(bf16)

        def do_o(p0, p1):
            ol = jnp.concatenate([osc[h, 0:mo, :] for h in range(2 * p0, 2 * p1)], axis=1)
            for n in range(4):
                y = _dot(ol, _bf(wo32[p0 * 128:p1 * 128, 128 * n:128 * n + 128]))
                acc[n] = y if acc[n] is None else acc[n] + y
                stream.append(y)

        def do_a3():
            zr = dyn(16 * s, 32)
            v0, v2, vc, vs = [_dot(_bf(z32[t, zr, :]), _bf(fi[:, 128 * t:128 * t + 128])) for t in range(4)]
            sp, sm = v0 + v2, v0 - v2
            first = _lane(2 * SEG) == 0
            al, be = vc + jnp.where(first, 0.0, vs), _mirror(vs - jnp.where(first, 0.0, vc))
            ya = jnp.concatenate([sp + al, sm + be, sp - al, sm - be], axis=1).astype(bf16)
            stage[pl.ds(s, 2), :, 0:D] = ya.reshape(2, SEG, D)

        for op in _SCHED:
            if op == 'a':
                if not second:
                    do_a3()
                continue
            p0, p1 = [int(v) for v in op[1:].split('-')]
            if op[0] == 'p':
                do_softmax(p0, p1)
            if op[0] == 'o':
                do_o(p0, p1)
            else:
                for hp in range(p0, p1):
                    {'k': do_qkp, 'v': do_v, 'q': do_qk, 'p': do_pv}[op[0]](hp)
        filler()
        return jnp.concatenate(acc, axis=1)

    nb = NSEG // SPB
    hv = [XVP, 10, 12, 16, XVL]

    def body(b, mem):
        nxt = jnp.minimum(b + 1, nb - 1)
        for k in range(0, SPB, 2):
            sa, sb = SPB * b + k, SPB * b + k + 1
            ya = step(b, k, mem, lambda: xv_part(nxt, hv[k], hv[k + 1]))
            stage[sa, 0:KEEP, D:2 * D] = ya[MEM:].astype(bf16)
            mem_b = ya[0:MEM].astype(bf16).astype(f32)
            yb = step(b, k + 1, mem_b, lambda: xv_part(nxt, hv[k + 1], hv[k + 2]))
            stage[sa, KEEP:SEG, D:2 * D] = yb[32:40].astype(bf16)
            stage[sb, :, D:2 * D] = jnp.concatenate([yb[MEM:32], yb[40:48]], axis=0).astype(bf16)
            mem = yb[0:MEM].astype(bf16).astype(f32)
            rows = pl.ds(sa, 2)
            cp(stage.at[rows], out_hbm.at[rows], _S_OUT).start()
        return mem

    with _scope('main'):
        lax.fori_loop(0, nb, body, m0[...].astype(f32))
    wait('w9', [cp(stage, out_hbm, _S_OUT)])


@jax.jit
def pallas_concat_heads__spectral_gfnet__memory_aug_recurrent_mem_tr__prompt_kernel(
    A_x: jax.Array,
    A_w_r: jax.Array,
    A_w_i: jax.Array,
    B_x: jax.Array,
    B_mem0: jax.Array,
    B_Wq: jax.Array,
    B_Wk: jax.Array,
    B_Wv: jax.Array,
    B_Wo: jax.Array,
    B_seg_len: jax.Array,
):
    del B_seg_len
    assert A_x.shape == (1, S, D) and B_x.shape == (1, S, D) and B_mem0.shape == (1, MEM, D)
    assert B_Wq.shape == (D, H, DH) and B_Wo.shape == (H, DH, D)
    fd, fi, sd = _dft_tables()
    vm = pltpu.VMEM
    scratch = [
        vm((NSEG, XT, D), bf16),
        vm((NSEG * XT // 2, D), u32),
        vm((2, S // 2, D), bf16),
        vm((4, 2, S // 4, 128), u32),
        vm((NC, 128, D), bf16),
        vm((12, D // 2, 2, 8, DH), bf16),
        vm((2, 2 * D, DH), u32),
        vm((2, 2 * D, DH), u32),
        vm((3 * H, D // 2, DH), u32),
        vm((NSEG // SPB, 3 * H, SPB * XT, DH), bf16),
        vm((64, 512), u32),
        vm((64, 512), u32),
        vm((NC, 64, 256), u32),
        vm((D // 2 + 1, S), bf16),
        vm((D // 2 + 1, S), bf16),
        vm((NC, 2, 272, 128), f32),
        vm((NC, 256, 256), bf16),
        vm((NC, 16, 256), f32),
        vm((4, S // 2, 128), u32),
        vm((H * DH, D), bf16),
        vm((H * DH // 2, D), u32),
        vm((NSEG, KEEP, D), bf16),
        vm((MEM, D), bf16),
        vm((NSEG, SEG, 2 * D), bf16),
        vm((8, 128), u32),
        vm((NP, R2, 128), bf16),
        vm((3, NP, 64, DH), bf16),
        vm((H, 48, DH), bf16),
        vm((NP, R2, 128), f32),
        vm((160, 128), f32),
        vm((8, NSEG * XT, DH), f32),
        pltpu.SemaphoreType.DMA((_NGRP + 1,)),
    ]
    w4 = lambda w: w.reshape(D // 2, 2, H, DH)
    out = pl.pallas_call(
        _kernel,
        out_shape=jax.ShapeDtypeStruct((NSEG, SEG, 2 * D), bf16),
        in_specs=[pl.BlockSpec(memory_space=pl.ANY)] * 12,
        out_specs=pl.BlockSpec(memory_space=pl.ANY),
        scratch_shapes=scratch,
        compiler_params=pltpu.CompilerParams(vmem_limit_bytes=110 * 1024 * 1024),
    )(A_x.reshape(2, S // 2, D), A_w_r.T, A_w_i.T, B_x.reshape(NSEG, SEG, D), B_mem0.reshape(MEM, D),
      w4(B_Wq), w4(B_Wk), w4(B_Wv), B_Wo.reshape(H * DH, D), fd, fi, sd)
    return out.reshape(1, S, 2 * D)
```

```python
import math

import numpy as np
import jax
import jax.numpy as jnp
from jax import lax
import jax.experimental.pallas as pl
import jax.experimental.pallas.tpu as pltpu

S, D = 2048, 512
H, DH = 32, 128
MEM, SEG = 8, 32
NSEG = S // SEG
NP = H // 2
XT = 8
KEEP = SEG - XT
R2 = 2 * (MEM + SEG)
SCALE = DH ** -0.5
LOG2E = 1.4426950408889634
NC = 16
SPB = 4
XVP = 6
XVL = 20

f32, bf16, u32 = jnp.float32, jnp.bfloat16, jnp.uint32
NT = (((1,), (1,)), ((), ()))


def _pack_rows(m):
    b = np.asarray(m, np.float32).astype(jnp.bfloat16).view(np.uint16).astype(np.uint32)
    return b[0::2, :] | (b[1::2, :] << 16)


def _dft_tables():
    k = np.arange(D // 2)[:, None]
    d = np.arange(D // 2)[None, :]
    ang = 2.0 * np.pi * ((k * d) % D) / D
    pm = np.cos(ang)
    qm = -np.sin(ang)
    qm[0] = (-1.0) ** np.arange(D // 2)
    qo = qm[:, :128].copy()
    qo[:, 0] = qm[:, 128]

    def inter(parts):
        c = parts[0].shape[1]
        return np.stack([p.reshape(-1, 8, c) for p in parts], axis=1).reshape(-1, c)

    f0 = inter([pm[0::4, :128], qm[0::4, :128]])
    f2 = inter([pm[2::4, :128], qm[2::4, :128]])
    fp = inter([pm[1::4, :128], pm[3::4, :128]])
    fq = inter([qo[1::4], qo[3::4]])
    fd = np.concatenate([np.concatenate([f0, f2, fp, fq], axis=1), np.zeros((16, 512))], axis=0)
    wgt = np.where(k == 0, 1.0, 2.0) / (S * D)
    pw, qw = wgt * pm, wgt * qm
    ii = np.arange(64)
    i0 = np.zeros((128, 128))
    i2 = np.zeros((128, 128))
    i0[2 * ii], i0[2 * ii + 1] = pw[0::4, :128], qw[0::4, :128]
    i2[2 * ii + 1], i2[(2 * ii + 2) % 128] = pw[2::4, :128], qw[2::4, :128]
    fi = np.concatenate([i0, i2, pw[1::2, :128], (wgt * qo)[1::2]], axis=1)
    k1 = np.arange(128)[None, :]
    mo = np.concatenate([ii[0::2], ii[1::2]])[:, None]
    ae = 2.0 * np.pi * ((NC * mo * k1) % S) / S
    at = 2.0 * np.pi * (np.arange(NC)[:, None] * k1) / S
    sd = np.concatenate([np.cos(ae), np.sin(ae), np.cos(at), np.sin(at)], axis=0).astype(np.float32)
    return _pack_rows(fd), _pack_rows(fi), sd


def _sadd(a, b):
    (sa, va), (sb, vb) = a, b
    if sa == sb:
        return (sa, va + vb)
    return (1, va - vb) if sa > 0 else (1, vb - va)


def _sneg(a):
    return (-a[0], a[1])


def _ssub(a, b):
    return _sadd(a, _sneg(b))


def _smul(a, c):
    return (a[0], a[1] * c) if c > 0 else (-a[0], a[1] * (-c))


def _cadd(a, b):
    return (_sadd(a[0], b[0]), _sadd(a[1], b[1]))


def _csub(a, b):
    return (_ssub(a[0], b[0]), _ssub(a[1], b[1]))


def _cmul_i(a, sgn):
    return (_sneg(a[1]), a[0]) if sgn > 0 else (a[1], _sneg(a[0]))


def _radix4(x, sgn):
    t0, t1 = _cadd(x[0], x[2]), _csub(x[0], x[2])
    t2, t3 = _cadd(x[1], x[3]), _cmul_i(_csub(x[1], x[3]), sgn)
    return [_cadd(t0, t2), _cadd(t1, t3), _csub(t0, t2), _csub(t1, t3)]


def _twiddle16(a, m, sgn):
    if m == 0:
        return a
    if m == 4:
        return _cmul_i(a, sgn)
    c, s = math.cos(2 * math.pi * m / 16), sgn * math.sin(2 * math.pi * m / 16)
    if m in (2, 6):
        if c * s > 0:
            return (_smul(_ssub(a[0], a[1]), c), _smul(_sadd(a[0], a[1]), c))
        return (_smul(_sadd(a[0], a[1]), c), _smul(_ssub(a[1], a[0]), c))
    return (_ssub(_smul(a[0], c), _smul(a[1], s)), _sadd(_smul(a[0], s), _smul(a[1], c)))


def _gate(x, t):
    if t is None:
        return x
    (sr, vr), (si, vi) = x
    return ((sr, vr + t), (si, vi + t))


def _fft16(x, sgn, g1=None, g2=None):
    g1 = g1 or [None] * 4
    g2 = g2 or [None] * 4
    a = [_radix4([_gate(x[n2], g1[n2])] + [x[4 * n1 + n2] for n1 in range(1, 4)], sgn) for n2 in range(4)]
    out = [None] * 16
    for k1 in range(4):
        y = _radix4([_gate(a[0][k1], g2[k1])]
                    + [_twiddle16(a[n2][k1], n2 * k1, sgn) for n2 in range(1, 4)], sgn)
        for k2 in range(4):
            out[k1 + 4 * k2] = y[k2]
    return out


def _val(a):
    return a[1] if a[0] > 0 else -a[1]


def _lo(u):
    return pltpu.bitcast(u << 16, f32)


def _hi(u):
    return pltpu.bitcast(u & jnp.uint32(0xFFFF0000), f32)


def _pack2(a, b):
    lo = pltpu.bitcast(a.astype(bf16).astype(f32), u32) >> 16
    return lo | pltpu.bitcast(b.astype(bf16).astype(f32), u32)


def _bf(u):
    return pltpu.bitcast(u, bf16)


def _dot(a, b):
    return jnp.dot(a, b, preferred_element_type=f32)


def _dot_nt(a, b):
    return lax.dot_general(a, b, NT, preferred_element_type=f32)


def _lane(rows):
    return lax.broadcasted_iota(jnp.int32, (rows, 128), 1)


def _mirror(v):
    return jnp.take_along_axis(v, (128 - _lane(v.shape[0])) & 127, axis=1)


def _rep(t, n):
    k = t.shape[0] // 8
    return jnp.broadcast_to(t.reshape(k, 1, 8, 128), (k, n, 8, 128)).reshape(k * n * 8, 128)


_NGRP = 9
_S_OUT = _NGRP

_SCHED = ('a k0-4 v0-4 q0-4 k4-8 v4-8 p0-4 q4-8 k8-12 v8-12 p4-8 q8-12 k12-16 v12-16 p8-12 q12-16 '
          'o0-4 o4-9 p12-16 o9-12 o12-16').split()


def _kernel(xa_hbm, wr_hbm, wi_hbm, xb_hbm, m0_hbm, wq_hbm, wk_hbm, wv_hbm, wo_hbm,
            fd_hbm, fi_hbm, sd_hbm, out_hbm,
            xe, xe32, xa, xst, xg, wst, wca, wcb, wsl, xq, fd, fi, gs, wr, wi, tsc, rv, rn,
            z32, wo, wo32, xb, m0, stage, zq, psc, qsc, osc, ssc, sd, part, sems):
    w_hbms = (wq_hbm, wk_hbm, wv_hbm)

    def dyn(start, size):
        return pl.ds(start, size) if isinstance(start, int) else pl.ds(pl.multiple_of(start, size), size)

    def cp(src, dst, sem):
        return pltpu.make_async_copy(src, dst, sems.at[sem])

    def cp_w(m, g, sem):
        return cp(w_hbms[m].at[:, :, pl.ds(8 * g, 8), :], wst.at[4 * m + g], sem)

    def cp_xa(c0, c1, sem):
        rows = pl.ds(128 * c0, 128 * (c1 - c0))
        return cp(xa_hbm.at[:, rows, :], xa.at[:, rows, :], sem)

    def cp_f(src, dst, part, sem):
        rows = pl.ds(0, 160) if part == 0 else pl.ds(160, D // 2 + 1 - 160)
        return cp(src.at[rows, :], dst.at[rows, :], sem)

    def cp_half(k, sem):
        rows, cols = pl.ds(128 * k, 128), pl.ds(256 * k, 256)
        return [cp(wq_hbm.at[rows, :, pl.ds(0, 8), :], wst.at[0, rows], sem),
                cp(xb_hbm.at[:, pl.ds(KEEP, XT), cols], xe.at[:, :, cols], sem)]

    grp = [
        cp_half(0, 0),
        cp_half(1, 1) + [cp(fd_hbm.at[pl.ds(64, 8), pl.ds(0, 128)], zq, 1)],
        [cp_w(0, 1, 2)],
        [cp(sd_hbm, sd, 3), cp_w(0, 2, 3), cp_xa(0, 4, 3)],
        [cp_w(0, 3, 4), cp_xa(4, 8, 4), cp(fd_hbm.at[pl.ds(0, 64), :], fd, 4)],
        [cp_w(1, 0, 5), cp_f(wr_hbm, wr, 0, 5), cp_f(wi_hbm, wi, 0, 5), cp_w(1, 1, 5)],
        [cp_f(wr_hbm, wr, 1, 6), cp_f(wi_hbm, wi, 1, 6),
         cp_w(1, 2, 6), cp_w(1, 3, 6), cp_w(2, 0, 6), cp_w(2, 1, 6)],
        [cp_w(2, 2, 7), cp_w(2, 3, 7), cp(wo_hbm, wo, 7)],
        [cp(fi_hbm, fi, 8), cp(m0_hbm, m0, 8), cp(xb_hbm.at[:, pl.ds(0, KEEP), :], xb, 8)],
    ]
    for g_ in grp:
        for c_ in g_:
            c_.start()

    def wait(copies):
        for c_ in copies:
            c_.wait()

    def tokens(stream):
        ys = jnp.concatenate(stream, axis=0)
        n = ys.shape[0] // 8

        def tok(start, count, step):
            assert start + (count - 1) * step < n, (start, count, step, n)
            first = min(start, n - count * step)
            y = ys[8 * first:8 * (first + count * step)].reshape(count, step, 8, 128)[:, start - first]
            return (pltpu.bitcast(y, u32) & zq[...][None]).reshape(count * 8, 128)
        return tok

    def opaque():
        z0 = zq[0, 0].astype(jnp.int32)
        idx = [jnp.clip(z0 + a, 0, NC - 1) for a in range(NC)]
        return lambda a: idx[a]

    def relayout(i, tok=None, start=0, step=1, r0=0, r1=D // 2):
        wc = (wca, wcb)[i % 2]
        n = r1 - r0
        m_lo, m_hi = jnp.uint32(0xFFFF), jnp.uint32(0xFFFF0000)
        if tok is not None:
            t1 = tok(start, n // 8, step)
            m_lo, m_hi = _rep(t1 | m_lo, 4), _rep(t1 | m_hi, 4)
            t2 = tok(start + 12, n // 8, step)
        ev = pltpu.bitcast(wst[i, r0:r1, 0].reshape(8 * n, DH), u32)
        od = pltpu.bitcast(wst[i, r0:r1, 1].reshape(8 * n, DH), u32)
        wc[0, 4 * r0:4 * r1, :] = (ev & m_lo) | (od << 16)
        wc[1, 4 * r0:4 * r1, :] = (ev >> 16) | (od & m_hi)
        for j in range(4):
            for p in range(2):
                v = wc[p, pl.ds(4 * r0 + j, n, stride=4), :]
                wsl[8 * i + 2 * j + p, r0:r1, :] = v if tok is None else v | t2

    def x_half(k, h0, h1):
        lhs = _bf(xe32[:, 256 * k:256 * k + 256])
        ys = []
        for h in range(h0, h1):
            ys.append(_dot(lhs, _bf(wsl[h, 128 * k:128 * k + 128, :])))
            if k == 0:
                part[h] = ys[-1]
            else:
                xq[:, h] = (ys[-1] + part[h]).astype(bf16).reshape(NSEG // SPB, SPB * XT, DH)
        return ys

    def pack_xe(k, tok=None):
        v = pltpu.bitcast(xe[:, :, 256 * k:256 * k + 256].reshape(NSEG * XT, 256), u32)
        if tok is not None:
            v = v | jnp.concatenate([tok(0, 32, 1)] * 2, axis=1)
        xe32[:, 256 * k:256 * k + 256] = v

    def x_heads(h0, h1):
        lhs = _bf(xe32[...])
        ys = []
        for h in range(h0, h1):
            ys.append(_dot(lhs, _bf(wsl[h])))
            xq[:, h] = ys[-1].astype(bf16).reshape(NSEG // SPB, SPB * XT, DH)
        return ys

    def gather_x(c0, c1, tok, per):
        nc = c1 - c0
        first = _lane(8 * nc) == 0
        for hf in range(2):
            tk = jnp.stack([tok((4 * hf + q) * per // 24, nc, per).reshape(nc, 8, 128) for q in range(4)], axis=1)
            tk = _rep(tk.reshape(32 * nc, 128), 2)
            u = pltpu.bitcast(xa[hf, 128 * c0:128 * c1, :], u32)
            for a in range(4):
                xst[a, hf, 64 * c0:64 * c1, :] = u[:, 128 * a:128 * a + 128] | tk
        for j in range(8):
            for p, part in enumerate((_lo, _hi)):
                tk = pltpu.bitcast(tok((8 + 2 * j + p) * per // 24, nc, per), f32)
                xl, xh = [[part(xst[a, hf, pl.ds(64 * c0 + j, 8 * nc, stride=8), :]) for a in range(4)]
                          for hf in range(2)]
                xl[0], xl[1] = xl[0] + tk, xl[1] + tk
                for hf in range(2):
                    x0, x1, x2, x3 = [(l + h if hf == 0 else l - h) for l, h in zip(xl, xh)]
                    s02, s13 = x0 + x2, x1 + x3
                    al, rb = x0 - x2, _mirror(x1 - x3)
                    v = jnp.concatenate([s02 + s13, s02 - s13, al - jnp.where(first, 0.0, rb),
                                         jnp.where(first, 0.0, al) + rb], axis=1)
                    xg[2 * j + p, 64 * hf + 8 * c0:64 * hf + 8 * c1, :] = v.astype(bf16)

    def build_gs(tok, step):
        tk = pltpu.bitcast(tok(0, 4 * NC, step), f32)
        ct, st = [jnp.concatenate([jnp.broadcast_to(sd[r0 + a:r0 + a + 1, :], (32, 128)) for a in range(NC)],
                                  axis=0) + tk for r0 in (128, 144)]
        ce, se = [[jnp.concatenate([sd[r0 + 32 * p:r0 + 32 * p + 32, :]] * NC, axis=0) for p in range(2)]
                  for r0 in (0, 64)]
        co = _pack2(*[ce[p] * ct - se[p] * st for p in range(2)])
        si = _pack2(*[se[p] * ct + ce[p] * st for p in range(2)])
        cr = pltpu.roll(co, 1, axis=1)
        ns = pltpu.roll(si, 1, axis=1) ^ jnp.uint32(0x80008000)
        ev = (_lane(32 * NC) & 1) == 0
        gs[:, 0:32, :] = jnp.concatenate(
            [jnp.where(ev, co, ns), jnp.where(ev, cr, si)], axis=1).reshape(NC, 32, 256)
        gs[:, 32:64, :] = jnp.concatenate(
            [jnp.where(ev, si, cr), jnp.where(ev, ns, co)], axis=1).reshape(NC, 32, 256)

    def d_fwd(a, at):
        y = [_dot_nt(_bf(fd[:, 128 * t:128 * t + 128]), xg[at(a), :, 128 * t:128 * t + 128]) for t in range(4)]
        ye = _pack2(y[0], y[1]).reshape(8, 2, 8, 128)
        po, qo = [y_.reshape(8, 2, 8, 128) for y_ in y[2:4]]
        p = jnp.concatenate([ye[:, 0], _pack2(po[:, 0], po[:, 1])], axis=0).reshape(128, 128)
        q = jnp.concatenate([ye[:, 1], _pack2(qo[:, 0], qo[:, 1])], axis=0).reshape(128, 128)
        q = pltpu.roll(q, 64, axis=1)
        q0 = q[0:8]
        row = lax.broadcasted_iota(jnp.int32, (8, 128), 0)
        q = jnp.concatenate([jnp.where(row == 0, q0 & jnp.uint32(0xFFFF0000), q0), q[8:]], axis=0)
        lo, lo8 = _lane(128) < 64, _lane(8) < 64
        nil = jnp.zeros((8, 128), u32)
        l0 = jnp.concatenate([jnp.where(lo, p, q), jnp.where(lo8, nil, q0)], axis=0)
        l1 = jnp.concatenate([jnp.where(lo, q, p), jnp.where(lo8, q0, nil)], axis=0)
        return _bf(l0), _bf(l1)

    def s_fwd(a, ls, at):
        o0 = _dot(ls[0], _bf(gs[at(a), :, 0:128]))[0:264]
        o1 = _dot(ls[1], _bf(gs[at(a), :, 128:256]))[0:264]
        ev = (_lane(264) & 1) == 0
        tsc[a, 0, 0:264, :] = jnp.where(ev, o0, o1)
        tsc[a, 1, 0:264, :] = jnp.where(ev, o1, o0)
        return o1

    def spectral_fwd(filler):
        at = opaque()
        ls = [d_fwd(a, at) for a in range(4)]
        stream = []
        for a in range(0, NC, 2):
            if a + 4 < NC:
                ls += [d_fwd(a + 4, at), d_fwd(a + 5, at)]
            if a == NC - 2:
                filler()
            s_fwd(a, ls[a], at)
            stream.append(s_fwd(a + 1, ls[a + 1], at))
        return stream

    rel = [0, 1, 2, 3, 4, 7, 10, 13, 16, 17.5, 19, 20.5]

    def spectral_mid(p, v0, v1, tok, start, per):
        nu = v1 - v0
        at = opaque()
        gate = lambda r: pltpu.bitcast(tok(start + int((r + 4) * per / 24), nu, per), f32)
        gates = [gate(r) for r in rel]
        pre = [gate(r - 4) for r in rel[0:4]]
        r0, r1 = 128 * p + 8 * v0, 128 * p + 8 * v1
        if p == 2:
            filt = lambda w, k2: w[256:257, 128 * k2:128 * k2 + 128].astype(f32)
        else:
            filt = lambda w, k2: (_lo, _hi)[p](pltpu.bitcast(w[16 * v0:16 * v1, 128 * k2:128 * k2 + 128], u32))
        t = [((1, tsc[at(a), 0, r0:r1, :]), (1, pltpu.roll(tsc[at(a), 1, r0:r1, :] + pre[a % 4], 127, axis=1)))
             for a in range(NC)]
        if p == 2:
            t = [_cmul_i(v, -1) for v in t]
        x = _fft16(t, -1, gates[0:4], gates[4:8])
        y = []
        for k2 in range(NC):
            fa, fb = filt(wr, k2), filt(wi, k2)
            (sr, xr), (si, xi) = x[k2]
            y.append((_ssub((sr, xr * fa), (si, xi * fb)), _sadd((sr, xr * fb), (si, xi * fa))))
        ev = (_lane(8 * nu) & 1) == 0
        u = _fft16(y, 1, None, gates[8:12])
        for k1 in range(4):
            ui = jnp.stack([_val(u[k1 + 4 * k2][1]).reshape(nu, 8, 128) for k2 in range(4)], axis=1)
            us4 = pltpu.roll(ui.reshape(32 * nu, 128), 1, axis=1).reshape(nu, 4, 8, 128)
            for k2 in range(4):
                ur, us = _val(u[k1 + 4 * k2][0]), us4[:, k2].reshape(8 * nu, 128)
                v01 = jnp.concatenate([jnp.where(ev, ur, us), jnp.where(ev, us, ur)], axis=1)
                if p == 2:
                    rn[k1 + 4 * k2, 0:8, :] = v01
                else:
                    rv[k1 + 4 * k2, r0:r1, :] = v01.astype(bf16)

    def spectral_inv():
        first = _lane(64) == 0
        ev = (_lane(64) & 1) == 0
        at = opaque()

        def comb(zs):
            return [_pack2(zs[0][0] + zs[0][1], zs[1][0] + zs[1][1]),
                    _pack2(zs[0][0] - zs[0][1], zs[1][0] - zs[1][1])]

        for j in range(8):
            gre, gri = [], []
            for a in (2 * j, 2 * j + 1):
                g = gs[at(a)]
                re = [g[0:32, 0:128], g[32:64, 128:256]]
                im = [g[32:64, 0:128], g[0:32, 128:256]]
                gre.append([_bf(v) for v in re])
                gri.append([_bf(jnp.stack([r_.reshape(4, 8, 128), i_.reshape(4, 8, 128)], axis=1).reshape(64, 128))
                            for r_, i_ in zip(re, im)])

            def tile(t):
                zs = [[_dot_nt(gri[c][e], rv[at(2 * j + c), 128 * t:128 * t + 128, 128 * e:128 * e + 128])
                       for e in range(2)] for c in range(2)]
                out = [z.reshape(4, 2, 16, 128) for z in comb(zs)]
                return [(z[:, 0].reshape(64, 128), z[:, 1].reshape(64, 128)) for z in out]

            if j < 7:
                odd = tile(1)
            nq = [jnp.concatenate([rn[at(2 * j + c), 0:8, :], jnp.zeros((120, 256), f32)], axis=0).astype(bf16)
                  for c in range(2)]
            nyq = comb([[_dot_nt(gre[c][e], nq[c][:, 128 * e:128 * e + 128]) for e in range(2)]
                        for c in range(2)])
            even = tile(0)
            if j == 7:
                odd = tile(1)
            for be in range(2):
                zr, zi = even[be]
                sh = pltpu.roll(jnp.where(first, nyq[be], zi), 1, axis=1)
                tiles = [jnp.where(ev, zr, sh), jnp.where(ev, sh, zr), odd[be][0], odd[be][1]]
                for t in range(4):
                    z32[t, pl.ds(512 * be + j, 64, stride=8), :] = tiles[t]

    def copy_wo(tok, step):
        tk = _rep(tok(0, 64, step), 4)
        wo32[...] = pltpu.bitcast(wo[...], u32) | jnp.concatenate([tk] * 4, axis=1)

    def xv_part(b, h0, h1):
        lhs = _bf(xe32[dyn(16 * b, 16), :])
        ys = []
        for h in range(h0, h1):
            ys.append(_dot(lhs, _bf(wsl[2 * H + h])))
            xq[b, 2 * H + h] = ys[-1].astype(bf16)
        return ys

    wait(grp[0])
    for c in range(4):
        relayout(0, r0=32 * c, r1=32 * c + 32)
    pack_xe(0)
    x_half(0, 0, 6)

    wait(grp[1])
    tok = tokens(x_half(0, 6, 8)[1:])
    relayout(0, tok, 0, 2, r0=128)
    pack_xe(1, tok)
    x_half(1, 0, 4)

    wait(grp[2])
    relayout(1, tokens(x_half(1, 4, 8)[1::2]), 0, 3)
    x_heads(8, 14)

    wait(grp[3])
    relayout(2, tokens(x_heads(14, 16)), 0, 3)
    tok = tokens(x_heads(16, 22))
    gather_x(0, 4, tok, 84)
    build_gs(tok, 5)

    wait(grp[4])
    relayout(3, tokens(x_heads(22, 24)), 0, 3)
    gather_x(4, 8, tokens(x_heads(24, 29)), 68)
    spectral_fwd(lambda: x_heads(29, 30))

    wait(grp[5])
    relayout(4, tokens(x_heads(30, 32)), 0, 3)
    tok = tokens(x_heads(32, 40))
    relayout(5, tok, 0, 14)
    spectral_mid(0, 0, 10, tok, 0, 50)
    spectral_mid(1, 0, 6, tokens(x_heads(40, 46)), 0, 54)

    wait(grp[6])
    relayout(6, tokens(x_heads(46, 48)), 0, 3)
    tok = tokens(x_heads(48, 56))
    relayout(7, tok, 0, 7)
    relayout(8, tok, 230, 7)
    spectral_mid(0, 10, 16, tok, 0, 72)
    spectral_mid(2, 0, 1, tok, 430, 72)
    tok = tokens(x_heads(56, 62) + x_heads(64, 64 + XVP // 2))
    relayout(9, tok, 0, 16)
    spectral_mid(1, 6, 16, tok, 0, 52)
    spectral_inv()

    wait(grp[7])
    st = x_heads(62, 64) + x_heads(64 + XVP // 2, 64 + XVP) + xv_part(0, XVP, 16)
    tok = tokens(st)
    relayout(10, tok, 0, 4)
    relayout(11, tok, 150, 4)
    copy_wo(tokens(st + xv_part(0, 16, XVL)), 5)
    wait(grp[8])

    r = lax.broadcasted_iota(jnp.int32, (R2, 128), 0)
    c = lax.broadcasted_iota(jnp.int32, (R2, 128), 1)

    def head_pos(i):
        head = jnp.where(i < 32, 0, jnp.where(i < 64, 1, jnp.where(i < 72, 0, jnp.where(i < R2, 1, 2))))
        pos = jnp.where(i < 32, i, jnp.where(i < 72, i - 32, i - 40))
        return head, pos

    rh, rpos = head_pos(r)
    ch, cpos = head_pos(c)
    same = (rh - ch) == 0
    ok = jnp.logical_and(same, jnp.logical_or(rpos < MEM, rpos >= cpos))
    fill = jnp.where(same, jnp.float32(-1e9 / SCALE), jnp.float32(-jnp.inf))

    def step(b, k, mem, filler):
        s = SPB * b + k
        second = k % 2 == 1
        mo = 48 if second else 32
        lhs = jnp.concatenate([mem, xb[s].astype(f32)], axis=0).astype(bf16)
        if not second:
            lhs48 = jnp.concatenate([lhs, _bf(xe32[dyn(4 * s, 8), :])], axis=0)
        acc = [None] * 4
        stream = []

        def proj(m, hp):
            y = jnp.concatenate([_dot(lhs, _bf(wsl[H * m + 2 * hp + hh])) for hh in range(2)], axis=0)
            qsc[m, hp] = y.astype(bf16)
            stream.append(y)

        def oper(m, hp):
            xs = [xq[b, H * m + 2 * hp + hh, XT * k:XT * k + XT, :] for hh in range(2)]
            if m > 0:
                xs.append(jnp.zeros((128 - R2, DH), bf16))
            return jnp.concatenate([qsc[m, hp]] + xs, axis=0)

        def do_qkp(hp):
            proj(0, hp)
            proj(1, hp)

        def do_v(hp):
            if second or 2 * hp < XVL:
                proj(2, hp)
                return
            ys = [_dot(lhs48, _bf(wsl[2 * H + 2 * hp + hh])) for hh in range(2)]
            y = jnp.concatenate([ys[0][0:32], ys[1][0:32]], axis=0)
            qsc[2, hp] = y.astype(bf16)
            for hh in range(2):
                xq[b, 2 * H + 2 * hp + hh, XT * k:XT * k + 2 * XT, :] = ys[hh][32:48].astype(bf16)
            stream.append(y)

        def do_qk(hp):
            ssc[hp] = jnp.where(ok, _dot_nt(oper(0, hp), oper(1, hp)), fill)
            stream.clear()

        def do_softmax(p0, p1):
            nt = 20 if p1 < NP else 5
            g = pltpu.bitcast(_rep(tokens(stream[0:3])(0, nt, 1), 40 // nt), f32)
            sc = ssc[p0:p1].reshape(4 * R2, 128) + g
            mx = jnp.max(sc, axis=-1, keepdims=True)
            e = jnp.exp2((sc - mx) * (SCALE * LOG2E))
            l = jnp.sum(e, axis=-1, keepdims=True)
            rl = pl.reciprocal(l, approx=True)
            rl = rl * (2.0 - l * rl)
            psc[p0:p1] = (e * rl).astype(bf16).reshape(4, R2, 128)

        def do_pv(hp):
            o2 = _dot(psc[hp], oper(2, hp))
            r0 = 40 if second else 32
            for hh in range(2):
                osc[2 * hp + hh, 0:32, :] = o2[32 * hh:32 * hh + 32].astype(bf16)
                osc[2 * hp + hh, r0:r0 + 8, :] = o2[64 + 8 * hh:72 + 8 * hh].astype(bf16)

        def do_o(p0, p1):
            ol = jnp.concatenate([osc[h, 0:mo, :] for h in range(2 * p0, 2 * p1)], axis=1)
            for n in range(4):
                y = _dot(ol, _bf(wo32[p0 * 128:p1 * 128, 128 * n:128 * n + 128]))
                acc[n] = y if acc[n] is None else acc[n] + y
                stream.append(y)

        def do_a3():
            zr = dyn(16 * s, 32)
            v0, v2, vc, vs = [_dot(_bf(z32[t, zr, :]), _bf(fi[:, 128 * t:128 * t + 128])) for t in range(4)]
            sp, sm = v0 + v2, v0 - v2
            first = _lane(2 * SEG) == 0
            al, be = vc + jnp.where(first, 0.0, vs), _mirror(vs - jnp.where(first, 0.0, vc))
            ya = jnp.concatenate([sp + al, sm + be, sp - al, sm - be], axis=1).astype(bf16)
            stage[pl.ds(s, 2), :, 0:D] = ya.reshape(2, SEG, D)

        for op in _SCHED:
            if op == 'a':
                if not second:
                    do_a3()
                continue
            p0, p1 = [int(v) for v in op[1:].split('-')]
            if op[0] == 'p':
                do_softmax(p0, p1)
            if op[0] == 'o':
                do_o(p0, p1)
            else:
                for hp in range(p0, p1):
                    {'k': do_qkp, 'v': do_v, 'q': do_qk, 'p': do_pv}[op[0]](hp)
        filler()
        return jnp.concatenate(acc, axis=1)

    nb = NSEG // SPB
    hv = [XVP, 10, 12, 16, XVL]

    def body(b, mem):
        nxt = jnp.minimum(b + 1, nb - 1)
        for k in range(0, SPB, 2):
            sa, sb = SPB * b + k, SPB * b + k + 1
            ya = step(b, k, mem, lambda: xv_part(nxt, hv[k], hv[k + 1]))
            stage[sa, 0:KEEP, D:2 * D] = ya[MEM:].astype(bf16)
            mem_b = ya[0:MEM].astype(bf16).astype(f32)
            yb = step(b, k + 1, mem_b, lambda: xv_part(nxt, hv[k + 1], hv[k + 2]))
            stage[sa, KEEP:SEG, D:2 * D] = yb[32:40].astype(bf16)
            stage[sb, :, D:2 * D] = jnp.concatenate([yb[MEM:32], yb[40:48]], axis=0).astype(bf16)
            mem = yb[0:MEM].astype(bf16).astype(f32)
            rows = pl.ds(sa, 2)
            cp(stage.at[rows], out_hbm.at[rows], _S_OUT).start()
        return mem

    lax.fori_loop(0, nb, body, m0[...].astype(f32))
    wait([cp(stage, out_hbm, _S_OUT)])


@jax.jit
def pallas_concat_heads__spectral_gfnet__memory_aug_recurrent_mem_tr__prompt_kernel(
    A_x: jax.Array,
    A_w_r: jax.Array,
    A_w_i: jax.Array,
    B_x: jax.Array,
    B_mem0: jax.Array,
    B_Wq: jax.Array,
    B_Wk: jax.Array,
    B_Wv: jax.Array,
    B_Wo: jax.Array,
    B_seg_len: jax.Array,
):
    del B_seg_len
    assert A_x.shape == (1, S, D) and B_x.shape == (1, S, D) and B_mem0.shape == (1, MEM, D)
    assert B_Wq.shape == (D, H, DH) and B_Wo.shape == (H, DH, D)
    fd, fi, sd = _dft_tables()
    vm = pltpu.VMEM
    scratch = [
        vm((NSEG, XT, D), bf16),
        vm((NSEG * XT // 2, D), u32),
        vm((2, S // 2, D), bf16),
        vm((4, 2, S // 4, 128), u32),
        vm((NC, 128, D), bf16),
        vm((12, D // 2, 2, 8, DH), bf16),
        vm((2, 2 * D, DH), u32),
        vm((2, 2 * D, DH), u32),
        vm((3 * H, D // 2, DH), u32),
        vm((NSEG // SPB, 3 * H, SPB * XT, DH), bf16),
        vm((64, 512), u32),
        vm((64, 512), u32),
        vm((NC, 64, 256), u32),
        vm((D // 2 + 1, S), bf16),
        vm((D // 2 + 1, S), bf16),
        vm((NC, 2, 272, 128), f32),
        vm((NC, 256, 256), bf16),
        vm((NC, 16, 256), f32),
        vm((4, S // 2, 128), u32),
        vm((H * DH, D), bf16),
        vm((H * DH // 2, D), u32),
        vm((NSEG, KEEP, D), bf16),
        vm((MEM, D), bf16),
        vm((NSEG, SEG, 2 * D), bf16),
        vm((8, 128), u32),
        vm((NP, R2, 128), bf16),
        vm((3, NP, 64, DH), bf16),
        vm((H, 48, DH), bf16),
        vm((NP, R2, 128), f32),
        vm((160, 128), f32),
        vm((8, NSEG * XT, DH), f32),
        pltpu.SemaphoreType.DMA((_NGRP + 1,)),
    ]
    w4 = lambda w: w.reshape(D // 2, 2, H, DH)
    out = pl.pallas_call(
        _kernel,
        out_shape=jax.ShapeDtypeStruct((NSEG, SEG, 2 * D), bf16),
        in_specs=[pl.BlockSpec(memory_space=pl.ANY)] * 12,
        out_specs=pl.BlockSpec(memory_space=pl.ANY),
        scratch_shapes=scratch,
        compiler_params=pltpu.CompilerParams(vmem_limit_bytes=110 * 1024 * 1024),
    )(A_x.reshape(2, S // 2, D), A_w_r.T, A_w_i.T, B_x.reshape(NSEG, SEG, D), B_mem0.reshape(MEM, D),
      w4(B_Wq), w4(B_Wk), w4(B_Wv), B_Wo.reshape(H * DH, D), fd, fi, sd)
    return out.reshape(1, S, 2 * D)
```

```python
import math

import numpy as np
import jax
import jax.numpy as jnp
from jax import lax
import jax.experimental.pallas as pl
import jax.experimental.pallas.tpu as pltpu

S, D = 2048, 512
H, DH = 32, 128
MEM, SEG = 8, 32
NSEG = S // SEG
NP = H // 2
XT = 8
KEEP = SEG - XT
R2 = 2 * (MEM + SEG)
SCALE = DH ** -0.5
LOG2E = 1.4426950408889634
NC = 16
SPB = 4
XVP = 6
XVL = 20

f32, bf16, u32 = jnp.float32, jnp.bfloat16, jnp.uint32
NT = (((1,), (1,)), ((), ()))


def _pack_rows(m):
    b = np.asarray(m, np.float32).astype(jnp.bfloat16).view(np.uint16).astype(np.uint32)
    return b[0::2, :] | (b[1::2, :] << 16)


def _dft_tables():
    k = np.arange(D // 2)[:, None]
    d = np.arange(D // 2)[None, :]
    ang = 2.0 * np.pi * ((k * d) % D) / D
    pm = np.cos(ang)
    qm = -np.sin(ang)
    qm[0] = (-1.0) ** np.arange(D // 2)
    qo = qm[:, :128].copy()
    qo[:, 0] = qm[:, 128]

    def inter(parts):
        c = parts[0].shape[1]
        return np.stack([p.reshape(-1, 8, c) for p in parts], axis=1).reshape(-1, c)

    f0 = inter([pm[0::4, :128], qm[0::4, :128]])
    f2 = inter([pm[2::4, :128], qm[2::4, :128]])
    fp = inter([pm[1::4, :128], pm[3::4, :128]])
    fq = inter([qo[1::4], qo[3::4]])
    fd = np.concatenate([np.concatenate([f0, f2, fp, fq], axis=1), np.zeros((16, 512))], axis=0)
    wgt = np.where(k == 0, 1.0, 2.0) / (S * D)
    pw, qw = wgt * pm, wgt * qm
    ii = np.arange(64)
    i0 = np.zeros((128, 128))
    i2 = np.zeros((128, 128))
    i0[2 * ii], i0[2 * ii + 1] = pw[0::4, :128], qw[0::4, :128]
    i2[2 * ii + 1], i2[(2 * ii + 2) % 128] = pw[2::4, :128], qw[2::4, :128]
    fi = np.concatenate([i0, i2, pw[1::2, :128], (wgt * qo)[1::2]], axis=1)
    k1 = np.arange(128)[None, :]
    mo = np.concatenate([ii[0::2], ii[1::2]])[:, None]
    ae = 2.0 * np.pi * ((NC * mo * k1) % S) / S
    at = 2.0 * np.pi * (np.arange(NC)[:, None] * k1) / S
    sd = np.concatenate([np.cos(ae), np.sin(ae), np.cos(at), np.sin(at)], axis=0).astype(np.float32)
    return _pack_rows(fd), _pack_rows(fi), sd


def _sadd(a, b):
    (sa, va), (sb, vb) = a, b
    if sa == sb:
        return (sa, va + vb)
    return (1, va - vb) if sa > 0 else (1, vb - va)


def _sneg(a):
    return (-a[0], a[1])


def _ssub(a, b):
    return _sadd(a, _sneg(b))


def _smul(a, c):
    return (a[0], a[1] * c) if c > 0 else (-a[0], a[1] * (-c))


def _cadd(a, b):
    return (_sadd(a[0], b[0]), _sadd(a[1], b[1]))


def _csub(a, b):
    return (_ssub(a[0], b[0]), _ssub(a[1], b[1]))


def _cmul_i(a, sgn):
    return (_sneg(a[1]), a[0]) if sgn > 0 else (a[1], _sneg(a[0]))


def _radix4(x, sgn):
    t0, t1 = _cadd(x[0], x[2]), _csub(x[0], x[2])
    t2, t3 = _cadd(x[1], x[3]), _cmul_i(_csub(x[1], x[3]), sgn)
    return [_cadd(t0, t2), _cadd(t1, t3), _csub(t0, t2), _csub(t1, t3)]


def _twiddle16(a, m, sgn):
    if m == 0:
        return a
    if m == 4:
        return _cmul_i(a, sgn)
    c, s = math.cos(2 * math.pi * m / 16), sgn * math.sin(2 * math.pi * m / 16)
    if m in (2, 6):
        if c * s > 0:
            return (_smul(_ssub(a[0], a[1]), c), _smul(_sadd(a[0], a[1]), c))
        return (_smul(_sadd(a[0], a[1]), c), _smul(_ssub(a[1], a[0]), c))
    return (_ssub(_smul(a[0], c), _smul(a[1], s)), _sadd(_smul(a[0], s), _smul(a[1], c)))


def _gate(x, t):
    if t is None:
        return x
    (sr, vr), (si, vi) = x
    return ((sr, vr + t), (si, vi + t))


def _fft16(x, sgn, g1=None, g2=None):
    g1 = g1 or [None] * 4
    g2 = g2 or [None] * 4
    a = [_radix4([_gate(x[n2], g1[n2])] + [x[4 * n1 + n2] for n1 in range(1, 4)], sgn) for n2 in range(4)]
    out = [None] * 16
    for k1 in range(4):
        y = _radix4([_gate(a[0][k1], g2[k1])]
                    + [_twiddle16(a[n2][k1], n2 * k1, sgn) for n2 in range(1, 4)], sgn)
        for k2 in range(4):
            out[k1 + 4 * k2] = y[k2]
    return out


def _val(a):
    return a[1] if a[0] > 0 else -a[1]


def _lo(u):
    return pltpu.bitcast(u << 16, f32)


def _hi(u):
    return pltpu.bitcast(u & jnp.uint32(0xFFFF0000), f32)


def _pack2(a, b):
    lo = pltpu.bitcast(a.astype(bf16).astype(f32), u32) >> 16
    return lo | pltpu.bitcast(b.astype(bf16).astype(f32), u32)


def _bf(u):
    return pltpu.bitcast(u, bf16)


def _dot(a, b):
    return jnp.dot(a, b, preferred_element_type=f32)


def _dot_nt(a, b):
    return lax.dot_general(a, b, NT, preferred_element_type=f32)


def _lane(rows):
    return lax.broadcasted_iota(jnp.int32, (rows, 128), 1)


def _mirror(v):
    return jnp.take_along_axis(v, (128 - _lane(v.shape[0])) & 127, axis=1)


def _rep(t, n):
    k = t.shape[0] // 8
    return jnp.broadcast_to(t.reshape(k, 1, 8, 128), (k, n, 8, 128)).reshape(k * n * 8, 128)


_NGRP = 9
_S_OUT = _NGRP

_SCHED = ('a k0-4 v0-4 q0-4 k4-8 v4-8 p0-4 q4-8 k8-12 v8-12 p4-8 q8-12 k12-16 v12-16 p8-12 q12-16 '
          'o0-4 o4-9 p12-16 o9-12 o12-16').split()


def _kernel(xa_hbm, wr_hbm, wi_hbm, xb_hbm, m0_hbm, wq_hbm, wk_hbm, wv_hbm, wo_hbm,
            fd_hbm, fi_hbm, sd_hbm, out_hbm,
            xe, xe32, xa, xst, xg, wst, wca, wcb, wsl, xq, fd, fi, gs, wr, wi, tsc, rv, ff,
            z32, wo, wo32, xb, m0, stage, zq, psc, qsc, osc, ssc, sd, part, sems):
    w_hbms = (wq_hbm, wk_hbm, wv_hbm)

    def dyn(start, size):
        return pl.ds(start, size) if isinstance(start, int) else pl.ds(pl.multiple_of(start, size), size)

    def cp(src, dst, sem):
        return pltpu.make_async_copy(src, dst, sems.at[sem])

    def cp_w(m, g, sem):
        return cp(w_hbms[m].at[:, :, pl.ds(8 * g, 8), :], wst.at[4 * m + g], sem)

    def cp_xa(c0, c1, sem):
        rows = pl.ds(128 * c0, 128 * (c1 - c0))
        return cp(xa_hbm.at[:, rows, :], xa.at[:, rows, :], sem)

    def cp_f(src, dst, part, sem):
        rows = pl.ds(0, 160) if part == 0 else pl.ds(160, D // 2 + 1 - 160)
        return cp(src.at[rows, :], dst.at[rows, :], sem)

    def cp_half(k, sem):
        rows, cols = pl.ds(128 * k, 128), pl.ds(256 * k, 256)
        return [cp(wq_hbm.at[rows, :, pl.ds(0, 8), :], wst.at[0, rows], sem),
                cp(xb_hbm.at[:, pl.ds(KEEP, XT), cols], xe.at[:, :, cols], sem)]

    grp = [
        cp_half(0, 0),
        cp_half(1, 1) + [cp(fd_hbm.at[pl.ds(64, 8), pl.ds(0, 128)], zq, 1)],
        [cp_w(0, 1, 2)],
        [cp(sd_hbm, sd, 3), cp_w(0, 2, 3), cp_xa(0, 4, 3)],
        [cp_w(0, 3, 4), cp_xa(4, 8, 4), cp(fd_hbm.at[pl.ds(0, 64), :], fd, 4)],
        [cp_w(1, 0, 5), cp_f(wr_hbm, wr, 0, 5), cp_f(wi_hbm, wi, 0, 5), cp_w(1, 1, 5)],
        [cp_f(wr_hbm, wr, 1, 6), cp_f(wi_hbm, wi, 1, 6),
         cp_w(1, 2, 6), cp_w(1, 3, 6), cp_w(2, 0, 6), cp_w(2, 1, 6)],
        [cp_w(2, 2, 7), cp_w(2, 3, 7), cp(wo_hbm, wo, 7)],
        [cp(fi_hbm, fi, 8), cp(m0_hbm, m0, 8), cp(xb_hbm.at[:, pl.ds(0, KEEP), :], xb, 8)],
    ]
    for g_ in grp:
        for c_ in g_:
            c_.start()

    def wait(copies):
        for c_ in copies:
            c_.wait()

    def tokens(stream):
        ys = jnp.concatenate(stream, axis=0)
        n = ys.shape[0] // 8

        def tok(start, count, step):
            assert start + (count - 1) * step < n, (start, count, step, n)
            first = min(start, n - count * step)
            y = ys[8 * first:8 * (first + count * step)].reshape(count, step, 8, 128)[:, start - first]
            return (pltpu.bitcast(y, u32) & zq[...][None]).reshape(count * 8, 128)
        return tok

    def opaque():
        z0 = zq[0, 0].astype(jnp.int32)
        idx = [jnp.clip(z0 + a, 0, NC - 1) for a in range(NC)]
        return lambda a: idx[a]

    def relayout(i, tok=None, start=0, step=1, r0=0, r1=D // 2):
        wc = (wca, wcb)[i % 2]
        n = r1 - r0
        m_lo, m_hi = jnp.uint32(0xFFFF), jnp.uint32(0xFFFF0000)
        if tok is not None:
            t1 = tok(start, n // 8, step)
            m_lo, m_hi = _rep(t1 | m_lo, 4), _rep(t1 | m_hi, 4)
            t2 = tok(start + 12, n // 8, step)
        ev = pltpu.bitcast(wst[i, r0:r1, 0].reshape(8 * n, DH), u32)
        od = pltpu.bitcast(wst[i, r0:r1, 1].reshape(8 * n, DH), u32)
        wc[0, 4 * r0:4 * r1, :] = (ev & m_lo) | (od << 16)
        wc[1, 4 * r0:4 * r1, :] = (ev >> 16) | (od & m_hi)
        for j in range(4):
            for p in range(2):
                v = wc[p, pl.ds(4 * r0 + j, n, stride=4), :]
                wsl[8 * i + 2 * j + p, r0:r1, :] = v if tok is None else v | t2

    def x_half(k, h0, h1):
        lhs = _bf(xe32[:, 256 * k:256 * k + 256])
        ys = []
        for h in range(h0, h1):
            ys.append(_dot(lhs, _bf(wsl[h, 128 * k:128 * k + 128, :])))
            if k == 0:
                part[h] = ys[-1]
            else:
                xq[:, h] = (ys[-1] + part[h]).astype(bf16).reshape(NSEG // SPB, SPB * XT, DH)
        return ys

    def pack_xe(k, tok=None):
        v = pltpu.bitcast(xe[:, :, 256 * k:256 * k + 256].reshape(NSEG * XT, 256), u32)
        if tok is not None:
            v = v | jnp.concatenate([tok(0, 32, 1)] * 2, axis=1)
        xe32[:, 256 * k:256 * k + 256] = v

    def x_heads(h0, h1):
        lhs = _bf(xe32[...])
        ys = []
        for h in range(h0, h1):
            ys.append(_dot(lhs, _bf(wsl[h])))
            xq[:, h] = ys[-1].astype(bf16).reshape(NSEG // SPB, SPB * XT, DH)
        return ys

    def gather_x(c0, c1, tok, per):
        nc = c1 - c0
        first = _lane(8 * nc) == 0
        for hf in range(2):
            tk = jnp.stack([tok((4 * hf + q) * per // 24, nc, per).reshape(nc, 8, 128) for q in range(4)], axis=1)
            tk = _rep(tk.reshape(32 * nc, 128), 2)
            u = pltpu.bitcast(xa[hf, 128 * c0:128 * c1, :], u32)
            for a in range(4):
                xst[a, hf, 64 * c0:64 * c1, :] = u[:, 128 * a:128 * a + 128] | tk
        for j in range(8):
            for p, part in enumerate((_lo, _hi)):
                tk = pltpu.bitcast(tok((8 + 2 * j + p) * per // 24, nc, per), f32)
                xl, xh = [[part(xst[a, hf, pl.ds(64 * c0 + j, 8 * nc, stride=8), :]) for a in range(4)]
                          for hf in range(2)]
                xl[0], xl[1] = xl[0] + tk, xl[1] + tk
                for hf in range(2):
                    x0, x1, x2, x3 = [(l + h if hf == 0 else l - h) for l, h in zip(xl, xh)]
                    s02, s13 = x0 + x2, x1 + x3
                    al, rb = x0 - x2, _mirror(x1 - x3)
                    v = jnp.concatenate([s02 + s13, s02 - s13, al - jnp.where(first, 0.0, rb),
                                         jnp.where(first, 0.0, al) + rb], axis=1)
                    xg[2 * j + p, 64 * hf + 8 * c0:64 * hf + 8 * c1, :] = v.astype(bf16)

    def build_gs(tok, step):
        tk = pltpu.bitcast(tok(0, 4 * NC, step), f32)
        ct, st = [jnp.concatenate([jnp.broadcast_to(sd[r0 + a:r0 + a + 1, :], (32, 128)) for a in range(NC)],
                                  axis=0) + tk for r0 in (128, 144)]
        ce, se = [[jnp.concatenate([sd[r0 + 32 * p:r0 + 32 * p + 32, :]] * NC, axis=0) for p in range(2)]
                  for r0 in (0, 64)]
        co = _pack2(*[ce[p] * ct - se[p] * st for p in range(2)])
        si = _pack2(*[se[p] * ct + ce[p] * st for p in range(2)])
        cr = pltpu.roll(co, 1, axis=1)
        ns = pltpu.roll(si, 1, axis=1) ^ jnp.uint32(0x80008000)
        ev = (_lane(32 * NC) & 1) == 0
        gs[:, 0:32, :] = jnp.concatenate(
            [jnp.where(ev, co, ns), jnp.where(ev, cr, si)], axis=1).reshape(NC, 32, 256)
        gs[:, 32:64, :] = jnp.concatenate(
            [jnp.where(ev, si, cr), jnp.where(ev, ns, co)], axis=1).reshape(NC, 32, 256)

    def d_fwd(a, at):
        y = [_dot_nt(_bf(fd[:, 128 * t:128 * t + 128]), xg[at(a), :, 128 * t:128 * t + 128]) for t in range(4)]
        ye = _pack2(y[0], y[1]).reshape(8, 2, 8, 128)
        po, qo = [y_.reshape(8, 2, 8, 128) for y_ in y[2:4]]
        p = jnp.concatenate([ye[:, 0], _pack2(po[:, 0], po[:, 1])], axis=0).reshape(128, 128)
        q = jnp.concatenate([ye[:, 1], _pack2(qo[:, 0], qo[:, 1])], axis=0).reshape(128, 128)
        q = pltpu.roll(q, 64, axis=1)
        lo = _lane(128) < 64
        return _bf(jnp.where(lo, p, q)), _bf(jnp.where(lo, q, p))

    def s_fwd(a, ls, at):
        o0 = _dot(ls[0], _bf(gs[at(a), :, 0:128]))
        o1 = _dot(ls[1], _bf(gs[at(a), :, 128:256]))
        ev = (_lane(256) & 1) == 0
        tsc[a, 0] = jnp.where(ev, o0, o1)
        tsc[a, 1] = jnp.where(ev, o1, o0)
        return o1

    def spectral_fwd(filler):
        at = opaque()
        ls = [d_fwd(a, at) for a in range(4)]
        stream = []
        for a in range(0, NC, 2):
            if a + 4 < NC:
                ls += [d_fwd(a + 4, at), d_fwd(a + 5, at)]
            if a == NC - 2:
                filler()
            s_fwd(a, ls[a], at)
            stream.append(s_fwd(a + 1, ls[a + 1], at))
        return stream

    rel = [0, 1, 2, 3, 4, 7, 10, 13, 16, 17.5, 19, 20.5]

    def negated(z):
        first = _lane(8) == 0
        return [jnp.where(first, z[(NC - k2) % NC], _mirror(z[NC - 1 - k2])) for k2 in range(NC)]

    def dc_filter(tok, start, step):
        tk = pltpu.bitcast(tok(start, NC, step), f32)
        row0 = lax.broadcasted_iota(jnp.int32, (8, 128), 0) == 0
        for c, (w, sg) in enumerate(((wr, 1.0), (wi, -1.0))):
            base = [_lo(pltpu.bitcast(w[0:16, 128 * k2:128 * k2 + 128], u32)) + tk[8 * k2:8 * k2 + 8]
                    for k2 in range(NC)]
            nyq = [w[256:257, 128 * k2:128 * k2 + 128].astype(f32) for k2 in range(NC)]
            pl_ = [b_ + n_ for b_, n_ in zip(base, nyq)]
            mi_ = [b_ - n_ for b_, n_ in zip(base, nyq)]
            f1 = [jnp.where(row0, 0.25 * (z + sg * zn), b_) for z, zn, b_ in zip(pl_, negated(pl_), base)]
            f2 = [jnp.where(row0, 0.25 * (z + sg * zn), 0.0) for z, zn in zip(mi_, negated(mi_))]
            ff[c] = jnp.concatenate(f1, axis=0)
            ff[2 + c] = jnp.concatenate(f2, axis=0)

    def spectral_mid(p, v0, v1, tok, start, per):
        nu = v1 - v0
        at = opaque()
        gate = lambda r: pltpu.bitcast(tok(start + int((r + 4) * per / 24), nu, per), f32)
        gates = [gate(r) for r in rel]
        pre = [gate(r - 4) for r in rel[0:4]]
        r0, r1 = 128 * p + 8 * v0, 128 * p + 8 * v1
        t = [((1, tsc[at(a), 0, r0:r1, :]), (1, pltpu.roll(tsc[at(a), 1, r0:r1, :] + pre[a % 4], 127, axis=1)))
             for a in range(NC)]
        x = _fft16(t, -1, gates[0:4], gates[4:8])
        y = []
        if r0 == 0:
            assert nu == 1
            xr, xi = [_val(v[0]) for v in x], [_val(v[1]) for v in x]
            for k2, (mr, mi) in enumerate(zip(negated(xr), negated(xi))):
                f1r, f1i, f2r, f2i = [ff[c, 8 * k2:8 * k2 + 8, :] for c in range(4)]
                y.append(((1, (xr[k2] * f1r - xi[k2] * f1i) + (mr * f2r + mi * f2i)),
                          (1, (xr[k2] * f1i + xi[k2] * f1r) + (mr * f2i - mi * f2r))))
        else:
            for k2 in range(NC):
                fa, fb = [(_lo, _hi)[p](pltpu.bitcast(w[16 * v0:16 * v1, 128 * k2:128 * k2 + 128], u32))
                          for w in (wr, wi)]
                (sr, xr), (si, xi) = x[k2]
                y.append((_ssub((sr, xr * fa), (si, xi * fb)), _sadd((sr, xr * fb), (si, xi * fa))))
        ev = (_lane(8 * nu) & 1) == 0
        u = _fft16(y, 1, None, gates[8:12])
        for k1 in range(4):
            ui = jnp.stack([_val(u[k1 + 4 * k2][1]).reshape(nu, 8, 128) for k2 in range(4)], axis=1)
            us4 = pltpu.roll(ui.reshape(32 * nu, 128), 1, axis=1).reshape(nu, 4, 8, 128)
            for k2 in range(4):
                ur, us = _val(u[k1 + 4 * k2][0]), us4[:, k2].reshape(8 * nu, 128)
                v01 = jnp.concatenate([jnp.where(ev, ur, us), jnp.where(ev, us, ur)], axis=1)
                rv[k1 + 4 * k2, r0:r1, :] = v01.astype(bf16)

    def spectral_inv():
        ev = (_lane(64) & 1) == 0
        at = opaque()
        for j in range(8):
            gri = []
            for a in (2 * j, 2 * j + 1):
                g = gs[at(a)]
                re = [g[0:32, 0:128], g[32:64, 128:256]]
                im = [g[32:64, 0:128], g[0:32, 128:256]]
                gri.append([_bf(jnp.stack([r_.reshape(4, 8, 128), i_.reshape(4, 8, 128)], axis=1).reshape(64, 128))
                            for r_, i_ in zip(re, im)])

            def tile(t):
                zs = [[_dot_nt(gri[c][e], rv[at(2 * j + c), 128 * t:128 * t + 128, 128 * e:128 * e + 128])
                       for e in range(2)] for c in range(2)]
                out = [_pack2(zs[0][0] + zs[0][1], zs[1][0] + zs[1][1]).reshape(4, 2, 16, 128),
                       _pack2(zs[0][0] - zs[0][1], zs[1][0] - zs[1][1]).reshape(4, 2, 16, 128)]
                return [(z[:, 0].reshape(64, 128), z[:, 1].reshape(64, 128)) for z in out]

            even = tile(0)
            odd = tile(1)
            for be in range(2):
                zr, zi = even[be]
                sh = pltpu.roll(zi, 1, axis=1)
                tiles = [jnp.where(ev, zr, sh), jnp.where(ev, sh, zr), odd[be][0], odd[be][1]]
                for t in range(4):
                    z32[t, pl.ds(512 * be + j, 64, stride=8), :] = tiles[t]

    def copy_wo(tok, step):
        tk = _rep(tok(0, 64, step), 4)
        wo32[...] = pltpu.bitcast(wo[...], u32) | jnp.concatenate([tk] * 4, axis=1)

    def xv_part(b, h0, h1):
        lhs = _bf(xe32[dyn(16 * b, 16), :])
        ys = []
        for h in range(h0, h1):
            ys.append(_dot(lhs, _bf(wsl[2 * H + h])))
            xq[b, 2 * H + h] = ys[-1].astype(bf16)
        return ys

    wait(grp[0])
    for c in range(4):
        relayout(0, r0=32 * c, r1=32 * c + 32)
    pack_xe(0)
    x_half(0, 0, 6)

    wait(grp[1])
    tok = tokens(x_half(0, 6, 8)[1:])
    relayout(0, tok, 0, 2, r0=128)
    pack_xe(1, tok)
    x_half(1, 0, 4)

    wait(grp[2])
    relayout(1, tokens(x_half(1, 4, 8)[1::2]), 0, 3)
    x_heads(8, 14)

    wait(grp[3])
    relayout(2, tokens(x_heads(14, 16)), 0, 3)
    tok = tokens(x_heads(16, 22))
    gather_x(0, 4, tok, 84)
    build_gs(tok, 5)

    wait(grp[4])
    relayout(3, tokens(x_heads(22, 24)), 0, 3)
    gather_x(4, 8, tokens(x_heads(24, 29)), 68)
    spectral_fwd(lambda: x_heads(29, 30))

    wait(grp[5])
    relayout(4, tokens(x_heads(30, 32)), 0, 3)
    tok = tokens(x_heads(32, 40))
    relayout(5, tok, 0, 14)
    spectral_mid(0, 1, 10, tok, 0, 56)
    spectral_mid(1, 0, 6, tokens(x_heads(40, 46)), 0, 54)

    wait(grp[6])
    relayout(6, tokens(x_heads(46, 48)), 0, 3)
    tok = tokens(x_heads(48, 56))
    relayout(7, tok, 0, 7)
    relayout(8, tok, 230, 7)
    dc_filter(tok, 0, 20)
    spectral_mid(0, 10, 16, tok, 0, 66)
    spectral_mid(0, 0, 1, tok, 400, 100)
    tok = tokens(x_heads(56, 62) + x_heads(64, 64 + XVP // 2))
    relayout(9, tok, 0, 16)
    spectral_mid(1, 6, 16, tok, 0, 52)
    spectral_inv()

    wait(grp[7])
    st = x_heads(62, 64) + x_heads(64 + XVP // 2, 64 + XVP) + xv_part(0, XVP, 16)
    tok = tokens(st)
    relayout(10, tok, 0, 4)
    relayout(11, tok, 150, 4)
    copy_wo(tokens(st + xv_part(0, 16, XVL)), 5)
    wait(grp[8])

    r = lax.broadcasted_iota(jnp.int32, (R2, 128), 0)
    c = lax.broadcasted_iota(jnp.int32, (R2, 128), 1)

    def head_pos(i):
        head = jnp.where(i < 32, 0, jnp.where(i < 64, 1, jnp.where(i < 72, 0, jnp.where(i < R2, 1, 2))))
        pos = jnp.where(i < 32, i, jnp.where(i < 72, i - 32, i - 40))
        return head, pos

    rh, rpos = head_pos(r)
    ch, cpos = head_pos(c)
    same = (rh - ch) == 0
    ok = jnp.logical_and(same, jnp.logical_or(rpos < MEM, rpos >= cpos))
    fill = jnp.where(same, jnp.float32(-1e9 / SCALE), jnp.float32(-jnp.inf))

    def step(b, k, mem, filler):
        s = SPB * b + k
        second = k % 2 == 1
        mo = 48 if second else 32
        lhs = jnp.concatenate([mem, xb[s].astype(f32)], axis=0).astype(bf16)
        if not second:
            lhs48 = jnp.concatenate([lhs, _bf(xe32[dyn(4 * s, 8), :])], axis=0)
        acc = [None] * 4
        stream = []

        def proj(m, hp):
            y = jnp.concatenate([_dot(lhs, _bf(wsl[H * m + 2 * hp + hh])) for hh in range(2)], axis=0)
            qsc[m, hp] = y.astype(bf16)
            stream.append(y)

        def oper(m, hp):
            xs = [xq[b, H * m + 2 * hp + hh, XT * k:XT * k + XT, :] for hh in range(2)]
            if m > 0:
                xs.append(jnp.zeros((128 - R2, DH), bf16))
            return jnp.concatenate([qsc[m, hp]] + xs, axis=0)

        def do_qkp(hp):
            proj(0, hp)
            proj(1, hp)

        def do_v(hp):
            if second or 2 * hp < XVL:
                proj(2, hp)
                return
            ys = [_dot(lhs48, _bf(wsl[2 * H + 2 * hp + hh])) for hh in range(2)]
            y = jnp.concatenate([ys[0][0:32], ys[1][0:32]], axis=0)
            qsc[2, hp] = y.astype(bf16)
            for hh in range(2):
                xq[b, 2 * H + 2 * hp + hh, XT * k:XT * k + 2 * XT, :] = ys[hh][32:48].astype(bf16)
            stream.append(y)

        def do_qk(hp):
            ssc[hp] = jnp.where(ok, _dot_nt(oper(0, hp), oper(1, hp)), fill)
            stream.clear()

        def do_softmax(p0, p1):
            nt = 20 if p1 < NP else 5
            g = pltpu.bitcast(_rep(tokens(stream[0:3])(0, nt, 1), 40 // nt), f32)
            sc = ssc[p0:p1].reshape(4 * R2, 128) + g
            mx = jnp.max(sc, axis=-1, keepdims=True)
            e = jnp.exp2((sc - mx) * (SCALE * LOG2E))
            l = jnp.sum(e, axis=-1, keepdims=True)
            rl = pl.reciprocal(l, approx=True)
            rl = rl * (2.0 - l * rl)
            psc[p0:p1] = (e * rl).astype(bf16).reshape(4, R2, 128)

        def do_pv(hp):
            o2 = _dot(psc[hp], oper(2, hp))
            r0 = 40 if second else 32
            for hh in range(2):
                osc[2 * hp + hh, 0:32, :] = o2[32 * hh:32 * hh + 32].astype(bf16)
                osc[2 * hp + hh, r0:r0 + 8, :] = o2[64 + 8 * hh:72 + 8 * hh].astype(bf16)

        def do_o(p0, p1):
            ol = jnp.concatenate([osc[h, 0:mo, :] for h in range(2 * p0, 2 * p1)], axis=1)
            for n in range(4):
                y = _dot(ol, _bf(wo32[p0 * 128:p1 * 128, 128 * n:128 * n + 128]))
                acc[n] = y if acc[n] is None else acc[n] + y
                stream.append(y)

        def do_a3():
            zr = dyn(16 * s, 32)
            v0, v2, vc, vs = [_dot(_bf(z32[t, zr, :]), _bf(fi[:, 128 * t:128 * t + 128])) for t in range(4)]
            sp, sm = v0 + v2, v0 - v2
            first = _lane(2 * SEG) == 0
            al, be = vc + jnp.where(first, 0.0, vs), _mirror(vs - jnp.where(first, 0.0, vc))
            ya = jnp.concatenate([sp + al, sm + be, sp - al, sm - be], axis=1).astype(bf16)
            stage[pl.ds(s, 2), :, 0:D] = ya.reshape(2, SEG, D)

        for op in _SCHED:
            if op == 'a':
                if not second:
                    do_a3()
                continue
            p0, p1 = [int(v) for v in op[1:].split('-')]
            if op[0] == 'p':
                do_softmax(p0, p1)
            if op[0] == 'o':
                do_o(p0, p1)
            else:
                for hp in range(p0, p1):
                    {'k': do_qkp, 'v': do_v, 'q': do_qk, 'p': do_pv}[op[0]](hp)
        filler()
        return jnp.concatenate(acc, axis=1)

    nb = NSEG // SPB
    hv = [XVP, 10, 12, 16, XVL]

    def body(b, mem):
        nxt = jnp.minimum(b + 1, nb - 1)
        for k in range(0, SPB, 2):
            sa, sb = SPB * b + k, SPB * b + k + 1
            ya = step(b, k, mem, lambda: xv_part(nxt, hv[k], hv[k + 1]))
            stage[sa, 0:KEEP, D:2 * D] = ya[MEM:].astype(bf16)
            mem_b = ya[0:MEM].astype(bf16).astype(f32)
            yb = step(b, k + 1, mem_b, lambda: xv_part(nxt, hv[k + 1], hv[k + 2]))
            stage[sa, KEEP:SEG, D:2 * D] = yb[32:40].astype(bf16)
            stage[sb, :, D:2 * D] = jnp.concatenate([yb[MEM:32], yb[40:48]], axis=0).astype(bf16)
            mem = yb[0:MEM].astype(bf16).astype(f32)
            rows = pl.ds(sa, 2)
            cp(stage.at[rows], out_hbm.at[rows], _S_OUT).start()
        return mem

    lax.fori_loop(0, nb, body, m0[...].astype(f32))
    wait([cp(stage, out_hbm, _S_OUT)])


@jax.jit
def pallas_concat_heads__spectral_gfnet__memory_aug_recurrent_mem_tr__prompt_kernel(
    A_x: jax.Array,
    A_w_r: jax.Array,
    A_w_i: jax.Array,
    B_x: jax.Array,
    B_mem0: jax.Array,
    B_Wq: jax.Array,
    B_Wk: jax.Array,
    B_Wv: jax.Array,
    B_Wo: jax.Array,
    B_seg_len: jax.Array,
):
    del B_seg_len
    assert A_x.shape == (1, S, D) and B_x.shape == (1, S, D) and B_mem0.shape == (1, MEM, D)
    assert B_Wq.shape == (D, H, DH) and B_Wo.shape == (H, DH, D)
    fd, fi, sd = _dft_tables()
    vm = pltpu.VMEM
    scratch = [
        vm((NSEG, XT, D), bf16),
        vm((NSEG * XT // 2, D), u32),
        vm((2, S // 2, D), bf16),
        vm((4, 2, S // 4, 128), u32),
        vm((NC, 128, D), bf16),
        vm((12, D // 2, 2, 8, DH), bf16),
        vm((2, 2 * D, DH), u32),
        vm((2, 2 * D, DH), u32),
        vm((3 * H, D // 2, DH), u32),
        vm((NSEG // SPB, 3 * H, SPB * XT, DH), bf16),
        vm((64, 512), u32),
        vm((64, 512), u32),
        vm((NC, 64, 256), u32),
        vm((D // 2 + 1, S), bf16),
        vm((D // 2 + 1, S), bf16),
        vm((NC, 2, 256, 128), f32),
        vm((NC, 256, 256), bf16),
        vm((4, NC * 8, 128), f32),
        vm((4, S // 2, 128), u32),
        vm((H * DH, D), bf16),
        vm((H * DH // 2, D), u32),
        vm((NSEG, KEEP, D), bf16),
        vm((MEM, D), bf16),
        vm((NSEG, SEG, 2 * D), bf16),
        vm((8, 128), u32),
        vm((NP, R2, 128), bf16),
        vm((3, NP, 64, DH), bf16),
        vm((H, 48, DH), bf16),
        vm((NP, R2, 128), f32),
        vm((160, 128), f32),
        vm((8, NSEG * XT, DH), f32),
        pltpu.SemaphoreType.DMA((_NGRP + 1,)),
    ]
    w4 = lambda w: w.reshape(D // 2, 2, H, DH)
    out = pl.pallas_call(
        _kernel,
        out_shape=jax.ShapeDtypeStruct((NSEG, SEG, 2 * D), bf16),
        in_specs=[pl.BlockSpec(memory_space=pl.ANY)] * 12,
        out_specs=pl.BlockSpec(memory_space=pl.ANY),
        scratch_shapes=scratch,
        compiler_params=pltpu.CompilerParams(vmem_limit_bytes=110 * 1024 * 1024),
    )(A_x.reshape(2, S // 2, D), A_w_r.T, A_w_i.T, B_x.reshape(NSEG, SEG, D), B_mem0.reshape(MEM, D),
      w4(B_Wq), w4(B_Wk), w4(B_Wv), B_Wo.reshape(H * DH, D), fd, fi, sd)
    return out.reshape(1, S, 2 * D)
```

```python
import math

import numpy as np
import jax
import jax.numpy as jnp
from jax import lax
import jax.experimental.pallas as pl
import jax.experimental.pallas.tpu as pltpu

S, D = 2048, 512
H, DH = 32, 128
MEM, SEG = 8, 32
NSEG = S // SEG
NP = H // 2
XT = 8
KEEP = SEG - XT
R2 = 2 * (MEM + SEG)
SCALE = DH ** -0.5
LOG2E = 1.4426950408889634
NC = 16
SPB = 4
XVP = 6
XVL = 20

f32, bf16, u32 = jnp.float32, jnp.bfloat16, jnp.uint32
NT = (((1,), (1,)), ((), ()))


def _pack_rows(m):
    b = np.asarray(m, np.float32).astype(jnp.bfloat16).view(np.uint16).astype(np.uint32)
    return b[0::2, :] | (b[1::2, :] << 16)


def _dft_tables():
    k = np.arange(D // 2)[:, None]
    d = np.arange(D // 2)[None, :]
    ang = 2.0 * np.pi * ((k * d) % D) / D
    pm = np.cos(ang)
    qm = -np.sin(ang)
    qm[0] = (-1.0) ** np.arange(D // 2)
    qo = qm[:, :128].copy()
    qo[:, 0] = qm[:, 128]

    def inter(parts):
        c = parts[0].shape[1]
        return np.stack([p.reshape(-1, 8, c) for p in parts], axis=1).reshape(-1, c)

    f0 = inter([pm[0::4, :128], qm[0::4, :128]])
    f2 = inter([pm[2::4, :128], qm[2::4, :128]])
    fp = inter([pm[1::4, :128], pm[3::4, :128]])
    fq = inter([qo[1::4], qo[3::4]])
    fd = np.concatenate([f0, f2, fp, fq], axis=1)
    wgt = np.where(k == 0, 1.0, 2.0) / (S * D)
    pw, qw = wgt * pm, wgt * qm
    ii = np.arange(64)
    i0 = np.zeros((128, 128))
    i2 = np.zeros((128, 128))
    i0[2 * ii], i0[2 * ii + 1] = pw[0::4, :128], qw[0::4, :128]
    i2[2 * ii + 1], i2[(2 * ii + 2) % 128] = pw[2::4, :128], qw[2::4, :128]
    fi = np.concatenate([i0, i2, pw[1::2, :128], (wgt * qo)[1::2]], axis=1)
    k1 = np.arange(128)[None, :]
    mo = np.concatenate([ii[0::2], ii[1::2]])[:, None]
    ae = 2.0 * np.pi * ((NC * mo * k1) % S) / S
    at = 2.0 * np.pi * (np.arange(NC)[:, None] * k1) / S
    side = lambda c, s_: np.concatenate(np.split(c, 2) + np.split(s_, 2), axis=1)
    sd = np.concatenate([side(np.cos(ae), np.sin(ae)), side(np.cos(at), np.sin(at))]).astype(np.float32)
    return np.concatenate([_pack_rows(fd), sd.view(np.uint32)], axis=0), _pack_rows(fi)


def _sadd(a, b):
    (sa, va), (sb, vb) = a, b
    if sa == sb:
        return (sa, va + vb)
    return (1, va - vb) if sa > 0 else (1, vb - va)


def _sneg(a):
    return (-a[0], a[1])


def _ssub(a, b):
    return _sadd(a, _sneg(b))


def _smul(a, c):
    return (a[0], a[1] * c) if c > 0 else (-a[0], a[1] * (-c))


def _cadd(a, b):
    return (_sadd(a[0], b[0]), _sadd(a[1], b[1]))


def _csub(a, b):
    return (_ssub(a[0], b[0]), _ssub(a[1], b[1]))


def _cmul_i(a, sgn):
    return (_sneg(a[1]), a[0]) if sgn > 0 else (a[1], _sneg(a[0]))


def _radix4(x, sgn):
    t0, t1 = _cadd(x[0], x[2]), _csub(x[0], x[2])
    t2, t3 = _cadd(x[1], x[3]), _cmul_i(_csub(x[1], x[3]), sgn)
    return [_cadd(t0, t2), _cadd(t1, t3), _csub(t0, t2), _csub(t1, t3)]


def _twiddle16(a, m, sgn):
    if m == 0:
        return a
    if m == 4:
        return _cmul_i(a, sgn)
    c, s = math.cos(2 * math.pi * m / 16), sgn * math.sin(2 * math.pi * m / 16)
    if m in (2, 6):
        if c * s > 0:
            return (_smul(_ssub(a[0], a[1]), c), _smul(_sadd(a[0], a[1]), c))
        return (_smul(_sadd(a[0], a[1]), c), _smul(_ssub(a[1], a[0]), c))
    return (_ssub(_smul(a[0], c), _smul(a[1], s)), _sadd(_smul(a[0], s), _smul(a[1], c)))


def _gate(x, t):
    if t is None:
        return x
    (sr, vr), (si, vi) = x
    return ((sr, vr + t), (si, vi + t))


def _fft16(x, sgn, g1=None, g2=None):
    g1 = g1 or [None] * 4
    g2 = g2 or [None] * 4
    a = [_radix4([_gate(x[n2], g1[n2])] + [x[4 * n1 + n2] for n1 in range(1, 4)], sgn) for n2 in range(4)]
    out = [None] * 16
    for k1 in range(4):
        y = _radix4([_gate(a[0][k1], g2[k1])]
                    + [_twiddle16(a[n2][k1], n2 * k1, sgn) for n2 in range(1, 4)], sgn)
        for k2 in range(4):
            out[k1 + 4 * k2] = y[k2]
    return out


def _val(a):
    return a[1] if a[0] > 0 else -a[1]


def _lo(u):
    return pltpu.bitcast(u << 16, f32)


def _hi(u):
    return pltpu.bitcast(u & jnp.uint32(0xFFFF0000), f32)


def _pack2(a, b):
    lo = pltpu.bitcast(a.astype(bf16).astype(f32), u32) >> 16
    return lo | pltpu.bitcast(b.astype(bf16).astype(f32), u32)


def _bf(u):
    return pltpu.bitcast(u, bf16)


def _dot(a, b):
    return jnp.dot(a, b, preferred_element_type=f32)


def _dot_nt(a, b):
    return lax.dot_general(a, b, NT, preferred_element_type=f32)


def _lane(rows):
    return lax.broadcasted_iota(jnp.int32, (rows, 128), 1)


def _mirror(v):
    return jnp.take_along_axis(v, (128 - _lane(v.shape[0])) & 127, axis=1)


def _rep(t, n):
    k = t.shape[0] // 8
    return jnp.broadcast_to(t.reshape(k, 1, 8, 128), (k, n, 8, 128)).reshape(k * n * 8, 128)


_NGRP = 10
_S_OUT = _NGRP

_SCHED = ('a k0-4 v0-4 q0-4 k4-8 v4-8 p0-4 q4-8 k8-12 v8-12 p4-8 q8-12 k12-16 v12-16 p8-12 q12-16 '
          'o0-4 o4-9 p12-16 o9-12 o12-16').split()


def _kernel(xa_hbm, wr_hbm, wi_hbm, xb_hbm, m0_hbm, wq_hbm, wk_hbm, wv_hbm, wo_hbm,
            fd_hbm, fi_hbm, out_hbm,
            xe, xe32, xa, xst, xg, wst, wca, wcb, wsl, xq, fd, fi, gs, wr, wi, tsc, rv, ff,
            z32, wo, wo32, xb, m0, stage, zq, psc, qsc, osc, ssc, part, sems):
    w_hbms = (wq_hbm, wk_hbm, wv_hbm)

    def dyn(start, size):
        return pl.ds(start, size) if isinstance(start, int) else pl.ds(pl.multiple_of(start, size), size)

    def cp(src, dst, sem):
        return pltpu.make_async_copy(src, dst, sems.at[sem])

    def cp_w(m, g, sem):
        return cp(w_hbms[m].at[:, :, pl.ds(8 * g, 8), :], wst.at[4 * m + g], sem)

    def cp_xa(c0, c1, sem):
        rows = pl.ds(128 * c0, 128 * (c1 - c0))
        return cp(xa_hbm.at[:, rows, :], xa.at[:, rows, :], sem)

    def cp_f(src, dst, part, sem):
        rows = pl.ds(0, 160) if part == 0 else pl.ds(160, D // 2 + 1 - 160)
        return cp(src.at[rows, :], dst.at[rows, :], sem)

    def cp_half(k, sem_w, sem_x):
        rows, cols = pl.ds(128 * k, 128), pl.ds(256 * k, 256)
        return [cp(wq_hbm.at[rows, :, pl.ds(0, 8), :], wst.at[0, rows], sem_w),
                cp(xb_hbm.at[:, pl.ds(KEEP, XT), cols], xe.at[:, :, cols], sem_x)]

    grp = [
        cp_half(0, 0, 9),
        cp_half(1, 1, 1),
        [cp_w(0, 1, 2)],
        [cp(fd_hbm, fd, 3), cp_w(0, 2, 3), cp_xa(0, 3, 3)],
        [cp_w(0, 3, 4), cp_xa(3, 8, 4)],
        [cp_w(1, 0, 5), cp_f(wr_hbm, wr, 0, 5), cp_f(wi_hbm, wi, 0, 5), cp_w(1, 1, 5)],
        [cp_f(wr_hbm, wr, 1, 6), cp_f(wi_hbm, wi, 1, 6),
         cp_w(1, 2, 6), cp_w(1, 3, 6), cp_w(2, 0, 6), cp_w(2, 1, 6)],
        [cp_w(2, 2, 7), cp_w(2, 3, 7), cp(wo_hbm, wo, 7)],
        [cp(fi_hbm, fi, 8), cp(m0_hbm, m0, 8), cp(xb_hbm.at[:, pl.ds(0, KEEP), :], xb, 8)],
    ]
    for g_ in grp:
        for c_ in g_:
            c_.start()

    for p in range(2):
        zq[pl.ds(p, 8, stride=2), :] = jnp.zeros((8, 128), u32)

    def wait(copies):
        for c_ in copies:
            c_.wait()

    def tokens(stream):
        ys = jnp.concatenate(stream, axis=0)
        n = ys.shape[0] // 8

        def tok(start, count, step):
            assert start + (count - 1) * step < n, (start, count, step, n)
            first = min(start, n - count * step)
            y = ys[8 * first:8 * (first + count * step)].reshape(count, step, 8, 128)[:, start - first]
            return (pltpu.bitcast(y, u32) & zq[0:8, :][None]).reshape(count * 8, 128)
        return tok

    def opaque():
        z0 = zq[0, 0].astype(jnp.int32)
        idx = [jnp.clip(z0 + a, 0, NC - 1) for a in range(NC)]
        return lambda a: idx[a]

    def relayout(i, tok=None, start=0, step=1, r0=0, r1=D // 2):
        wc = (wca, wcb)[i % 2]
        n = r1 - r0
        m_lo, m_hi = jnp.uint32(0xFFFF), jnp.uint32(0xFFFF0000)
        if tok is not None:
            t1 = tok(start, n // 8, step)
            m_lo, m_hi = _rep(t1 | m_lo, 4), _rep(t1 | m_hi, 4)
            t2 = tok(start + 12, n // 8, step)
        ev = pltpu.bitcast(wst[i, r0:r1, 0].reshape(8 * n, DH), u32)
        od = pltpu.bitcast(wst[i, r0:r1, 1].reshape(8 * n, DH), u32)
        wc[0, 4 * r0:4 * r1, :] = (ev & m_lo) | (od << 16)
        wc[1, 4 * r0:4 * r1, :] = (ev >> 16) | (od & m_hi)
        for j in range(4):
            for p in range(2):
                v = wc[p, pl.ds(4 * r0 + j, n, stride=4), :]
                wsl[8 * i + 2 * j + p, r0:r1, :] = v if tok is None else v | t2

    def x_half(k, h0, h1, r0=0, r1=NSEG * XT):
        lhs = _bf(xe32[r0 // 2:r1 // 2, 256 * k:256 * k + 256])
        ys = []
        for h in range(h0, h1):
            ys.append(_dot(lhs, _bf(wsl[h, 128 * k:128 * k + 128, :])))
            if k == 0:
                part[h, r0:r1, :] = ys[-1]
            else:
                xq[r0 // 32:r1 // 32, h] = (ys[-1] + part[h, r0:r1, :]).astype(bf16).reshape(-1, SPB * XT, DH)
        return ys

    def pack_xe(k, tok=None):
        v = pltpu.bitcast(xe[:, :, 256 * k:256 * k + 256].reshape(NSEG * XT, 256), u32)
        if tok is not None:
            v = v | jnp.concatenate([tok(0, 32, 1)] * 2, axis=1)
        xe32[:, 256 * k:256 * k + 256] = v

    def x_heads(h0, h1, r0=0, r1=NSEG * XT):
        lhs = _bf(xe32[r0 // 2:r1 // 2, :])
        ys = []
        for h in range(h0, h1):
            ys.append(_dot(lhs, _bf(wsl[h])))
            xq[r0 // 32:r1 // 32, h] = ys[-1].astype(bf16).reshape(-1, SPB * XT, DH)
        return ys

    def gather_x(c0, c1, tok, per):
        nc = c1 - c0
        first = _lane(8 * nc) == 0
        for hf in range(2):
            tk = jnp.stack([tok((4 * hf + q) * per // 24, nc, per).reshape(nc, 8, 128) for q in range(4)], axis=1)
            tk = _rep(tk.reshape(32 * nc, 128), 2)
            u = pltpu.bitcast(xa[hf, 128 * c0:128 * c1, :], u32)
            for a in range(4):
                xst[a, hf, 64 * c0:64 * c1, :] = u[:, 128 * a:128 * a + 128] | tk
        for j in range(8):
            for p, part in enumerate((_lo, _hi)):
                tk = pltpu.bitcast(tok((8 + 2 * j + p) * per // 24, nc, per), f32)
                xl, xh = [[part(xst[a, hf, pl.ds(64 * c0 + j, 8 * nc, stride=8), :]) for a in range(4)]
                          for hf in range(2)]
                xl[0], xl[1] = xl[0] + tk, xl[1] + tk
                for hf in range(2):
                    x0, x1, x2, x3 = [(l + h if hf == 0 else l - h) for l, h in zip(xl, xh)]
                    s02, s13 = x0 + x2, x1 + x3
                    al, rb = x0 - x2, _mirror(x1 - x3)
                    v = jnp.concatenate([s02 + s13, s02 - s13, al - jnp.where(first, 0.0, rb),
                                         jnp.where(first, 0.0, al) + rb], axis=1)
                    xg[2 * j + p, 64 * hf + 8 * c0:64 * hf + 8 * c1, :] = v.astype(bf16)

    def build_gs(tok, step):
        tk = pltpu.bitcast(tok(0, 4 * NC, step), f32)
        sd = lambda r0, r1, t: pltpu.bitcast(fd[64 + r0:64 + r1, 128 * t:128 * t + 128], f32)
        ct, st = [jnp.concatenate([jnp.broadcast_to(sd(32 + a % 8, 33 + a % 8, t + a // 8), (32, 128))
                                   for a in range(NC)], axis=0) + tk for t in (0, 2)]
        ce, se = [[jnp.concatenate([sd(0, 32, t + p)] * NC, axis=0) for p in range(2)] for t in (0, 2)]
        co = _pack2(*[ce[p] * ct - se[p] * st for p in range(2)])
        si = _pack2(*[se[p] * ct + ce[p] * st for p in range(2)])
        cr = pltpu.roll(co, 1, axis=1)
        ns = pltpu.roll(si, 1, axis=1) ^ jnp.uint32(0x80008000)
        ev = (_lane(32 * NC) & 1) == 0
        gs[:, 0:32, :] = jnp.concatenate(
            [jnp.where(ev, co, ns), jnp.where(ev, cr, si)], axis=1).reshape(NC, 32, 256)
        gs[:, 32:64, :] = jnp.concatenate(
            [jnp.where(ev, si, cr), jnp.where(ev, ns, co)], axis=1).reshape(NC, 32, 256)

    def d_fwd(a, at):
        y = [_dot_nt(_bf(fd[0:64, 128 * t:128 * t + 128]), xg[at(a), :, 128 * t:128 * t + 128]) for t in range(4)]
        ye = _pack2(y[0], y[1]).reshape(8, 2, 8, 128)
        po, qo = [y_.reshape(8, 2, 8, 128) for y_ in y[2:4]]
        p = jnp.concatenate([ye[:, 0], _pack2(po[:, 0], po[:, 1])], axis=0).reshape(128, 128)
        q = jnp.concatenate([ye[:, 1], _pack2(qo[:, 0], qo[:, 1])], axis=0).reshape(128, 128)
        q = pltpu.roll(q, 64, axis=1)
        lo = _lane(128) < 64
        return _bf(jnp.where(lo, p, q)), _bf(jnp.where(lo, q, p))

    def s_fwd(a, ls, at):
        o0 = _dot(ls[0], _bf(gs[at(a), :, 0:128]))
        o1 = _dot(ls[1], _bf(gs[at(a), :, 128:256]))
        ev = (_lane(256) & 1) == 0
        tsc[a, 0] = jnp.where(ev, o0, o1)
        tsc[a, 1] = jnp.where(ev, o1, o0)
        return o1

    def spectral_fwd(filler):
        at = opaque()
        ls = [d_fwd(a, at) for a in range(4)]
        stream = []
        for a in range(0, NC, 2):
            if a + 4 < NC:
                ls += [d_fwd(a + 4, at), d_fwd(a + 5, at)]
            if a == NC - 2:
                filler()
            s_fwd(a, ls[a], at)
            stream.append(s_fwd(a + 1, ls[a + 1], at))
        return stream

    rel = [0, 1, 2, 3, 4, 7, 10, 13, 16, 17.5, 19, 20.5]

    def negated(z):
        first = _lane(8) == 0
        return [jnp.where(first, z[(NC - k2) % NC], _mirror(z[NC - 1 - k2])) for k2 in range(NC)]

    def dc_filter(tok, start, step):
        tk = pltpu.bitcast(tok(start, NC, step), f32)
        row0 = lax.broadcasted_iota(jnp.int32, (8, 128), 0) == 0
        for c, (w, sg) in enumerate(((wr, 1.0), (wi, -1.0))):
            base = [_lo(pltpu.bitcast(w[0:16, 128 * k2:128 * k2 + 128], u32)) + tk[8 * k2:8 * k2 + 8]
                    for k2 in range(NC)]
            nyq = [w[256:257, 128 * k2:128 * k2 + 128].astype(f32) for k2 in range(NC)]
            pl_ = [b_ + n_ for b_, n_ in zip(base, nyq)]
            mi_ = [b_ - n_ for b_, n_ in zip(base, nyq)]
            f1 = [jnp.where(row0, 0.25 * (z + sg * zn), b_) for z, zn, b_ in zip(pl_, negated(pl_), base)]
            f2 = [jnp.where(row0, 0.25 * (z + sg * zn), 0.0) for z, zn in zip(mi_, negated(mi_))]
            ff[c] = jnp.concatenate(f1, axis=0)
            ff[2 + c] = jnp.concatenate(f2, axis=0)

    def spectral_mid(p, v0, v1, tok, start, per):
        nu = v1 - v0
        at = opaque()
        gate = lambda r: pltpu.bitcast(tok(start + int((r + 4) * per / 24), nu, per), f32)
        gates = [gate(r) for r in rel]
        pre = [gate(r - 4) for r in rel[0:4]]
        r0, r1 = 128 * p + 8 * v0, 128 * p + 8 * v1
        t = [((1, tsc[at(a), 0, r0:r1, :]), (1, pltpu.roll(tsc[at(a), 1, r0:r1, :] + pre[a % 4], 127, axis=1)))
             for a in range(NC)]
        x = _fft16(t, -1, gates[0:4], gates[4:8])
        y = []
        if r0 == 0:
            assert nu == 1
            xr, xi = [_val(v[0]) for v in x], [_val(v[1]) for v in x]
            for k2, (mr, mi) in enumerate(zip(negated(xr), negated(xi))):
                f1r, f1i, f2r, f2i = [ff[c, 8 * k2:8 * k2 + 8, :] for c in range(4)]
                y.append(((1, (xr[k2] * f1r - xi[k2] * f1i) + (mr * f2r + mi * f2i)),
                          (1, (xr[k2] * f1i + xi[k2] * f1r) + (mr * f2i - mi * f2r))))
        else:
            for k2 in range(NC):
                fa, fb = [(_lo, _hi)[p](pltpu.bitcast(w[16 * v0:16 * v1, 128 * k2:128 * k2 + 128], u32))
                          for w in (wr, wi)]
                (sr, xr), (si, xi) = x[k2]
                y.append((_ssub((sr, xr * fa), (si, xi * fb)), _sadd((sr, xr * fb), (si, xi * fa))))
        ev = (_lane(8 * nu) & 1) == 0
        u = _fft16(y, 1, None, gates[8:12])
        for k1 in range(4):
            ui = jnp.stack([_val(u[k1 + 4 * k2][1]).reshape(nu, 8, 128) for k2 in range(4)], axis=1)
            us4 = pltpu.roll(ui.reshape(32 * nu, 128), 1, axis=1).reshape(nu, 4, 8, 128)
            for k2 in range(4):
                ur, us = _val(u[k1 + 4 * k2][0]), us4[:, k2].reshape(8 * nu, 128)
                v01 = jnp.concatenate([jnp.where(ev, ur, us), jnp.where(ev, us, ur)], axis=1)
                rv[k1 + 4 * k2, r0:r1, :] = v01.astype(bf16)

    def spectral_inv():
        ev = (_lane(64) & 1) == 0
        at = opaque()
        for j in range(8):
            gri = []
            for a in (2 * j, 2 * j + 1):
                g = gs[at(a)]
                re = [g[0:32, 0:128], g[32:64, 128:256]]
                im = [g[32:64, 0:128], g[0:32, 128:256]]
                gri.append([_bf(jnp.stack([r_.reshape(4, 8, 128), i_.reshape(4, 8, 128)], axis=1).reshape(64, 128))
                            for r_, i_ in zip(re, im)])

            def tile(t):
                zs = [[_dot_nt(gri[c][e], rv[at(2 * j + c), 128 * t:128 * t + 128, 128 * e:128 * e + 128])
                       for e in range(2)] for c in range(2)]
                out = [_pack2(zs[0][0] + zs[0][1], zs[1][0] + zs[1][1]).reshape(4, 2, 16, 128),
                       _pack2(zs[0][0] - zs[0][1], zs[1][0] - zs[1][1]).reshape(4, 2, 16, 128)]
                return [(z[:, 0].reshape(64, 128), z[:, 1].reshape(64, 128)) for z in out]

            even = tile(0)
            odd = tile(1)
            for be in range(2):
                zr, zi = even[be]
                sh = pltpu.roll(zi, 1, axis=1)
                tiles = [jnp.where(ev, zr, sh), jnp.where(ev, sh, zr), odd[be][0], odd[be][1]]
                for t in range(4):
                    z32[t, pl.ds(512 * be + j, 64, stride=8), :] = tiles[t]

    def copy_wo(tok, step):
        tk = _rep(tok(0, 64, step), 4)
        wo32[...] = pltpu.bitcast(wo[...], u32) | jnp.concatenate([tk] * 4, axis=1)

    def xv_part(b, h0, h1):
        lhs = _bf(xe32[dyn(16 * b, 16), :])
        ys = []
        for h in range(h0, h1):
            ys.append(_dot(lhs, _bf(wsl[2 * H + h])))
            xq[b, 2 * H + h] = ys[-1].astype(bf16)
        return ys

    wait(grp[0][0:1])
    for c in range(4):
        relayout(0, r0=32 * c, r1=32 * c + 32)
    wait(grp[0][1:2])
    pack_xe(0)
    x_half(0, 0, 6)

    wait(grp[1])
    tok = tokens(x_half(0, 6, 8)[1:])
    relayout(0, tok, 0, 2, r0=128)
    pack_xe(1, tok)
    x_half(1, 0, 4)
    x_half(1, 4, 6, 0, 256)

    wait(grp[2])
    relayout(1, tokens(x_half(1, 4, 6, 256)[1:] + x_half(1, 6, 8)[1:]), 0, 2)
    x_heads(8, 14)
    x_heads(14, 15, 0, 256)

    wait(grp[3])
    relayout(2, tokens(x_heads(14, 15, 256) + x_heads(15, 16)), 0, 2)
    tok = tokens(x_heads(16, 22))
    gather_x(0, 3, tok, 120)
    build_gs(tok, 5)
    x_heads(22, 23, 0, 256)

    wait(grp[4])
    relayout(3, tokens(x_heads(22, 23, 256) + x_heads(23, 24)), 0, 2)
    gather_x(3, 8, tokens(x_heads(24, 29)), 55)
    spectral_fwd(lambda: x_heads(29, 30))

    wait(grp[5])
    relayout(4, tokens(x_heads(30, 32)), 0, 3)
    tok = tokens(x_heads(32, 40))
    relayout(5, tok, 0, 14)
    spectral_mid(0, 1, 10, tok, 0, 56)
    spectral_mid(1, 0, 6, tokens(x_heads(40, 46)), 0, 54)

    wait(grp[6])
    relayout(6, tokens(x_heads(46, 48)), 0, 3)
    tok = tokens(x_heads(48, 56))
    relayout(7, tok, 0, 7)
    relayout(8, tok, 230, 7)
    dc_filter(tok, 0, 20)
    spectral_mid(0, 10, 16, tok, 0, 66)
    spectral_mid(0, 0, 1, tok, 400, 100)
    tok = tokens(x_heads(56, 62) + x_heads(64, 64 + XVP // 2))
    relayout(9, tok, 0, 16)
    spectral_mid(1, 6, 16, tok, 0, 52)
    spectral_inv()

    wait(grp[7])
    st = x_heads(62, 64) + x_heads(64 + XVP // 2, 64 + XVP) + xv_part(0, XVP, 16)
    tok = tokens(st)
    relayout(10, tok, 0, 4)
    relayout(11, tok, 150, 4)
    copy_wo(tokens(st + xv_part(0, 16, XVL)), 5)
    wait(grp[8])

    r = lax.broadcasted_iota(jnp.int32, (R2, 128), 0)
    c = lax.broadcasted_iota(jnp.int32, (R2, 128), 1)

    def head_pos(i):
        head = jnp.where(i < 32, 0, jnp.where(i < 64, 1, jnp.where(i < 72, 0, jnp.where(i < R2, 1, 2))))
        pos = jnp.where(i < 32, i, jnp.where(i < 72, i - 32, i - 40))
        return head, pos

    rh, rpos = head_pos(r)
    ch, cpos = head_pos(c)
    same = (rh - ch) == 0
    ok = jnp.logical_and(same, jnp.logical_or(rpos < MEM, rpos >= cpos))
    fill = jnp.where(same, jnp.float32(-1e9 / SCALE), jnp.float32(-jnp.inf))

    def step(b, k, mem, filler):
        s = SPB * b + k
        second = k % 2 == 1
        mo = 48 if second else 32
        lhs = jnp.concatenate([mem, xb[s].astype(f32)], axis=0).astype(bf16)
        if not second:
            lhs48 = jnp.concatenate([lhs, _bf(xe32[dyn(4 * s, 8), :])], axis=0)
        acc = [None] * 4
        stream = []

        def proj(m, hp):
            y = jnp.concatenate([_dot(lhs, _bf(wsl[H * m + 2 * hp + hh])) for hh in range(2)], axis=0)
            qsc[m, hp] = y.astype(bf16)
            stream.append(y)

        def oper(m, hp):
            xs = [xq[b, H * m + 2 * hp + hh, XT * k:XT * k + XT, :] for hh in range(2)]
            if m > 0:
                xs.append(jnp.zeros((128 - R2, DH), bf16))
            return jnp.concatenate([qsc[m, hp]] + xs, axis=0)

        def do_qkp(hp):
            proj(0, hp)
            proj(1, hp)

        def do_v(hp):
            if second or 2 * hp < XVL:
                proj(2, hp)
                return
            ys = [_dot(lhs48, _bf(wsl[2 * H + 2 * hp + hh])) for hh in range(2)]
            y = jnp.concatenate([ys[0][0:32], ys[1][0:32]], axis=0)
            qsc[2, hp] = y.astype(bf16)
            for hh in range(2):
                xq[b, 2 * H + 2 * hp + hh, XT * k:XT * k + 2 * XT, :] = ys[hh][32:48].astype(bf16)
            stream.append(y)

        def do_qk(hp):
            ssc[hp] = jnp.where(ok, _dot_nt(oper(0, hp), oper(1, hp)), fill)
            stream.clear()

        def do_softmax(p0, p1):
            nt = 20 if p1 < NP else 5
            g = pltpu.bitcast(_rep(tokens(stream[0:3])(0, nt, 1), 40 // nt), f32)
            sc = ssc[p0:p1].reshape(4 * R2, 128) + g
            mx = jnp.max(sc, axis=-1, keepdims=True)
            e = jnp.exp2((sc - mx) * (SCALE * LOG2E))
            l = jnp.sum(e, axis=-1, keepdims=True)
            rl = pl.reciprocal(l, approx=True)
            rl = rl * (2.0 - l * rl)
            psc[p0:p1] = (e * rl).astype(bf16).reshape(4, R2, 128)

        def do_pv(hp):
            o2 = _dot(psc[hp], oper(2, hp))
            r0 = 40 if second else 32
            for hh in range(2):
                osc[2 * hp + hh, 0:32, :] = o2[32 * hh:32 * hh + 32].astype(bf16)
                osc[2 * hp + hh, r0:r0 + 8, :] = o2[64 + 8 * hh:72 + 8 * hh].astype(bf16)

        def do_o(p0, p1):
            ol = jnp.concatenate([osc[h, 0:mo, :] for h in range(2 * p0, 2 * p1)], axis=1)
            for n in range(4):
                y = _dot(ol, _bf(wo32[p0 * 128:p1 * 128, 128 * n:128 * n + 128]))
                acc[n] = y if acc[n] is None else acc[n] + y
                stream.append(y)

        def do_a3():
            zr = dyn(16 * s, 32)
            v0, v2, vc, vs = [_dot(_bf(z32[t, zr, :]), _bf(fi[:, 128 * t:128 * t + 128])) for t in range(4)]
            sp, sm = v0 + v2, v0 - v2
            first = _lane(2 * SEG) == 0
            al, be = vc + jnp.where(first, 0.0, vs), _mirror(vs - jnp.where(first, 0.0, vc))
            ya = jnp.concatenate([sp + al, sm + be, sp - al, sm - be], axis=1).astype(bf16)
            stage[pl.ds(s, 2), :, 0:D] = ya.reshape(2, SEG, D)

        for op in _SCHED:
            if op == 'a':
                if not second:
                    do_a3()
                continue
            p0, p1 = [int(v) for v in op[1:].split('-')]
            if op[0] == 'p':
                do_softmax(p0, p1)
            if op[0] == 'o':
                do_o(p0, p1)
            else:
                for hp in range(p0, p1):
                    {'k': do_qkp, 'v': do_v, 'q': do_qk, 'p': do_pv}[op[0]](hp)
        filler()
        return jnp.concatenate(acc, axis=1)

    nb = NSEG // SPB
    hv = [XVP, 10, 12, 16, XVL]

    def body(b, mem):
        nxt = jnp.minimum(b + 1, nb - 1)
        for k in range(0, SPB, 2):
            sa, sb = SPB * b + k, SPB * b + k + 1
            ya = step(b, k, mem, lambda: xv_part(nxt, hv[k], hv[k + 1]))
            stage[sa, 0:KEEP, D:2 * D] = ya[MEM:].astype(bf16)
            mem_b = ya[0:MEM].astype(bf16).astype(f32)
            yb = step(b, k + 1, mem_b, lambda: xv_part(nxt, hv[k + 1], hv[k + 2]))
            stage[sa, KEEP:SEG, D:2 * D] = yb[32:40].astype(bf16)
            stage[sb, :, D:2 * D] = jnp.concatenate([yb[MEM:32], yb[40:48]], axis=0).astype(bf16)
            mem = yb[0:MEM].astype(bf16).astype(f32)
            rows = pl.ds(sa, 2)
            cp(stage.at[rows], out_hbm.at[rows], _S_OUT).start()
        return mem

    lax.fori_loop(0, nb, body, m0[...].astype(f32))
    wait([cp(stage, out_hbm, _S_OUT)])


@jax.jit
def pallas_concat_heads__spectral_gfnet__memory_aug_recurrent_mem_tr__prompt_kernel(
    A_x: jax.Array,
    A_w_r: jax.Array,
    A_w_i: jax.Array,
    B_x: jax.Array,
    B_mem0: jax.Array,
    B_Wq: jax.Array,
    B_Wk: jax.Array,
    B_Wv: jax.Array,
    B_Wo: jax.Array,
    B_seg_len: jax.Array,
):
    del B_seg_len
    assert A_x.shape == (1, S, D) and B_x.shape == (1, S, D) and B_mem0.shape == (1, MEM, D)
    assert B_Wq.shape == (D, H, DH) and B_Wo.shape == (H, DH, D)
    fd, fi = _dft_tables()
    vm = pltpu.VMEM
    scratch = [
        vm((NSEG, XT, D), bf16),
        vm((NSEG * XT // 2, D), u32),
        vm((2, S // 2, D), bf16),
        vm((4, 2, S // 4, 128), u32),
        vm((NC, 128, D), bf16),
        vm((12, D // 2, 2, 8, DH), bf16),
        vm((2, 2 * D, DH), u32),
        vm((2, 2 * D, DH), u32),
        vm((3 * H, D // 2, DH), u32),
        vm((NSEG // SPB, 3 * H, SPB * XT, DH), bf16),
        vm((104, 512), u32),
        vm((64, 512), u32),
        vm((NC, 64, 256), u32),
        vm((D // 2 + 1, S), bf16),
        vm((D // 2 + 1, S), bf16),
        vm((NC, 2, 256, 128), f32),
        vm((NC, 256, 256), bf16),
        vm((4, NC * 8, 128), f32),
        vm((4, S // 2, 128), u32),
        vm((H * DH, D), bf16),
        vm((H * DH // 2, D), u32),
        vm((NSEG, KEEP, D), bf16),
        vm((MEM, D), bf16),
        vm((NSEG, SEG, 2 * D), bf16),
        vm((16, 128), u32),
        vm((NP, R2, 128), bf16),
        vm((3, NP, 64, DH), bf16),
        vm((H, 48, DH), bf16),
        vm((NP, R2, 128), f32),
        vm((8, NSEG * XT, DH), f32),
        pltpu.SemaphoreType.DMA((_NGRP + 1,)),
    ]
    w4 = lambda w: w.reshape(D // 2, 2, H, DH)
    out = pl.pallas_call(
        _kernel,
        out_shape=jax.ShapeDtypeStruct((NSEG, SEG, 2 * D), bf16),
        in_specs=[pl.BlockSpec(memory_space=pl.ANY)] * 11,
        out_specs=pl.BlockSpec(memory_space=pl.ANY),
        scratch_shapes=scratch,
        compiler_params=pltpu.CompilerParams(vmem_limit_bytes=110 * 1024 * 1024),
    )(A_x.reshape(2, S // 2, D), A_w_r.T, A_w_i.T, B_x.reshape(NSEG, SEG, D), B_mem0.reshape(MEM, D),
      w4(B_Wq), w4(B_Wk), w4(B_Wv), B_Wo.reshape(H * DH, D), fd, fi)
    return out.reshape(1, S, 2 * D)
```

```python
import math

import numpy as np
import jax
import jax.numpy as jnp
from jax import lax
import jax.experimental.pallas as pl
import jax.experimental.pallas.tpu as pltpu

S, D = 2048, 512
H, DH = 32, 128
MEM, SEG = 8, 32
NSEG = S // SEG
NP = H // 2
XT = 8
KEEP = SEG - XT
R2 = 2 * (MEM + SEG)
SCALE = DH ** -0.5
LOG2E = 1.4426950408889634
NC = 16
SPB = 4
XVP = 6
XVL = 20

f32, bf16, u32 = jnp.float32, jnp.bfloat16, jnp.uint32
NT = (((1,), (1,)), ((), ()))


def _pack_rows(m):
    b = np.asarray(m, np.float32).astype(jnp.bfloat16).view(np.uint16).astype(np.uint32)
    return b[0::2, :] | (b[1::2, :] << 16)


def _dft_tables():
    k = np.arange(D // 2)[:, None]
    d = np.arange(D // 2)[None, :]
    ang = 2.0 * np.pi * ((k * d) % D) / D
    pm = np.cos(ang)
    qm = -np.sin(ang)
    qm[0] = (-1.0) ** np.arange(D // 2)
    qo = qm[:, :128].copy()
    qo[:, 0] = qm[:, 128]

    def inter(parts):
        c = parts[0].shape[1]
        return np.stack([p.reshape(-1, 8, c) for p in parts], axis=1).reshape(-1, c)

    f0 = inter([pm[0::4, :128], qm[0::4, :128]])
    f2 = inter([pm[2::4, :128], qm[2::4, :128]])
    fp = inter([pm[1::4, :128], pm[3::4, :128]])
    fq = inter([qo[1::4], qo[3::4]])
    fd = np.concatenate([f0, f2, fp, fq], axis=1)
    wgt = np.where(k == 0, 1.0, 2.0) / (S * D)
    pw, qw = wgt * pm, wgt * qm
    ii = np.arange(64)
    i0 = np.zeros((128, 128))
    i2 = np.zeros((128, 128))
    i0[2 * ii], i0[2 * ii + 1] = pw[0::4, :128], qw[0::4, :128]
    i2[2 * ii + 1], i2[(2 * ii + 2) % 128] = pw[2::4, :128], qw[2::4, :128]
    fi = np.concatenate([i0, i2, pw[1::2, :128], (wgt * qo)[1::2]], axis=1)
    k1 = np.arange(128)[None, :]
    mo = np.concatenate([ii[0::2], ii[1::2]])[:, None]
    ae = 2.0 * np.pi * ((NC * mo * k1) % S) / S
    at = 2.0 * np.pi * (np.arange(NC)[:, None] * k1) / S
    side = lambda c, s_: np.concatenate(np.split(c, 2) + np.split(s_, 2), axis=1)
    sd = np.concatenate([side(np.cos(ae), np.sin(ae)), side(np.cos(at), np.sin(at))]).astype(np.float32)
    return np.concatenate([_pack_rows(fd), sd.view(np.uint32)], axis=0), _pack_rows(fi)


def _sadd(a, b):
    (sa, va), (sb, vb) = a, b
    if sa == sb:
        return (sa, va + vb)
    return (1, va - vb) if sa > 0 else (1, vb - va)


def _sneg(a):
    return (-a[0], a[1])


def _ssub(a, b):
    return _sadd(a, _sneg(b))


def _smul(a, c):
    return (a[0], a[1] * c) if c > 0 else (-a[0], a[1] * (-c))


def _cadd(a, b):
    return (_sadd(a[0], b[0]), _sadd(a[1], b[1]))


def _csub(a, b):
    return (_ssub(a[0], b[0]), _ssub(a[1], b[1]))


def _cmul_i(a, sgn):
    return (_sneg(a[1]), a[0]) if sgn > 0 else (a[1], _sneg(a[0]))


def _radix4(x, sgn):
    t0, t1 = _cadd(x[0], x[2]), _csub(x[0], x[2])
    t2, t3 = _cadd(x[1], x[3]), _cmul_i(_csub(x[1], x[3]), sgn)
    return [_cadd(t0, t2), _cadd(t1, t3), _csub(t0, t2), _csub(t1, t3)]


def _twiddle16(a, m, sgn):
    if m == 0:
        return a
    if m == 4:
        return _cmul_i(a, sgn)
    c, s = math.cos(2 * math.pi * m / 16), sgn * math.sin(2 * math.pi * m / 16)
    if m in (2, 6):
        if c * s > 0:
            return (_smul(_ssub(a[0], a[1]), c), _smul(_sadd(a[0], a[1]), c))
        return (_smul(_sadd(a[0], a[1]), c), _smul(_ssub(a[1], a[0]), c))
    return (_ssub(_smul(a[0], c), _smul(a[1], s)), _sadd(_smul(a[0], s), _smul(a[1], c)))


def _gate(x, t):
    if t is None:
        return x
    (sr, vr), (si, vi) = x
    return ((sr, vr + t), (si, vi + t))


def _fft16(x, sgn, g1=None, g2=None):
    g1 = g1 or [None] * 4
    g2 = g2 or [None] * 4
    a = [_radix4([_gate(x[n2], g1[n2])] + [x[4 * n1 + n2] for n1 in range(1, 4)], sgn) for n2 in range(4)]
    out = [None] * 16
    for k1 in range(4):
        y = _radix4([_gate(a[0][k1], g2[k1])]
                    + [_twiddle16(a[n2][k1], n2 * k1, sgn) for n2 in range(1, 4)], sgn)
        for k2 in range(4):
            out[k1 + 4 * k2] = y[k2]
    return out


def _val(a):
    return a[1] if a[0] > 0 else -a[1]


def _lo(u):
    return pltpu.bitcast(u << 16, f32)


def _hi(u):
    return pltpu.bitcast(u & jnp.uint32(0xFFFF0000), f32)


def _pack2(a, b):
    lo = pltpu.bitcast(a.astype(bf16).astype(f32), u32) >> 16
    return lo | (pltpu.bitcast(b.astype(bf16).astype(f32), u32) & jnp.uint32(0xFFFF0000))


def _bf(u):
    return pltpu.bitcast(u, bf16)


def _dot(a, b):
    return jnp.dot(a, b, preferred_element_type=f32)


def _dot_nt(a, b):
    return lax.dot_general(a, b, NT, preferred_element_type=f32)


def _lane(rows):
    return lax.broadcasted_iota(jnp.int32, (rows, 128), 1)


def _mirror(v):
    return jnp.take_along_axis(v, (128 - _lane(v.shape[0])) & 127, axis=1)


def _rep(t, n):
    k = t.shape[0] // 8
    return jnp.broadcast_to(t.reshape(k, 1, 8, 128), (k, n, 8, 128)).reshape(k * n * 8, 128)


_NGRP = 11
_S_OUT = _NGRP

_SCHED = ('a k0-4 v0-4 q0-4 k4-8 v4-8 p0-4 q4-8 k8-12 v8-12 p4-8 q8-12 k12-16 v12-16 p8-12 q12-16 '
          'o0-4 o4-9 p12-16 o9-12 o12-16').split()


def _kernel(xa_hbm, wr_hbm, wi_hbm, xb_hbm, m0_hbm, wq_hbm, wk_hbm, wv_hbm, wo_hbm,
            fd_hbm, fi_hbm, out_hbm,
            xe, xe32, xa, xst, xg, wst, wca, wcb, wsl, xq, fd, fi, gs, wr, wi, tsc, rv, ff,
            z32, wo, wo32, xb, m0, stage, zq, psc, qsc, osc, ssc, part, sems):
    w_hbms = (wq_hbm, wk_hbm, wv_hbm)

    def dyn(start, size):
        return pl.ds(start, size) if isinstance(start, int) else pl.ds(pl.multiple_of(start, size), size)

    def cp(src, dst, sem):
        return pltpu.make_async_copy(src, dst, sems.at[sem])

    def cp_w(m, g, sem):
        return cp(w_hbms[m].at[:, :, pl.ds(8 * g, 8), :], wst.at[4 * m + g], sem)

    def cp_xa(c0, c1, sem):
        rows = pl.ds(128 * c0, 128 * (c1 - c0))
        return cp(xa_hbm.at[:, rows, :], xa.at[:, rows, :], sem)

    def cp_f(src, dst, part, sem):
        rows = pl.ds(0, 160) if part == 0 else pl.ds(160, D // 2 + 1 - 160)
        return cp(src.at[rows, :], dst.at[rows, :], sem)

    def cp_half(k, sem_w, sem_x):
        rows, cols = pl.ds(128 * k, 128), pl.ds(256 * k, 256)
        return [cp(wq_hbm.at[rows, :, pl.ds(0, 8), :], wst.at[0, rows], sem_w),
                cp(xb_hbm.at[:, pl.ds(KEEP, XT), cols], xe.at[:, :, cols], sem_x)]

    def cp_xb(s0, s1, sem):
        rows = pl.ds(s0, s1 - s0)
        return cp(xb_hbm.at[rows, pl.ds(0, KEEP), :], xb.at[rows], sem)

    grp = [
        cp_half(0, 0, 9),
        cp_half(1, 1, 1),
        [cp_w(0, 1, 2)],
        [cp(fd_hbm, fd, 3), cp_w(0, 2, 3), cp_xa(0, 3, 3)],
        [cp_w(0, 3, 4), cp_xa(3, 8, 4)],
        [cp_w(1, 0, 5), cp_f(wr_hbm, wr, 0, 5), cp_f(wi_hbm, wi, 0, 5), cp_w(1, 1, 5)],
        [cp_f(wr_hbm, wr, 1, 6), cp_f(wi_hbm, wi, 1, 6),
         cp_w(1, 2, 6), cp_w(1, 3, 6), cp_w(2, 0, 6), cp_w(2, 1, 6)],
        [cp_w(2, 2, 7), cp_w(2, 3, 7), cp(wo_hbm, wo, 7)],
        [cp(fi_hbm, fi, 8), cp(m0_hbm, m0, 8), cp_xb(0, SPB, 8)],
        [cp_xb(SPB, NSEG, 10)],
    ]
    for g_ in grp:
        for c_ in g_:
            c_.start()

    for p in range(2):
        zq[pl.ds(p, 8, stride=2), :] = jnp.zeros((8, 128), u32)

    def wait(copies):
        for c_ in copies:
            c_.wait()

    def tokens(stream):
        ys = jnp.concatenate(stream, axis=0)
        n = ys.shape[0] // 8

        def tok(start, count, step):
            assert start + (count - 1) * step < n, (start, count, step, n)
            first = min(start, n - count * step)
            y = ys[8 * first:8 * (first + count * step)].reshape(count, step, 8, 128)[:, start - first]
            return (pltpu.bitcast(y, u32) & zq[0:8, :][None]).reshape(count * 8, 128)
        return tok

    def opaque():
        z0 = zq[0, 0].astype(jnp.int32)
        idx = [jnp.clip(z0 + a, 0, NC - 1) for a in range(NC)]
        return lambda a: idx[a]

    def relayout(i, tok=None, start=0, step=1, r0=0, r1=D // 2):
        wc = (wca, wcb)[i % 2]
        n = r1 - r0
        m_lo, m_hi = jnp.uint32(0xFFFF), jnp.uint32(0xFFFF0000)
        if tok is not None:
            t1 = tok(start, n // 8, step)
            m_lo, m_hi = _rep(t1 | m_lo, 4), _rep(t1 | m_hi, 4)
            t2 = tok(start + 12, n // 8, step)
        ev = pltpu.bitcast(wst[i, r0:r1, 0].reshape(8 * n, DH), u32)
        od = pltpu.bitcast(wst[i, r0:r1, 1].reshape(8 * n, DH), u32)
        wc[0, 4 * r0:4 * r1, :] = (ev & m_lo) | (od << 16)
        wc[1, 4 * r0:4 * r1, :] = (ev >> 16) | (od & m_hi)
        for j in range(4):
            for p in range(2):
                v = wc[p, pl.ds(4 * r0 + j, n, stride=4), :]
                wsl[8 * i + 2 * j + p, r0:r1, :] = v if tok is None else v | t2

    def x_half(k, h0, h1, r0=0, r1=NSEG * XT):
        lhs = _bf(xe32[r0 // 2:r1 // 2, 256 * k:256 * k + 256])
        ys = []
        for h in range(h0, h1):
            ys.append(_dot(lhs, _bf(wsl[h, 128 * k:128 * k + 128, :])))
            if k == 0:
                part[h, r0:r1, :] = ys[-1]
            else:
                xq[r0 // 32:r1 // 32, h] = (ys[-1] + part[h, r0:r1, :]).astype(bf16).reshape(-1, SPB * XT, DH)
        return ys

    def pack_xe(k, tok=None):
        v = pltpu.bitcast(xe[:, :, 256 * k:256 * k + 256].reshape(NSEG * XT, 256), u32)
        if tok is not None:
            v = v | jnp.concatenate([tok(0, 32, 1)] * 2, axis=1)
        xe32[:, 256 * k:256 * k + 256] = v

    def x_heads(h0, h1, r0=0, r1=NSEG * XT):
        lhs = _bf(xe32[r0 // 2:r1 // 2, :])
        ys = []
        for h in range(h0, h1):
            ys.append(_dot(lhs, _bf(wsl[h])))
            xq[r0 // 32:r1 // 32, h] = ys[-1].astype(bf16).reshape(-1, SPB * XT, DH)
        return ys

    def gather_x(c0, c1, tok, per):
        nc = c1 - c0
        first = _lane(8 * nc) == 0
        for hf in range(2):
            tk = jnp.stack([tok((4 * hf + q) * per // 24, nc, per).reshape(nc, 8, 128) for q in range(4)], axis=1)
            tk = _rep(tk.reshape(32 * nc, 128), 2)
            u = pltpu.bitcast(xa[hf, 128 * c0:128 * c1, :], u32)
            for a in range(4):
                xst[a, hf, 64 * c0:64 * c1, :] = u[:, 128 * a:128 * a + 128] | tk
        for j in range(8):
            for p, part in enumerate((_lo, _hi)):
                tk = pltpu.bitcast(tok((8 + 2 * j + p) * per // 24, nc, per), f32)
                xl, xh = [[part(xst[a, hf, pl.ds(64 * c0 + j, 8 * nc, stride=8), :]) for a in range(4)]
                          for hf in range(2)]
                xl[0], xl[1] = xl[0] + tk, xl[1] + tk
                for hf in range(2):
                    x0, x1, x2, x3 = [(l + h if hf == 0 else l - h) for l, h in zip(xl, xh)]
                    s02, s13 = x0 + x2, x1 + x3
                    al, rb = x0 - x2, _mirror(x1 - x3)
                    v = jnp.concatenate([s02 + s13, s02 - s13, al - jnp.where(first, 0.0, rb),
                                         jnp.where(first, 0.0, al) + rb], axis=1)
                    xg[2 * j + p, 64 * hf + 8 * c0:64 * hf + 8 * c1, :] = v.astype(bf16)

    def build_gs(tok, step):
        tk = pltpu.bitcast(tok(0, 4 * NC, step), f32)
        sd = lambda r0, r1, t: pltpu.bitcast(fd[64 + r0:64 + r1, 128 * t:128 * t + 128], f32)
        ct, st = [jnp.concatenate([jnp.broadcast_to(sd(32 + a % 8, 33 + a % 8, t + a // 8), (32, 128))
                                   for a in range(NC)], axis=0) + tk for t in (0, 2)]
        ce, se = [[jnp.concatenate([sd(0, 32, t + p)] * NC, axis=0) for p in range(2)] for t in (0, 2)]
        co = _pack2(*[ce[p] * ct - se[p] * st for p in range(2)])
        si = _pack2(*[se[p] * ct + ce[p] * st for p in range(2)])
        cr = pltpu.roll(co, 1, axis=1)
        ns = pltpu.roll(si, 1, axis=1) ^ jnp.uint32(0x80008000)
        ev = (_lane(32 * NC) & 1) == 0
        gs[:, 0:32, :] = jnp.concatenate(
            [jnp.where(ev, co, ns), jnp.where(ev, cr, si)], axis=1).reshape(NC, 32, 256)
        gs[:, 32:64, :] = jnp.concatenate(
            [jnp.where(ev, si, cr), jnp.where(ev, ns, co)], axis=1).reshape(NC, 32, 256)

    def d_fwd(a, at):
        y = [_dot_nt(_bf(fd[0:64, 128 * t:128 * t + 128]), xg[at(a), :, 128 * t:128 * t + 128]) for t in range(4)]
        ye = _pack2(y[0], y[1]).reshape(8, 2, 8, 128)
        po, qo = [y_.reshape(8, 2, 8, 128) for y_ in y[2:4]]
        p = jnp.concatenate([ye[:, 0], _pack2(po[:, 0], po[:, 1])], axis=0).reshape(128, 128)
        q = jnp.concatenate([ye[:, 1], _pack2(qo[:, 0], qo[:, 1])], axis=0).reshape(128, 128)
        q = pltpu.roll(q, 64, axis=1)
        lo = _lane(128) < 64
        return _bf(jnp.where(lo, p, q)), _bf(jnp.where(lo, q, p))

    def s_fwd(a, ls, at):
        o0 = _dot(ls[0], _bf(gs[at(a), :, 0:128]))
        o1 = _dot(ls[1], _bf(gs[at(a), :, 128:256]))
        ev = (_lane(256) & 1) == 0
        tsc[a, 0] = jnp.where(ev, o0, o1)
        tsc[a, 1] = jnp.where(ev, o1, o0)
        return o1

    def spectral_fwd(filler):
        at = opaque()
        ls = [d_fwd(a, at) for a in range(4)]
        stream = []
        for a in range(0, NC, 2):
            if a + 4 < NC:
                ls += [d_fwd(a + 4, at), d_fwd(a + 5, at)]
            if a == NC - 2:
                filler()
            s_fwd(a, ls[a], at)
            stream.append(s_fwd(a + 1, ls[a + 1], at))
        return stream

    rel = [0, 1, 2, 3, 4, 7, 10, 13, 16, 17.5, 19, 20.5]

    def negated(z):
        first = _lane(8) == 0
        return [jnp.where(first, z[(NC - k2) % NC], _mirror(z[NC - 1 - k2])) for k2 in range(NC)]

    def dc_filter(tok, start, step):
        tk = pltpu.bitcast(tok(start, NC, step), f32)
        row0 = lax.broadcasted_iota(jnp.int32, (8, 128), 0) == 0
        for c, (w, sg) in enumerate(((wr, 1.0), (wi, -1.0))):
            base = [_lo(pltpu.bitcast(w[0:16, 128 * k2:128 * k2 + 128], u32)) + tk[8 * k2:8 * k2 + 8]
                    for k2 in range(NC)]
            nyq = [w[256:257, 128 * k2:128 * k2 + 128].astype(f32) for k2 in range(NC)]
            pl_ = [b_ + n_ for b_, n_ in zip(base, nyq)]
            mi_ = [b_ - n_ for b_, n_ in zip(base, nyq)]
            f1 = [jnp.where(row0, 0.25 * (z + sg * zn), b_) for z, zn, b_ in zip(pl_, negated(pl_), base)]
            f2 = [jnp.where(row0, 0.25 * (z + sg * zn), 0.0) for z, zn in zip(mi_, negated(mi_))]
            ff[c] = jnp.concatenate(f1, axis=0)
            ff[2 + c] = jnp.concatenate(f2, axis=0)

    def spectral_mid(p, v0, v1, tok, start, per):
        nu = v1 - v0
        at = opaque()
        gate = lambda r: pltpu.bitcast(tok(start + int((r + 4) * per / 24), nu, per), f32)
        gates = [gate(r) for r in rel]
        pre = [gate(r - 4) for r in rel[0:4]]
        r0, r1 = 128 * p + 8 * v0, 128 * p + 8 * v1
        t = [((1, tsc[at(a), 0, r0:r1, :]), (1, pltpu.roll(tsc[at(a), 1, r0:r1, :] + pre[a % 4], 127, axis=1)))
             for a in range(NC)]
        x = _fft16(t, -1, gates[0:4], gates[4:8])
        y = []
        if r0 == 0:
            assert nu == 1
            xr, xi = [_val(v[0]) for v in x], [_val(v[1]) for v in x]
            for k2, (mr, mi) in enumerate(zip(negated(xr), negated(xi))):
                f1r, f1i, f2r, f2i = [ff[c, 8 * k2:8 * k2 + 8, :] for c in range(4)]
                y.append(((1, (xr[k2] * f1r - xi[k2] * f1i) + (mr * f2r + mi * f2i)),
                          (1, (xr[k2] * f1i + xi[k2] * f1r) + (mr * f2i - mi * f2r))))
        else:
            for k2 in range(NC):
                fa, fb = [(_lo, _hi)[p](pltpu.bitcast(w[16 * v0:16 * v1, 128 * k2:128 * k2 + 128], u32))
                          for w in (wr, wi)]
                (sr, xr), (si, xi) = x[k2]
                y.append((_ssub((sr, xr * fa), (si, xi * fb)), _sadd((sr, xr * fb), (si, xi * fa))))
        ev = (_lane(8 * nu) & 1) == 0
        u = _fft16(y, 1, None, gates[8:12])
        for k1 in range(4):
            ui = jnp.stack([_val(u[k1 + 4 * k2][1]).reshape(nu, 8, 128) for k2 in range(4)], axis=1)
            us4 = pltpu.roll(ui.reshape(32 * nu, 128), 1, axis=1).reshape(nu, 4, 8, 128)
            for k2 in range(4):
                ur, us = _val(u[k1 + 4 * k2][0]), us4[:, k2].reshape(8 * nu, 128)
                v01 = jnp.concatenate([jnp.where(ev, ur, us), jnp.where(ev, us, ur)], axis=1)
                rv[k1 + 4 * k2, r0:r1, :] = v01.astype(bf16)

    def spectral_inv():
        ev = (_lane(64) & 1) == 0
        at = opaque()
        for j in range(8):
            gri = []
            for a in (2 * j, 2 * j + 1):
                g = gs[at(a)]
                re = [g[0:32, 0:128], g[32:64, 128:256]]
                im = [g[32:64, 0:128], g[0:32, 128:256]]
                gri.append([_bf(jnp.stack([r_.reshape(4, 8, 128), i_.reshape(4, 8, 128)], axis=1).reshape(64, 128))
                            for r_, i_ in zip(re, im)])

            def tile(t):
                zs = [[_dot_nt(gri[c][e], rv[at(2 * j + c), 128 * t:128 * t + 128, 128 * e:128 * e + 128])
                       for e in range(2)] for c in range(2)]
                out = [_pack2(zs[0][0] + zs[0][1], zs[1][0] + zs[1][1]).reshape(4, 2, 16, 128),
                       _pack2(zs[0][0] - zs[0][1], zs[1][0] - zs[1][1]).reshape(4, 2, 16, 128)]
                return [(z[:, 0].reshape(64, 128), z[:, 1].reshape(64, 128)) for z in out]

            even = tile(0)
            odd = tile(1)
            for be in range(2):
                zr, zi = even[be]
                sh = pltpu.roll(zi, 1, axis=1)
                tiles = [jnp.where(ev, zr, sh), jnp.where(ev, sh, zr), odd[be][0], odd[be][1]]
                for t in range(4):
                    z32[t, pl.ds(768 * be + j, 64, stride=12), :] = tiles[t]

    def copy_wo(tok, step):
        tk = _rep(tok(0, 64, step), 4)
        wo32[...] = pltpu.bitcast(wo[...], u32) | jnp.concatenate([tk] * 4, axis=1)

    def xv_part(b, h0, h1):
        lhs = _bf(xe32[dyn(16 * b, 16), :])
        ys = []
        for h in range(h0, h1):
            ys.append(_dot(lhs, _bf(wsl[2 * H + h])))
            xq[b, 2 * H + h] = ys[-1].astype(bf16)
        return ys

    wait(grp[0][0:1])
    for c in range(4):
        relayout(0, r0=32 * c, r1=32 * c + 32)
    wait(grp[0][1:2])
    pack_xe(0)
    x_half(0, 0, 6)

    wait(grp[1])
    tok = tokens(x_half(0, 6, 8)[1:])
    relayout(0, tok, 0, 2, r0=128)
    pack_xe(1, tok)
    x_half(1, 0, 4)
    x_half(1, 4, 6, 0, 256)

    wait(grp[2])
    relayout(1, tokens(x_half(1, 4, 6, 256)[1:] + x_half(1, 6, 8)[1:]), 0, 2)
    x_heads(8, 14)
    x_heads(14, 15, 0, 256)

    wait(grp[3])
    relayout(2, tokens(x_heads(14, 15, 256) + x_heads(15, 16)), 0, 2)
    tok = tokens(x_heads(16, 22))
    gather_x(0, 3, tok, 120)
    build_gs(tok, 5)
    x_heads(22, 23, 0, 256)

    wait(grp[4])
    relayout(3, tokens(x_heads(22, 23, 256) + x_heads(23, 24)), 0, 2)
    gather_x(3, 8, tokens(x_heads(24, 29)), 55)
    spectral_fwd(lambda: x_heads(29, 30))

    wait(grp[5])
    relayout(4, tokens(x_heads(30, 32)), 0, 3)
    tok = tokens(x_heads(32, 40))
    relayout(5, tok, 0, 14)
    spectral_mid(0, 1, 10, tok, 0, 56)
    spectral_mid(1, 0, 6, tokens(x_heads(40, 46)), 0, 54)

    wait(grp[6])
    relayout(6, tokens(x_heads(46, 48)), 0, 3)
    tok = tokens(x_heads(48, 56))
    relayout(7, tok, 0, 7)
    relayout(8, tok, 230, 7)
    dc_filter(tok, 0, 20)
    spectral_mid(0, 10, 16, tok, 0, 66)
    spectral_mid(0, 0, 1, tok, 400, 100)
    tok = tokens(x_heads(56, 62) + x_heads(64, 64 + XVP // 2))
    relayout(9, tok, 0, 16)
    spectral_mid(1, 6, 16, tok, 0, 52)
    spectral_inv()

    wait(grp[7])
    st = x_heads(62, 64) + x_heads(64 + XVP // 2, 64 + XVP) + xv_part(0, XVP, 16)
    tok = tokens(st)
    relayout(10, tok, 0, 4)
    relayout(11, tok, 150, 4)
    copy_wo(tokens(st + xv_part(0, 16, XVL)), 5)
    wait(grp[8])

    r = lax.broadcasted_iota(jnp.int32, (R2, 128), 0)
    c = lax.broadcasted_iota(jnp.int32, (R2, 128), 1)

    def head_pos(i):
        head = jnp.where(i < 32, 0, jnp.where(i < 64, 1, jnp.where(i < 72, 0, jnp.where(i < R2, 1, 2))))
        pos = jnp.where(i < 32, i, jnp.where(i < 72, i - 32, i - 40))
        return head, pos

    rh, rpos = head_pos(r)
    ch, cpos = head_pos(c)
    same = (rh - ch) == 0
    ok = jnp.logical_and(same, jnp.logical_or(rpos < MEM, rpos >= cpos))
    fill = jnp.where(same, jnp.float32(-1e9 / SCALE), jnp.float32(-jnp.inf))

    def step(b, k, mem, filler):
        s = SPB * b + k
        second = k % 2 == 1
        mo = 48 if second else 32
        lhs = jnp.concatenate([mem, xb[s].astype(f32)], axis=0).astype(bf16)
        if not second:
            lhs48 = jnp.concatenate([lhs, _bf(xe32[dyn(4 * s, 8), :])], axis=0)
        acc = [None] * 4
        stream = []

        def proj(m, hp):
            y = jnp.concatenate([_dot(lhs, _bf(wsl[H * m + 2 * hp + hh])) for hh in range(2)], axis=0)
            qsc[m, hp] = y.astype(bf16)
            stream.append(y)

        def oper(m, hp):
            xs = [xq[b, H * m + 2 * hp + hh, XT * k:XT * k + XT, :] for hh in range(2)]
            if m > 0:
                xs.append(jnp.zeros((128 - R2, DH), bf16))
            return jnp.concatenate([qsc[m, hp]] + xs, axis=0)

        def do_qkp(hp):
            proj(0, hp)
            proj(1, hp)

        def do_v(hp):
            if second or 2 * hp < XVL:
                proj(2, hp)
                return
            ys = [_dot(lhs48, _bf(wsl[2 * H + 2 * hp + hh])) for hh in range(2)]
            y = jnp.concatenate([ys[0][0:32], ys[1][0:32]], axis=0)
            qsc[2, hp] = y.astype(bf16)
            for hh in range(2):
                xq[b, 2 * H + 2 * hp + hh, XT * k:XT * k + 2 * XT, :] = ys[hh][32:48].astype(bf16)
            stream.append(y)

        def do_qk(hp):
            ssc[hp] = jnp.where(ok, _dot_nt(oper(0, hp), oper(1, hp)), fill)
            stream.clear()

        def do_softmax(p0, p1):
            nt = 20 if p1 < NP else 5
            g = pltpu.bitcast(_rep(tokens(stream[0:3])(0, nt, 1), 40 // nt), f32)
            sc = ssc[p0:p1].reshape(4 * R2, 128) + g
            mx = jnp.max(sc, axis=-1, keepdims=True)
            e = jnp.exp2((sc - mx) * (SCALE * LOG2E))
            l = jnp.sum(e, axis=-1, keepdims=True)
            rl = pl.reciprocal(l, approx=True)
            rl = rl * (2.0 - l * rl)
            psc[p0:p1] = (e * rl).astype(bf16).reshape(4, R2, 128)

        def do_pv(hp):
            o2 = _dot(psc[hp], oper(2, hp))
            r0 = 40 if second else 32
            for hh in range(2):
                osc[2 * hp + hh, 0:32, :] = o2[32 * hh:32 * hh + 32].astype(bf16)
                osc[2 * hp + hh, r0:r0 + 8, :] = o2[64 + 8 * hh:72 + 8 * hh].astype(bf16)

        def do_o(p0, p1):
            ol = jnp.concatenate([osc[h, 0:mo, :] for h in range(2 * p0, 2 * p1)], axis=1)
            for n in range(4):
                y = _dot(ol, _bf(wo32[p0 * 128:p1 * 128, 128 * n:128 * n + 128]))
                acc[n] = y if acc[n] is None else acc[n] + y
                stream.append(y)

        def do_a3():
            def zrows(t):
                blk = z32.at[t, dyn(24 * s, 48), :]
                return _bf(jnp.concatenate([blk[12 * g:12 * g + 8, :] for g in range(4)], axis=0))
            v0, v2, vc, vs = [_dot(zrows(t), _bf(fi[:, 128 * t:128 * t + 128])) for t in range(4)]
            sp, sm = v0 + v2, v0 - v2
            first = _lane(2 * SEG) == 0
            al, be = vc + jnp.where(first, 0.0, vs), _mirror(vs - jnp.where(first, 0.0, vc))
            ya = jnp.concatenate([sp + al, sm + be, sp - al, sm - be], axis=1).astype(bf16)
            stage[pl.ds(s, 2), :, 0:D] = ya.reshape(2, SEG, D)

        for op in _SCHED:
            if op == 'a':
                if not second:
                    do_a3()
                continue
            p0, p1 = [int(v) for v in op[1:].split('-')]
            if op[0] == 'p':
                do_softmax(p0, p1)
            if op[0] == 'o':
                do_o(p0, p1)
            else:
                for hp in range(p0, p1):
                    {'k': do_qkp, 'v': do_v, 'q': do_qk, 'p': do_pv}[op[0]](hp)
        filler()
        return jnp.concatenate(acc, axis=1)

    nb = NSEG // SPB
    hv = [XVP, 10, 12, 16, XVL]

    def body(b, mem):
        @pl.when(b == 1)
        def _():
            grp[9][0].wait()
        nxt = jnp.minimum(b + 1, nb - 1)
        for k in range(0, SPB, 2):
            sa, sb = SPB * b + k, SPB * b + k + 1
            ya = step(b, k, mem, lambda: xv_part(nxt, hv[k], hv[k + 1]))
            stage[sa, 0:KEEP, D:2 * D] = ya[MEM:].astype(bf16)
            mem_b = ya[0:MEM].astype(bf16).astype(f32)
            yb = step(b, k + 1, mem_b, lambda: xv_part(nxt, hv[k + 1], hv[k + 2]))
            stage[sa, KEEP:SEG, D:2 * D] = yb[32:40].astype(bf16)
            stage[sb, :, D:2 * D] = jnp.concatenate([yb[MEM:32], yb[40:48]], axis=0).astype(bf16)
            mem = yb[0:MEM].astype(bf16).astype(f32)
            rows = pl.ds(sa, 2)
            cp(stage.at[rows], out_hbm.at[rows], _S_OUT).start()
        return mem

    lax.fori_loop(0, nb, body, m0[...].astype(f32))
    wait([cp(stage, out_hbm, _S_OUT)])


@jax.jit
def pallas_concat_heads__spectral_gfnet__memory_aug_recurrent_mem_tr__prompt_kernel(
    A_x: jax.Array,
    A_w_r: jax.Array,
    A_w_i: jax.Array,
    B_x: jax.Array,
    B_mem0: jax.Array,
    B_Wq: jax.Array,
    B_Wk: jax.Array,
    B_Wv: jax.Array,
    B_Wo: jax.Array,
    B_seg_len: jax.Array,
):
    del B_seg_len
    assert A_x.shape == (1, S, D) and B_x.shape == (1, S, D) and B_mem0.shape == (1, MEM, D)
    assert B_Wq.shape == (D, H, DH) and B_Wo.shape == (H, DH, D)
    fd, fi = _dft_tables()
    vm = pltpu.VMEM
    scratch = [
        vm((NSEG, XT, D), bf16),
        vm((NSEG * XT // 2, D), u32),
        vm((2, S // 2, D), bf16),
        vm((4, 2, S // 4, 128), u32),
        vm((NC, 128, D), bf16),
        vm((12, D // 2, 2, 8, DH), bf16),
        vm((2, 2 * D, DH), u32),
        vm((2, 2 * D, DH), u32),
        vm((3 * H, D // 2, DH), u32),
        vm((NSEG // SPB, 3 * H, SPB * XT, DH), bf16),
        vm((104, 512), u32),
        vm((64, 512), u32),
        vm((NC, 64, 256), u32),
        vm((D // 2 + 1, S), bf16),
        vm((D // 2 + 1, S), bf16),
        vm((NC, 2, 256, 128), f32),
        vm((NC, 256, 256), bf16),
        vm((4, NC * 8, 128), f32),
        vm((4, 3 * S // 4, 128), u32),
        vm((H * DH, D), bf16),
        vm((H * DH // 2, D), u32),
        vm((NSEG, KEEP, D), bf16),
        vm((MEM, D), bf16),
        vm((NSEG, SEG, 2 * D), bf16),
        vm((16, 128), u32),
        vm((NP, R2, 128), bf16),
        vm((3, NP, 64, DH), bf16),
        vm((H, 48, DH), bf16),
        vm((NP, R2, 128), f32),
        vm((8, NSEG * XT, DH), f32),
        pltpu.SemaphoreType.DMA((_NGRP + 1,)),
    ]
    w4 = lambda w: w.reshape(D // 2, 2, H, DH)
    out = pl.pallas_call(
        _kernel,
        out_shape=jax.ShapeDtypeStruct((NSEG, SEG, 2 * D), bf16),
        in_specs=[pl.BlockSpec(memory_space=pl.ANY)] * 11,
        out_specs=pl.BlockSpec(memory_space=pl.ANY),
        scratch_shapes=scratch,
        compiler_params=pltpu.CompilerParams(vmem_limit_bytes=110 * 1024 * 1024),
    )(A_x.reshape(2, S // 2, D), A_w_r.T, A_w_i.T, B_x.reshape(NSEG, SEG, D), B_mem0.reshape(MEM, D),
      w4(B_Wq), w4(B_Wk), w4(B_Wv), B_Wo.reshape(H * DH, D), fd, fi)
    return out.reshape(1, S, 2 * D)
```
